```python
import jax
import jax.numpy as jnp

def _softmax(x, axis=-1):
    return jax.nn.softmax(x, axis=axis)

def _gelu(x):
    return jax.nn.gelu(x, approximate=True)

def _silu(x):
    return jax.nn.silu(x)

def _sigmoid(x):
    return jax.nn.sigmoid(x)

def _layernorm(x, axis=-1, eps=1e-05):
    m = jnp.mean(x, axis=axis, keepdims=True)
    v = jnp.var(x, axis=axis, keepdims=True)
    return (x - m) / jnp.sqrt(v + eps)

def _scatter_add(tgt, idx, src, axis=0):
    return tgt.at[idx].add(src)

def _segment_sum(src, seg, n):
    return jax.ops.segment_sum(src, seg, n)

class _Rng:

    def __init__(self, key):
        self._k = key

    def _next(self):
        self._k, sub = jax.random.split(self._k)
        return sub

    def normal(self, shape):
        return jax.random.normal(self._next(), shape, dtype=jnp.bfloat16)

    def randint(self, lo, hi, shape):
        return jax.random.randint(self._next(), shape, lo, hi, dtype=jnp.int32)

    def uniform(self, shape, lo=0.0, hi=1.0):
        return jax.random.uniform(self._next(), shape, jnp.bfloat16, lo, hi)

    def permutation(self, n):
        return jax.random.permutation(self._next(), n)
kernel_name = 'interleave_layers__memory_aug_recurrent_mem_tr__glu_gated_geglu__prompt'

def setup_inputs():
    _rng = _Rng(jax.random.key(int.from_bytes(__import__("os").urandom(4), "little")))
    _w = lambda a: (lambda t: t.astype(jnp.bfloat16) if jnp.issubdtype(t.dtype, jnp.floating) else t)(jnp.asarray(a))

    def _A_setup():
        B, S, Dm = (1, 2048, 1024)
        H, Dh = (32, 128)
        M, seg = (8, 32)
        seg = min(seg, S)
        S = S // seg * seg
        return {'x': _w((lambda *s: _rng.normal(s) * 0.05)(B, S, Dm)), 'mem0': _w((lambda *s: _rng.normal(s) * 0.05)(B, M, Dm)), 'Wq': _w((lambda *s: _rng.normal(s) * 0.05)(Dm, H, Dh) * Dm ** (-0.5)), 'Wk': _w((lambda *s: _rng.normal(s) * 0.05)(Dm, H, Dh) * Dm ** (-0.5)), 'Wv': _w((lambda *s: _rng.normal(s) * 0.05)(Dm, H, Dh) * Dm ** (-0.5)), 'Wo': _w((lambda *s: _rng.normal(s) * 0.05)(H, Dh, Dm) * (H * Dh) ** (-0.5)), 'seg_len': seg}
    _A_in = _A_setup()

    def _B_setup():
        B, S, Dm, Df = (1, 2048, 1024, 3584)
        return {'x': _w((lambda *s: _rng.normal(s) * 0.05)(B, S, Dm)), 'w_gate': _w((lambda *s: _rng.normal(s) * 0.05)(Dm, Df) * Dm ** (-0.5)), 'w_up': _w((lambda *s: _rng.normal(s) * 0.05)(Dm, Df) * Dm ** (-0.5)), 'w_down': _w((lambda *s: _rng.normal(s) * 0.05)(Df, Dm) * Df ** (-0.5))}
    _B_in = _B_setup()
    return {'A_x': _A_in['x'], 'A_mem0': _A_in['mem0'], 'A_Wq': _A_in['Wq'], 'A_Wk': _A_in['Wk'], 'A_Wv': _A_in['Wv'], 'A_Wo': _A_in['Wo'], 'A_seg_len': _A_in['seg_len'], 'B_x': _B_in['x'], 'B_w_gate': _B_in['w_gate'], 'B_w_up': _B_in['w_up'], 'B_w_down': _B_in['w_down']}

def reference(A_x, A_mem0, A_Wq, A_Wk, A_Wv, A_Wo, A_seg_len, B_x, B_w_gate, B_w_up, B_w_down):

    def _A_ref(x, mem0, Wq, Wk, Wv, Wo, seg_len):
        B, S, Dm = x.shape
        H, Dh = (Wq.shape[1], Wq.shape[2])
        M = mem0.shape[1]
        scale = Dh ** (-0.5)
        n_seg = S // seg_len
        L = M + seg_len
        idx = jnp.arange(L)
        mask = (idx[:, None] < M) | (idx[:, None] >= idx[None, :])
        mem = mem0
        outs = []
        for s in range(n_seg):
            xs = x[:, s * seg_len:(s + 1) * seg_len, :].copy()
            h = jnp.concatenate([mem, xs], axis=1)
            q = jnp.einsum('btd,dhe->bhte', h, Wq)
            k = jnp.einsum('btd,dhe->bhte', h, Wk)
            v = jnp.einsum('btd,dhe->bhte', h, Wv)
            scores = jnp.einsum('bhqe,bhke->bhqk', q, k) * scale
            scores = jnp.where(mask[None, None], scores, -1000000000.0)
            p = _softmax(scores, axis=-1)
            o = jnp.einsum('bhqk,bhke->bhqe', p, v)
            o = jnp.einsum('bhte,hed->btd', o, Wo)
            mem = o[:, :M, :].copy()
            outs.append(o[:, M:, :])
        return jnp.concatenate(outs, axis=1)

    def _B_ref(x, w_gate, w_up, w_down):
        g = jnp.einsum('bsd,df->bsf', x, w_gate)
        u = jnp.einsum('bsd,df->bsf', x, w_up)
        h = _gelu(g) * u
        return jnp.einsum('bsf,fd->bsd', h, w_down)
    x = A_x
    x = x + _A_ref(_layernorm(x, axis=-1), A_mem0, A_Wq, A_Wk, A_Wv, A_Wo, A_seg_len)
    x = x + _B_ref(_layernorm(x, axis=-1), B_w_gate, B_w_up, B_w_down)
    x = x + _A_ref(_layernorm(x, axis=-1), A_mem0, A_Wq, A_Wk, A_Wv, A_Wo, A_seg_len)
    x = x + _B_ref(_layernorm(x, axis=-1), B_w_gate, B_w_up, B_w_down)
    return x
```

```python
import functools
import jax
import jax.numpy as jnp
import numpy as np
import jax.experimental.pallas as pl
import jax.experimental.pallas.tpu as pltpu

F32 = jnp.float32
BF16 = jnp.bfloat16
LOG2E = 1.4426950408889634


def _ln(x):
    m = jnp.mean(x, axis=-1, keepdims=True)
    d = x - m
    v = jnp.mean(d * d, axis=-1, keepdims=True)
    return d * jax.lax.rsqrt(v + 1e-5)


def _gelu(x):
    c = 0.7978845608028654
    return 0.5 * x * (1.0 + jnp.tanh(c * (x + 0.044715 * (x * x * x))))


def build(cfg):
    G = cfg.get("G", 4)
    FC = cfg.get("FC", 512)
    CS = 2

    def kernel(x_ref, mem0_ref, wq_ref, wk_ref, wv_ref, wo_ref, wg_ref, wu_ref, wd_ref, o_ref,
               xs_ref, mem_ref, h_ref, *, M, seg, H, Dh, n_chunks):
        c = pl.program_id(0)
        CH = CS * seg
        R = 2 * (M + seg)
        scale = Dh ** -0.5

        @pl.when(c == 0)
        def _():
            xs_ref[CH:2 * CH, :] = jnp.zeros((CH, xs_ref.shape[1]), F32)
            mem_ref[0:M, :] = mem0_ref[...].astype(F32)

        @pl.when(c <= 1)
        def _():
            mem_ref[M:2 * M, :] = mem0_ref[...].astype(F32)

        xs_ref[0:CH, :] = x_ref[...].astype(F32)

        ri = jax.lax.broadcasted_iota(jnp.int32, (R, 128), 0)
        ci = jax.lax.broadcasted_iota(jnp.int32, (R, 128), 1)

        def layer_pos(i):
            lay = jnp.where(i < 2 * M, (i >= M).astype(jnp.int32), (i >= 2 * M + seg).astype(jnp.int32))
            pos = jnp.where(i < 2 * M, i - lay * M, i - M - lay * seg)
            return lay, pos
        rl, rp = layer_pos(ri)
        cl, cp = layer_pos(ci)
        same = (rl == cl) & (ci < R)
        keep = same & ((rp < M) | (rp >= cp))
        fill = jnp.where(same, -1e9, -jnp.inf).astype(F32)

        def a_step(j, carry):
            r1 = pl.multiple_of(j * seg, seg)
            r2 = pl.multiple_of(CH + j * seg, seg)
            h_ref[0:2 * M, :] = mem_ref[...].astype(BF16)
            h_ref[2 * M:2 * M + seg, :] = _ln(xs_ref[pl.ds(r1, seg), :]).astype(BF16)
            h_ref[2 * M + seg:R, :] = _ln(xs_ref[pl.ds(r2, seg), :]).astype(BF16)
            h = h_ref[...]
            acc = None
            for g in range(H // G):
                cs = slice(g * G * Dh, (g + 1) * G * Dh)
                q = jnp.dot(h, wq_ref[:, cs], preferred_element_type=F32).astype(BF16)
                k = jnp.dot(h, wk_ref[:, cs], preferred_element_type=F32).astype(BF16)
                v = jnp.dot(h, wv_ref[:, cs], preferred_element_type=F32).astype(BF16)
                os = []
                z = jnp.zeros((128 - R, Dh), BF16)
                for i in range(G):
                    hs = slice(i * Dh, (i + 1) * Dh)
                    kp = jnp.concatenate([k[:, hs], z], axis=0)
                    vp = jnp.concatenate([v[:, hs], z], axis=0)
                    s = jax.lax.dot_general(q[:, hs], kp, (((1,), (1,)), ((), ())), preferred_element_type=F32)
                    s = jnp.where(keep, s * scale, fill)
                    m = jnp.max(s, axis=-1, keepdims=True)
                    e = jnp.exp(s - m)
                    l = jnp.sum(e, axis=-1, keepdims=True)
                    p = (e * pl.reciprocal(l, approx=False)).astype(BF16)
                    os.append(jnp.dot(p, vp, preferred_element_type=F32).astype(BF16))
                o = jnp.concatenate(os, axis=1)
                t = jnp.dot(o, wo_ref[cs, :], preferred_element_type=F32)
                acc = t if acc is None else acc + t
            mem_ref[...] = acc[0:2 * M]
            xs_ref[pl.ds(r1, seg), :] += acc[2 * M:2 * M + seg]
            xs_ref[pl.ds(r2, seg), :] += acc[2 * M + seg:R]
            return carry

        jax.lax.fori_loop(0, CS, a_step, 0)

        xs = xs_ref[...]
        hb = _ln(xs).astype(BF16)
        acc = xs
        DF = wg_ref.shape[1]
        for f in range(DF // FC):
            cs = slice(f * FC, (f + 1) * FC)
            g = jnp.dot(hb, wg_ref[:, cs], preferred_element_type=F32)
            u = jnp.dot(hb, wu_ref[:, cs], preferred_element_type=F32)
            a = (_gelu(g) * u).astype(BF16)
            acc = acc + jnp.dot(a, wd_ref[cs, :], preferred_element_type=F32)
        xs_ref[CH:2 * CH, :] = acc[0:CH]
        o_ref[...] = acc[CH:2 * CH].astype(o_ref.dtype)

    @functools.partial(jax.jit, static_argnames=("A_seg_len",))
    def run(A_x, A_mem0, A_Wq, A_Wk, A_Wv, A_Wo, A_seg_len, B_x, B_w_gate, B_w_up, B_w_down):
        B, S, Dm = A_x.shape
        H, Dh = A_Wq.shape[1:]
        M = A_mem0.shape[1]
        seg = A_seg_len
        CH = CS * seg
        n_chunks = S // CH
        DF = B_w_gate.shape[1]
        one = pl.Buffered(1)
        full = lambda shape: pl.BlockSpec(shape, lambda c: (0, 0), pipeline_mode=one)
        out = pl.pallas_call(
            functools.partial(kernel, M=M, seg=seg, H=H, Dh=Dh, n_chunks=n_chunks),
            grid=(n_chunks + 1,),
            in_specs=[
                pl.BlockSpec((CH, Dm), lambda c: (jnp.minimum(c, n_chunks - 1), 0)),
                full((M, Dm)),
                full((Dm, H * Dh)), full((Dm, H * Dh)), full((Dm, H * Dh)), full((H * Dh, Dm)),
                full((Dm, DF)), full((Dm, DF)), full((DF, Dm)),
            ],
            out_specs=pl.BlockSpec((CH, Dm), lambda c: (jnp.maximum(c - 1, 0), 0)),
            out_shape=jax.ShapeDtypeStruct((S, Dm), A_x.dtype),
            scratch_shapes=[
                pltpu.VMEM((2 * CH, Dm), F32),
                pltpu.VMEM((2 * M, Dm), F32),
                pltpu.VMEM((2 * (M + seg), Dm), BF16),
            ],
            compiler_params=pltpu.CompilerParams(
                dimension_semantics=("arbitrary",), vmem_limit_bytes=110 * 1024 * 1024),
        )(A_x.reshape(S, Dm), A_mem0.reshape(M, Dm),
          A_Wq.reshape(Dm, H * Dh), A_Wk.reshape(Dm, H * Dh), A_Wv.reshape(Dm, H * Dh),
          A_Wo.reshape(H * Dh, Dm), B_w_gate, B_w_up, B_w_down)
        return out.reshape(B, S, Dm)
    return run


_run = build({})


@functools.partial(jax.jit, static_argnames=("A_seg_len",))
def pallas_interleave_layers__memory_aug_recurrent_mem_tr__glu_gated_geglu__prompt_kernel(
    A_x, A_mem0, A_Wq, A_Wk, A_Wv, A_Wo, A_seg_len, B_x, B_w_gate, B_w_up, B_w_down
):
    return _run(A_x, A_mem0, A_Wq, A_Wk, A_Wv, A_Wo, A_seg_len, B_x, B_w_gate, B_w_up, B_w_down)
```

```python
import functools
import jax
import jax.numpy as jnp
import numpy as np
import jax.experimental.pallas as pl
import jax.experimental.pallas.tpu as pltpu

F32 = jnp.float32
BF16 = jnp.bfloat16
U32 = jnp.uint32


def _ln(x):
    m = jnp.mean(x, axis=-1, keepdims=True)
    d = x - m
    v = jnp.mean(d * d, axis=-1, keepdims=True)
    return d * jax.lax.rsqrt(v + 1e-5)


def _gelu(x):
    c = 0.7978845608028654
    return 0.5 * x * (1.0 + jnp.tanh(c * (x + 0.044715 * (x * x * x))))


def build(cfg):
    G = cfg.get("G", 2)
    FC = cfg.get("FC", 512)
    CS = 2
    RC = cfg.get("RC", 128)
    NS = cfg.get("NS", 4)
    UNROLL = cfg.get("unroll", 0)

    def kernel(x_h, mem0_ref, wq_h, wk_h, wv_h, wo_h, wg_h, wu_h, wd_h, o_h,
               wq_ref, wk_ref, wv_ref, wo_ref, wg_ref, wu_ref, wd_ref, stage_ref,
               xs_ref, mem_ref, x_ref, o_ref, sem_s, sem_o, sem_f, sem_x, sem_out, *, M, seg, H, Dh, n_chunks):
        CH = CS * seg
        Dm = xs_ref.shape[1]
        DF = wg_ref.shape[1]
        scale = Dh ** -0.5
        NG = H // G
        NF = DF // FC
        cs = lambda g: slice(g * G * Dh, (g + 1) * G * Dh)
        fs = lambda f: slice(f * FC, (f + 1) * FC)
        hsl = lambda i: slice(i * Dh, (i + 1) * Dh)

        NRC = Dm // RC
        raw = [(src, dst, r) for src, dst in ((wq_h, wq_ref), (wk_h, wk_ref), (wv_h, wv_ref)) for r in range(NRC)]

        def raw_copy(i):
            src, _, r = raw[i]
            return pltpu.make_async_copy(src.at[pl.ds(r * RC * H, RC * H), :], stage_ref.at[i % NS], sem_s.at[i % NS])

        NO = 8
        OR = H * Dh // NO

        def wo_copy(i):
            return pltpu.make_async_copy(wo_h.at[pl.ds(i * OR, OR), :], wo_ref.at[pl.ds(i * OR, OR), :], sem_o.at[i])

        def ffn_copy(i):
            f, w = divmod(i, 3)
            if w == 0:
                return pltpu.make_async_copy(wg_h.at[:, fs(f)], wg_ref.at[:, fs(f)], sem_f.at[i])
            if w == 1:
                return pltpu.make_async_copy(wu_h.at[:, fs(f)], wu_ref.at[:, fs(f)], sem_f.at[i])
            return pltpu.make_async_copy(wd_h.at[fs(f), :], wd_ref.at[fs(f), :], sem_f.at[i])

        queue = [raw_copy(i) for i in range(len(raw))] + [wo_copy(i) for i in range(NO)] + [ffn_copy(i) for i in range(3 * NF)]
        state = {"next": 0}

        def start_upto(n):
            while state["next"] < min(n, len(queue)):
                queue[state["next"]].start()
                state["next"] += 1

        def relayout(i):
            _, dst, r = raw[i]
            u = stage_ref.at[i % NS].bitcast(U32)
            HP = H // 2

            def body(b, carry):
                d0 = pl.multiple_of(b * 16, 16)
                ub = u.at[pl.ds(pl.multiple_of(b * (16 * HP), 16 * HP), 16 * HP), :]
                for j in range(HP):
                    a = ub[pl.ds(j, 8, stride=2 * HP), :]
                    bb = ub[pl.ds(HP + j, 8, stride=2 * HP), :]
                    ev = (a & 0xFFFF) | (bb << 16)
                    od = (a >> 16) | (bb & jnp.uint32(0xFFFF0000))
                    rows = pl.ds(pl.multiple_of(r * RC + d0, 16), 16)
                    dst[rows, hsl(2 * j)] = pltpu.bitcast(ev, BF16)
                    dst[rows, hsl(2 * j + 1)] = pltpu.bitcast(od, BF16)
                return carry
            jax.lax.fori_loop(0, RC // 16, body, 0)

        def load_qkv():
            start_upto(NS)
            for i in range(len(raw)):
                queue[i].wait()
                if not cfg.get('norelayout'):
                    relayout(i)
                start_upto(i + NS + 1)

        def a_step(j, layers, wait_wo=None):
            nl = len(layers)
            R = 2 * M + nl * seg
            ri = jax.lax.broadcasted_iota(jnp.int32, (R, 128), 0)
            ci = jax.lax.broadcasted_iota(jnp.int32, (R, 128), 1)

            def layer_pos(i):
                tok = jnp.where(i >= 2 * M + seg, layers[-1], layers[0])
                lay = jnp.where(i < 2 * M, (i >= M).astype(jnp.int32), tok)
                pos = jnp.where(i < 2 * M, i - lay * M, i - M - (i >= 2 * M + seg).astype(jnp.int32) * seg)
                return lay, pos
            rl, rp = layer_pos(ri)
            cl, cp = layer_pos(ci)
            same = (rl == cl) & (ci < R)
            keep = same & ((rp < M) | (rp >= cp))
            fill = jnp.where(same, -1e9, -jnp.inf).astype(F32)

            def rows(l):
                r = l * CH + j * seg
                return pl.ds(r if isinstance(r, int) else pl.multiple_of(r, seg), seg)

            h = jnp.concatenate([mem_ref[...].astype(BF16)] + [_ln(xs_ref[rows(l), :]).astype(BF16) for l in layers], axis=0)
            z = jnp.zeros((128 - R, Dh), BF16)
            proj = lambda w, g: jnp.dot(h, w[:, cs(g)], preferred_element_type=F32).astype(BF16)

            def qk(q, k):
                return [jax.lax.dot_general(q[:, hsl(i)], jnp.concatenate([k[:, hsl(i)], z], axis=0),
                                            (((1,), (1,)), ((), ())), preferred_element_type=F32) for i in range(G)]

            def softmax(ss):
                ps = []
                for s in ss:
                    s = jnp.where(keep, s * scale, fill)
                    m = jnp.max(s, axis=-1, keepdims=True)
                    e = jnp.exp(s - m)
                    l = jnp.sum(e, axis=-1, keepdims=True)
                    ps.append((e * pl.reciprocal(l, approx=False)).astype(BF16))
                return ps

            def pv(ps, v):
                return jnp.concatenate(
                    [jnp.dot(ps[i], jnp.concatenate([v[:, hsl(i)], z], axis=0), preferred_element_type=F32).astype(BF16)
                     for i in range(G)], axis=1)

            def wo(o, g):
                if wait_wo is not None:
                    wait_wo(g)
                return jnp.dot(o, wo_ref[cs(g), :], preferred_element_type=F32)

            acc = None
            o_prev = None
            q = proj(wq_ref, 0)
            k = proj(wk_ref, 0)
            for g in range(NG):
                v = proj(wv_ref, g)
                ss = qk(q, k)
                if g + 1 < NG:
                    q = proj(wq_ref, g + 1)
                if o_prev is not None:
                    t = wo(o_prev, g - 1)
                    acc = t if acc is None else acc + t
                o_prev = pv(softmax(ss), v)
                if g + 1 < NG:
                    k = proj(wk_ref, g + 1)
            acc = acc + wo(o_prev, NG - 1)
            mem_ref[...] = acc[0:2 * M]
            for n, l in enumerate(layers):
                xs_ref[rows(l), :] += acc[2 * M + n * seg:2 * M + (n + 1) * seg]

        def chunk(c):
            return pl.ds(c * CH if isinstance(c, int) else pl.multiple_of(c * CH, CH), CH)

        def out_copy(c):
            return pltpu.make_async_copy(o_ref.at[chunk(c), :], o_h.at[chunk(c), :], sem_out)

        def b_step(c, layers, wait_f=None):
            xs = xs_ref[layers[0] * CH:(layers[-1] + 1) * CH, :]
            hb = _ln(xs).astype(BF16)
            acc = xs
            for f in range(NF):
                if wait_f is not None:
                    wait_f(f)
                g = jnp.dot(hb, wg_ref[:, fs(f)], preferred_element_type=F32)
                u = jnp.dot(hb, wu_ref[:, fs(f)], preferred_element_type=F32)
                a = (_gelu(g) * u).astype(BF16)
                acc = acc + jnp.dot(a, wd_ref[fs(f), :], preferred_element_type=F32)
            for n, l in enumerate(layers):
                if l == 0:
                    xs_ref[CH:2 * CH, :] = acc[n * CH:(n + 1) * CH]
                else:
                    o_ref[chunk(c - 1), :] = acc[n * CH:(n + 1) * CH].astype(o_ref.dtype)
                    out_copy(c - 1).start()

        def a_steps(layers):
            if UNROLL:
                for j in range(CS):
                    a_step(j, layers)
            else:
                def body(j, carry):
                    a_step(j, layers)
                    return carry
                jax.lax.fori_loop(0, CS, body, 0)

        x_first = pltpu.make_async_copy(x_h.at[0:CH, :], x_ref.at[0:CH, :], sem_x.at[0])
        S = x_ref.shape[0]
        x_rest = pltpu.make_async_copy(x_h.at[CH:S, :], x_ref.at[CH:S, :], sem_x.at[1])
        queue.append(x_rest)

        x_first.start()
        load_qkv()
        nr = len(raw)
        m0 = mem0_ref[...].astype(F32)
        mem_ref[0:M, :] = m0
        mem_ref[M:2 * M, :] = m0
        x_first.wait()
        xs_ref[0:CH, :] = x_ref[0:CH, :].astype(F32)

        def wait_wo(g):
            r0 = g * G * Dh
            if r0 % OR == 0:
                i = nr + r0 // OR
                queue[i].wait()
                start_upto(i + NS + 1)
        a_step(0, (0,), wait_wo)
        start_upto(len(queue))
        for j in range(1, CS):
            a_step(j, (0,))
        mem_ref[M:2 * M, :] = mem0_ref[...].astype(F32)

        def wait_f(f):
            for w in range(3):
                queue[nr + NO + 3 * f + w].wait()
        b_step(0, (0,), wait_f)
        x_rest.wait()

        def steady(c, carry):
            xs_ref[0:CH, :] = x_ref[chunk(c), :].astype(F32)
            a_steps((0, 1))
            b_step(c, (0, 1))
            return carry
        jax.lax.fori_loop(1, n_chunks, steady, 0)

        a_steps((1,))
        b_step(n_chunks, (1,))
        for c in range(n_chunks):
            out_copy(c).wait()

    @functools.partial(jax.jit, static_argnames=("A_seg_len",))
    def run(A_x, A_mem0, A_Wq, A_Wk, A_Wv, A_Wo, A_seg_len, B_x, B_w_gate, B_w_up, B_w_down):
        B, S, Dm = A_x.shape
        H, Dh = A_Wq.shape[1:]
        M = A_mem0.shape[1]
        seg = A_seg_len
        CH = CS * seg
        n_chunks = cfg.get('nc', S // CH)
        DF = B_w_gate.shape[1]
        hbm = pl.BlockSpec(memory_space=pl.ANY)
        out = pl.pallas_call(
            functools.partial(kernel, M=M, seg=seg, H=H, Dh=Dh, n_chunks=n_chunks),
            in_specs=[hbm, pl.BlockSpec(memory_space=pltpu.VMEM), hbm, hbm, hbm, hbm, hbm, hbm, hbm],
            out_specs=hbm,
            out_shape=jax.ShapeDtypeStruct((S, Dm), A_x.dtype),
            scratch_shapes=[
                pltpu.VMEM((Dm, H * Dh), BF16), pltpu.VMEM((Dm, H * Dh), BF16), pltpu.VMEM((Dm, H * Dh), BF16),
                pltpu.VMEM((H * Dh, Dm), BF16),
                pltpu.VMEM((Dm, DF), BF16), pltpu.VMEM((Dm, DF), BF16), pltpu.VMEM((DF, Dm), BF16),
                pltpu.VMEM((NS, RC * H, Dh), BF16),
                pltpu.VMEM((2 * CH, Dm), F32),
                pltpu.VMEM((2 * M, Dm), F32),
                pltpu.VMEM((S, Dm), BF16),
                pltpu.VMEM((S, Dm), A_x.dtype),
                pltpu.SemaphoreType.DMA((NS,)),
                pltpu.SemaphoreType.DMA((8,)),
                pltpu.SemaphoreType.DMA((3 * (DF // FC),)),
                pltpu.SemaphoreType.DMA((2,)),
                pltpu.SemaphoreType.DMA(()),
            ],
            compiler_params=pltpu.CompilerParams(
                vmem_limit_bytes=110 * 1024 * 1024),
        )(A_x.reshape(S, Dm), A_mem0.reshape(M, Dm),
          A_Wq.reshape(Dm * H, Dh), A_Wk.reshape(Dm * H, Dh), A_Wv.reshape(Dm * H, Dh),
          A_Wo.reshape(H * Dh, Dm), B_w_gate, B_w_up, B_w_down)
        return out.reshape(B, S, Dm)
    return run


_run = build({})


@functools.partial(jax.jit, static_argnames=("A_seg_len",))
def pallas_interleave_layers__memory_aug_recurrent_mem_tr__glu_gated_geglu__prompt_kernel(
    A_x, A_mem0, A_Wq, A_Wk, A_Wv, A_Wo, A_seg_len, B_x, B_w_gate, B_w_up, B_w_down
):
    return _run(A_x, A_mem0, A_Wq, A_Wk, A_Wv, A_Wo, A_seg_len, B_x, B_w_gate, B_w_up, B_w_down)
```

```python
import functools
import jax
import jax.numpy as jnp
import numpy as np
import jax.experimental.pallas as pl
import jax.experimental.pallas.tpu as pltpu

F32 = jnp.float32
BF16 = jnp.bfloat16
U32 = jnp.uint32


def _ln(x):
    m = jnp.mean(x, axis=-1, keepdims=True)
    d = x - m
    v = jnp.mean(d * d, axis=-1, keepdims=True)
    return (d * jax.lax.rsqrt(v + 1e-5)).astype(BF16)


def _gelu(x):
    c = 0.7978845608028654
    return 0.5 * x * (1.0 + jnp.tanh(c * (x + 0.044715 * (x * x * x))))


def _dot(a, b):
    return jnp.dot(a, b, preferred_element_type=F32)


def build(cfg):
    G = cfg.get("G", 2)
    FC = cfg.get("FC", 512)
    RC = cfg.get("RC", 256)
    NS = cfg.get("NS", 2)
    LAG = cfg.get("lag", 2)
    NO = 8

    def kernel(x_h, mem0_ref, wq_h, wk_h, wv_h, wo_h, wg_h, wu_h, wd_h, o_h,
               wq_ref, wk_ref, wv_ref, wo_ref, wg_ref, wu_ref, wd_ref, stage_ref,
               xs_ref, hc_ref, hn_ref, hb_ref, x_ref, y_ref, out_ref,
               sem_s, sem_o, sem_f, sem_x, sem_out, *, M, seg, H, Dh, n_seg):
        Dm = xs_ref.shape[1]
        DF = wg_ref.shape[1]
        scale = Dh ** -0.5
        NG = H // G
        NF = DF // FC
        S2 = 2 * seg
        cs = lambda g: slice(g * G * Dh, (g + 1) * G * Dh)
        fs = lambda f: slice(f * FC, (f + 1) * FC)
        hsl = lambda i: slice(i * Dh, (i + 1) * Dh)

        def aligned(r, n):
            return pl.ds(r if isinstance(r, int) else pl.multiple_of(r, seg), n)

        NRC = Dm // RC
        raw = [(src, dst, r) for src, dst in ((wq_h, wq_ref), (wk_h, wk_ref), (wv_h, wv_ref)) for r in range(NRC)]
        nr = len(raw)
        OR = H * Dh // NO

        def raw_copy(i):
            src, _, r = raw[i]
            return pltpu.make_async_copy(src.at[pl.ds(r * RC * H, RC * H), :], stage_ref.at[i % NS], sem_s.at[i % NS])

        def wo_copy(i):
            return pltpu.make_async_copy(wo_h.at[pl.ds(i * OR, OR), :], wo_ref.at[pl.ds(i * OR, OR), :], sem_o.at[i])

        def ffn_copy(i):
            f, w = divmod(i, 3)
            if w == 0:
                return pltpu.make_async_copy(wg_h.at[:, fs(f)], wg_ref.at[:, fs(f)], sem_f.at[i])
            if w == 1:
                return pltpu.make_async_copy(wu_h.at[:, fs(f)], wu_ref.at[:, fs(f)], sem_f.at[i])
            return pltpu.make_async_copy(wd_h.at[fs(f), :], wd_ref.at[fs(f), :], sem_f.at[i])

        queue = [raw_copy(i) for i in range(nr)] + [wo_copy(i) for i in range(NO)] + [ffn_copy(i) for i in range(3 * NF)]
        started = [0]

        def start_upto(n):
            while started[0] < min(n, len(queue)):
                queue[started[0]].start()
                started[0] += 1

        def relayout(i):
            _, dst, r = raw[i]
            u = stage_ref.at[i % NS].bitcast(U32)
            HP = H // 2

            def body(b, carry):
                ub = u.at[pl.ds(pl.multiple_of(b * (16 * HP), 16 * HP), 16 * HP), :]
                rows = pl.ds(pl.multiple_of(r * RC + b * 16, 16), 16)
                for j in range(HP):
                    a = ub[pl.ds(j, 8, stride=2 * HP), :]
                    bb = ub[pl.ds(HP + j, 8, stride=2 * HP), :]
                    ev = (a & 0xFFFF) | (bb << 16)
                    od = (a >> 16) | (bb & jnp.uint32(0xFFFF0000))
                    dst[rows, hsl(2 * j)] = pltpu.bitcast(ev, BF16)
                    dst[rows, hsl(2 * j + 1)] = pltpu.bitcast(od, BF16)
                return carry
            jax.lax.fori_loop(0, RC // 16, body, 0)

        def segs(t, n=1):
            return aligned(t * seg, n * seg)

        x_first = pltpu.make_async_copy(x_h.at[0:4 * seg, :], x_ref.at[0:4 * seg, :], sem_x.at[0])
        x_rest = pltpu.make_async_copy(x_h.at[4 * seg:n_seg * seg, :], x_ref.at[4 * seg:n_seg * seg, :], sem_x.at[1])

        def out_copy(t, n):
            return pltpu.make_async_copy(out_ref.at[segs(t, n), :], o_h.at[segs(t, n), :], sem_out)

        def attention(h, lays, wait_wo=None):
            R = h.shape[0]
            ri = jax.lax.broadcasted_iota(jnp.int32, (R, 128), 0)
            ci = jax.lax.broadcasted_iota(jnp.int32, (R, 128), 1)

            def layer_pos(i):
                tok = jnp.where(i >= 2 * M + seg, lays[-1], lays[0])
                lay = jnp.where(i < 2 * M, (i >= M).astype(jnp.int32), tok)
                pos = jnp.where(i < 2 * M, i - lay * M, i - M - (i >= 2 * M + seg).astype(jnp.int32) * seg)
                return lay, pos
            rl, rp = layer_pos(ri)
            cl, cp = layer_pos(ci)
            same = (rl == cl) & (ci < R)
            keep = same & ((rp < M) | (rp >= cp))
            fill = jnp.where(same, -1e9, -jnp.inf).astype(F32)
            z = jnp.zeros((128 - R, Dh), BF16)
            proj = lambda w, g: _dot(h, w[:, cs(g)]).astype(BF16)

            def qk(q, k):
                return [jax.lax.dot_general(q[:, hsl(i)], jnp.concatenate([k[:, hsl(i)], z], axis=0),
                                            (((1,), (1,)), ((), ())), preferred_element_type=F32) for i in range(G)]

            def softmax(ss):
                ps = []
                for s in ss:
                    s = jnp.where(keep, s * scale, fill)
                    m = jnp.max(s, axis=-1, keepdims=True)
                    e = jnp.exp(s - m)
                    l = jnp.sum(e, axis=-1, keepdims=True)
                    ps.append((e * pl.reciprocal(l, approx=False)).astype(BF16))
                return ps

            def pv(ps, v):
                return jnp.concatenate(
                    [_dot(ps[i], jnp.concatenate([v[:, hsl(i)], z], axis=0)).astype(BF16) for i in range(G)], axis=1)

            acc = [None]
            os = {}

            def wo(g):
                if g < 0:
                    return
                if wait_wo is not None:
                    wait_wo(g)
                t = _dot(os.pop(g), wo_ref[cs(g), :])
                acc[0] = t if acc[0] is None else acc[0] + t

            q = proj(wq_ref, 0)
            k = proj(wk_ref, 0)
            for g in range(NG):
                v = proj(wv_ref, g)
                ss = qk(q, k)
                if g + 1 < NG:
                    q = proj(wq_ref, g + 1)
                wo(g - LAG)
                os[g] = pv(softmax(ss), v)
                if g + 1 < NG:
                    k = proj(wk_ref, g + 1)
            for g in range(NG - LAG, NG):
                wo(g)
            return acc[0]

        def ffn(lazy):
            def hidden(hb, f):
                return (_gelu(_dot(hb, wg_ref[:, fs(f)])) * _dot(hb, wu_ref[:, fs(f)])).astype(BF16)
            if lazy:
                ha = hb_ref[...]
                hbb = _ln(xs_ref[S2:2 * S2, :])
                prev = jnp.concatenate([hidden(ha, 0), hidden(hbb, 0)], axis=0)
                hb = jnp.concatenate([ha, hbb], axis=0)
            else:
                hb = _ln(xs_ref[...])
                prev = hidden(hb, 0)
            acc = xs_ref[...]
            for f in range(1, NF):
                a = hidden(hb, f)
                acc = acc + _dot(prev, wd_ref[fs(f - 1), :])
                prev = a
            return acc + _dot(prev, wd_ref[fs(NF - 1), :])

        R1 = 2 * M + seg
        R2 = 2 * M + 2 * seg

        def single(j, lay, x, wait_wo=None):
            h = jnp.concatenate([hc_ref[0:2 * M, :], _ln(x)], axis=0)
            acc = attention(h, (lay,), wait_wo)
            hc_ref[0:2 * M, :] = acc[0:2 * M].astype(BF16)
            xs_ref[segs(j), :] = x + acc[2 * M:R1]

        x_first.start()
        start_upto(NS)
        for i in range(nr):
            queue[i].wait()
            relayout(i)
            start_upto(i + NS + 1)
        m0 = mem0_ref[...].astype(F32)
        hc_ref[0:2 * M, :] = jnp.concatenate([m0, m0], axis=0).astype(BF16)
        x_first.wait()

        def wait_wo(g):
            r0 = g * G * Dh
            if r0 % OR == 0:
                i = nr + r0 // OR
                queue[i].wait()
                start_upto(i + NS + 2)
        single(0, 0, x_ref[segs(0), :].astype(F32), wait_wo)
        start_upto(len(queue))

        def pro(j, carry):
            single(j, 0, x_ref[segs(j), :].astype(F32))
            return carry
        jax.lax.fori_loop(1, 4, pro, 0)
        m1 = hc_ref[0:2 * M, :].astype(F32)[0:M]
        hc_ref[0:2 * M, :] = jnp.concatenate([m1, mem0_ref[...].astype(F32)], axis=0).astype(BF16)
        for i in range(nr + NO, len(queue)):
            queue[i].wait()
        x_rest.start()
        y_ref[0:4 * seg, :] = ffn(False)
        x_rest.wait()
        hc_ref[2 * M:R1, :] = _ln(x_ref[segs(4), :].astype(F32))
        hc_ref[R1:R2, :] = _ln(y_ref[segs(0), :])

        def a_step(c, j):
            t = 2 * c + j
            hn_ref[0:seg, :] = _ln(x_ref[segs(jnp.minimum(t + 5, n_seg - 1)), :].astype(F32))
            hn_ref[seg:S2, :] = _ln(y_ref[segs(t + 1), :])
            hb_ref[...] = _ln(xs_ref[0:S2, :])
            acc = attention(hc_ref[...], (0, 1))
            hc_ref[2 * M:R2, :] = hn_ref[...]
            hc_ref[0:2 * M, :] = acc[0:2 * M].astype(BF16)
            xs_ref[segs(2 * j), :] = x_ref[segs(t + 4), :].astype(F32) + acc[2 * M:R1]
            xs_ref[segs(2 * j + 1), :] = y_ref[segs(t), :] + acc[R1:R2]

        def steady(c, carry):
            jax.lax.fori_loop(0, 2, lambda j, z: (a_step(c, j), z)[1], 0)
            r = ffn(True)
            for j in range(2):
                y_ref[segs(2 * c + 4 + j), :] = r[j * S2:j * S2 + seg]
                out_ref[segs(2 * c + j), :] = r[j * S2 + seg:(j + 1) * S2].astype(out_ref.dtype)
            out_copy(2 * c, 2).start()
            return carry
        NC = (n_seg - 4) // 2
        jax.lax.fori_loop(0, NC, steady, 0)

        def epi(j, carry):
            single(j, 1, y_ref[segs(n_seg - 4 + j), :])
            return carry
        jax.lax.fori_loop(0, 4, epi, 0)
        out_ref[segs(n_seg - 4, 4), :] = ffn(False).astype(out_ref.dtype)
        out_copy(n_seg - 4, 4).start()
        for c in range(NC):
            out_copy(2 * c, 2).wait()
        out_copy(n_seg - 4, 4).wait()

    @functools.partial(jax.jit, static_argnames=("A_seg_len",))
    def run(A_x, A_mem0, A_Wq, A_Wk, A_Wv, A_Wo, A_seg_len, B_x, B_w_gate, B_w_up, B_w_down):
        B, S, Dm = A_x.shape
        H, Dh = A_Wq.shape[1:]
        M = A_mem0.shape[1]
        seg = A_seg_len
        DF = B_w_gate.shape[1]
        hbm = pl.BlockSpec(memory_space=pl.ANY)
        out = pl.pallas_call(
            functools.partial(kernel, M=M, seg=seg, H=H, Dh=Dh, n_seg=cfg.get("ns", S // seg)),
            in_specs=[hbm, pl.BlockSpec(memory_space=pltpu.VMEM), hbm, hbm, hbm, hbm, hbm, hbm, hbm],
            out_specs=hbm,
            out_shape=jax.ShapeDtypeStruct((S, Dm), A_x.dtype),
            scratch_shapes=[
                pltpu.VMEM((Dm, H * Dh), BF16), pltpu.VMEM((Dm, H * Dh), BF16), pltpu.VMEM((Dm, H * Dh), BF16),
                pltpu.VMEM((H * Dh, Dm), BF16),
                pltpu.VMEM((Dm, DF), BF16), pltpu.VMEM((Dm, DF), BF16), pltpu.VMEM((DF, Dm), BF16),
                pltpu.VMEM((NS, RC * H, Dh), BF16),
                pltpu.VMEM((4 * seg, Dm), F32),
                pltpu.VMEM((2 * (M + seg), Dm), BF16),
                pltpu.VMEM((2 * seg, Dm), BF16),
                pltpu.VMEM((2 * seg, Dm), BF16),
                pltpu.VMEM((S, Dm), BF16),
                pltpu.VMEM((S, Dm), F32),
                pltpu.VMEM((S, Dm), A_x.dtype),
                pltpu.SemaphoreType.DMA((NS,)),
                pltpu.SemaphoreType.DMA((NO,)),
                pltpu.SemaphoreType.DMA((3 * (DF // FC),)),
                pltpu.SemaphoreType.DMA((2,)),
                pltpu.SemaphoreType.DMA(()),
            ],
            compiler_params=pltpu.CompilerParams(vmem_limit_bytes=110 * 1024 * 1024),
        )(A_x.reshape(S, Dm), A_mem0.reshape(M, Dm),
          A_Wq.reshape(Dm * H, Dh), A_Wk.reshape(Dm * H, Dh), A_Wv.reshape(Dm * H, Dh),
          A_Wo.reshape(H * Dh, Dm), B_w_gate, B_w_up, B_w_down)
        return out.reshape(B, S, Dm)
    return run


_run = build({})


@functools.partial(jax.jit, static_argnames=("A_seg_len",))
def pallas_interleave_layers__memory_aug_recurrent_mem_tr__glu_gated_geglu__prompt_kernel(
    A_x, A_mem0, A_Wq, A_Wk, A_Wv, A_Wo, A_seg_len, B_x, B_w_gate, B_w_up, B_w_down
):
    return _run(A_x, A_mem0, A_Wq, A_Wk, A_Wv, A_Wo, A_seg_len, B_x, B_w_gate, B_w_up, B_w_down)
```

```python
import functools
import jax
import jax.numpy as jnp
import numpy as np
import jax.experimental.pallas as pl
import jax.experimental.pallas.tpu as pltpu

F32 = jnp.float32
BF16 = jnp.bfloat16
U32 = jnp.uint32


def _ln(x):
    m = jnp.mean(x, axis=-1, keepdims=True)
    d = x - m
    v = jnp.mean(d * d, axis=-1, keepdims=True)
    return (d * jax.lax.rsqrt(v + 1e-5)).astype(BF16)


def _gelu(x):
    c = 0.7978845608028654
    return 0.5 * x * (1.0 + jnp.tanh(c * (x + 0.044715 * (x * x * x))))


def _dot(a, b):
    return jnp.dot(a, b, preferred_element_type=F32)


def build(cfg):
    G = cfg.get("G", 2)
    FC = cfg.get("FC", 512)
    RC = cfg.get("RC", 256)
    NS = cfg.get("NS", 2)
    LAG = cfg.get("lag", 2)
    NO = 8

    def kernel(x_h, mem0_ref, wq_h, wk_h, wv_h, wo_h, wg_h, wu_h, wd_h, o_h,
               wq_ref, wk_ref, wv_ref, wo_ref, wg_ref, wu_ref, wd_ref, stage_ref,
               xs_ref, hc_ref, hn_ref, hb_ref, x_ref, y_ref, out_ref,
               sem_s, sem_o, sem_f, sem_x, sem_out, *, M, seg, H, Dh, n_seg):
        Dm = xs_ref.shape[1]
        DF = wg_ref.shape[1]
        scale = Dh ** -0.5
        NG = H // G
        NF = DF // FC
        S2 = 2 * seg
        cs = lambda g: slice(g * G * Dh, (g + 1) * G * Dh)
        fs = lambda f: slice(f * FC, (f + 1) * FC)
        hsl = lambda i: slice(i * Dh, (i + 1) * Dh)

        def aligned(r, n):
            return pl.ds(r if isinstance(r, int) else pl.multiple_of(r, seg), n)

        NRC = Dm // RC
        raw = [(src, dst, r) for src, dst in ((wq_h, wq_ref), (wk_h, wk_ref), (wv_h, wv_ref)) for r in range(NRC)]
        nr = len(raw)
        OR = H * Dh // NO

        def raw_copy(i):
            src, _, r = raw[i]
            return pltpu.make_async_copy(src.at[pl.ds(r * RC * H, RC * H), :], stage_ref.at[i % NS], sem_s.at[i % NS])

        def wo_copy(i):
            return pltpu.make_async_copy(wo_h.at[pl.ds(i * OR, OR), :], wo_ref.at[pl.ds(i * OR, OR), :], sem_o.at[i])

        def ffn_copy(i):
            f, w = divmod(i, 3)
            if w == 0:
                return pltpu.make_async_copy(wg_h.at[:, fs(f)], wg_ref.at[:, fs(f)], sem_f.at[i])
            if w == 1:
                return pltpu.make_async_copy(wu_h.at[:, fs(f)], wu_ref.at[:, fs(f)], sem_f.at[i])
            return pltpu.make_async_copy(wd_h.at[fs(f), :], wd_ref.at[fs(f), :], sem_f.at[i])

        queue = [raw_copy(i) for i in range(nr)] + [wo_copy(i) for i in range(NO)] + [ffn_copy(i) for i in range(3 * NF)]
        started = [0]

        def start_upto(n):
            while started[0] < min(n, len(queue)):
                queue[started[0]].start()
                started[0] += 1

        def relayout(i):
            _, dst, r = raw[i]
            u = stage_ref.at[i % NS].bitcast(U32)
            HP = H // 2

            def body(b, carry):
                ub = u.at[pl.ds(pl.multiple_of(b * (16 * HP), 16 * HP), 16 * HP), :]
                rows = pl.ds(pl.multiple_of(r * RC + b * 16, 16), 16)

                def pair(j, carry2):
                    a = ub[pl.ds(j, 8, stride=2 * HP), :]
                    bb = ub[pl.ds(HP + j, 8, stride=2 * HP), :]
                    ev = (a & 0xFFFF) | (bb << 16)
                    od = (a >> 16) | (bb & jnp.uint32(0xFFFF0000))
                    dst[rows, hsl(2 * j)] = pltpu.bitcast(ev, BF16)
                    dst[rows, hsl(2 * j + 1)] = pltpu.bitcast(od, BF16)
                    return carry2
                for j in range(HP):
                    pair(j, 0)
                return carry
            jax.lax.fori_loop(0, RC // 16, body, 0)

        def segs(t, n=1):
            return aligned(t * seg, n * seg)

        x_first = pltpu.make_async_copy(x_h.at[0:4 * seg, :], x_ref.at[0:4 * seg, :], sem_x.at[0])
        x_rest = pltpu.make_async_copy(x_h.at[4 * seg:n_seg * seg, :], x_ref.at[4 * seg:n_seg * seg, :], sem_x.at[1])

        def out_copy(t, n):
            return pltpu.make_async_copy(out_ref.at[segs(t, n), :], o_h.at[segs(t, n), :], sem_out)

        def attention(h, lays, wait_wo=None, order=cfg.get('order', 's0 q1 k1 v1 w-2 e0 p0'), G=G):
            NG = H // G
            cs = lambda g: slice(g * G * Dh, (g + 1) * G * Dh)
            R = h.shape[0]
            ri = jax.lax.broadcasted_iota(jnp.int32, (R, 128), 0)
            ci = jax.lax.broadcasted_iota(jnp.int32, (R, 128), 1)

            def layer_pos(i):
                tok = jnp.where(i >= 2 * M + seg, lays[-1], lays[0])
                lay = jnp.where(i < 2 * M, (i >= M).astype(jnp.int32), tok)
                pos = jnp.where(i < 2 * M, i - lay * M, i - M - (i >= 2 * M + seg).astype(jnp.int32) * seg)
                return lay, pos
            rl, rp = layer_pos(ri)
            cl, cp = layer_pos(ci)
            same = (rl == cl) & (ci < R)
            keep = same & ((rp < M) | (rp >= cp))
            fill = jnp.where(same, -1e9, -jnp.inf).astype(F32)
            z = jnp.zeros((128 - R, Dh), BF16)
            proj = lambda w, g: _dot(h, w[:, cs(g)]).astype(BF16)

            def qk(q, k):
                return [jax.lax.dot_general(q[:, hsl(i)], jnp.concatenate([k[:, hsl(i)], z], axis=0),
                                            (((1,), (1,)), ((), ())), preferred_element_type=F32) for i in range(G)]

            def softmax(ss):
                ps = []
                for s in ss:
                    s = jnp.where(keep, s * scale, fill)
                    m = jnp.max(s, axis=-1, keepdims=True)
                    e = jnp.exp(s - m)
                    l = jnp.sum(e, axis=-1, keepdims=True)
                    ps.append((e * pl.reciprocal(l, approx=False)).astype(BF16))
                return ps

            def pv(ps, v):
                return jnp.concatenate(
                    [_dot(ps[i], jnp.concatenate([v[:, hsl(i)], z], axis=0)).astype(BF16) for i in range(G)], axis=1)

            acc = [None]
            os = {}

            def wo(g):
                if g < 0:
                    return
                if g == 0 and wait_wo is not None:
                    wait_wo()
                t = _dot(os.pop(g), wo_ref[cs(g), :])
                acc[0] = t if acc[0] is None else acc[0] + t

            steps = [(w[0], int(w[1:])) for w in order.split()]
            q, k, v, sc = {}, {}, {}, {}
            for g in range(-max(o for _, o in steps), NG - min(o for _, o in steps)):
                for op, off in steps:
                    i = g + off
                    if not 0 <= i < NG:
                        continue
                    if op == "q":
                        q[i] = proj(wq_ref, i)
                    elif op == "k":
                        k[i] = proj(wk_ref, i)
                    elif op == "v":
                        v[i] = proj(wv_ref, i)
                    elif op == "s":
                        sc[i] = qk(q.pop(i), k.pop(i))
                    elif op == "e":
                        sc[i] = softmax(sc[i])
                    elif op == "p":
                        os[i] = pv(sc.pop(i), v.pop(i))
                    elif op == "w":
                        wo(i)
            return acc[0]

        R1 = 2 * M + seg
        R2 = 2 * M + 2 * seg
        NC = (n_seg - 4) // 2 + 2
        last = NC - 1

        def ffn():
            def hidden(hb, f):
                return (_gelu(_dot(hb, wg_ref[:, fs(f)])) * _dot(hb, wu_ref[:, fs(f)])).astype(BF16)
            ha = hb_ref[...]
            hbb = _ln(xs_ref[S2:2 * S2, :])
            prev = jnp.concatenate([hidden(ha, 0), hidden(hbb, 0)], axis=0)
            hb = jnp.concatenate([ha, hbb], axis=0)
            acc = xs_ref[...]
            for f in range(1, NF):
                a = hidden(hb, f)
                acc = acc + _dot(prev, wd_ref[fs(f - 1), :])
                prev = a
            return acc + _dot(prev, wd_ref[fs(NF - 1), :])

        x_first.start()
        start_upto(NS)
        for i in range(nr):
            queue[i].wait()
            relayout(i)
            start_upto(i + NS + 1)
        start_upto(nr + NO)
        x_first.wait()

        def single_block(c):
            m0 = mem0_ref[...].astype(F32)

            @pl.when(c == 0)
            def _():
                hc_ref[0:2 * M, :] = jnp.concatenate([m0, m0], axis=0).astype(BF16)
                y_ref[0:4 * seg, :] = x_ref[0:4 * seg, :].astype(F32)

            @pl.when(c == last)
            def _():
                m2 = hc_ref[0:2 * M, :].astype(F32)[M:2 * M]
                hc_ref[0:2 * M, :] = jnp.concatenate([m2, m2], axis=0).astype(BF16)

            s0 = jnp.where(c == 0, 0, n_seg - 4)

            def single(j, carry):
                first = (c == 0) & (j == 0)

                def wait_wo():
                    @pl.when(first)
                    def _():
                        for i in range(nr, nr + NO):
                            queue[i].wait()
                        for i in range(nr + NO, len(queue)):
                            queue[i].start()
                x = y_ref[segs(s0 + j), :]
                h = jnp.concatenate([hc_ref[0:2 * M, :], _ln(x)], axis=0)
                acc = attention(h, (0,), wait_wo, cfg.get('sorder', 's0 q1 k1 v1 e0 p0') + ' w-%d' % (2 * H), cfg.get('sG', 2))
                hc_ref[0:2 * M, :] = acc[0:2 * M].astype(BF16)
                xs_ref[segs(j), :] = x + acc[2 * M:R1]
                return carry
            jax.lax.fori_loop(0, 4, single, 0)
            hb_ref[...] = _ln(xs_ref[0:S2, :])

            @pl.when(c == 0)
            def _():
                m1 = hc_ref[0:2 * M, :].astype(F32)[0:M]
                hc_ref[0:2 * M, :] = jnp.concatenate([m1, m0], axis=0).astype(BF16)
                for i in range(nr + NO, len(queue)):
                    queue[i].wait()
                x_rest.start()

        def a_step(c, j):
            t = 2 * (c - 1) + j
            hn_ref[0:seg, :] = _ln(x_ref[segs(jnp.minimum(t + 5, n_seg - 1)), :].astype(F32))
            hn_ref[seg:S2, :] = _ln(y_ref[segs(t + 1), :])
            hb_ref[...] = _ln(xs_ref[0:S2, :])
            done = jnp.maximum(t - 2, 0)
            out_ref[segs(done), :] = y_ref[segs(done), :].astype(out_ref.dtype)
            acc = attention(hc_ref[...], (0, 1))
            hc_ref[2 * M:R2, :] = hn_ref[...]
            hc_ref[0:2 * M, :] = acc[0:2 * M].astype(BF16)
            xs_ref[segs(2 * j), :] = x_ref[segs(t + 4), :].astype(F32) + acc[2 * M:R1]
            xs_ref[segs(2 * j + 1), :] = y_ref[segs(t), :] + acc[R1:R2]

        def step(c, carry):
            edge = (c == 0) | (c == last)

            @pl.when(edge)
            def _():
                single_block(c)

            @pl.when(jnp.logical_not(edge))
            def _():
                @pl.when(c == 1)
                def _():
                    x_rest.wait()
                    hc_ref[2 * M:R1, :] = _ln(x_ref[segs(4), :].astype(F32))
                    hc_ref[R1:R2, :] = _ln(y_ref[segs(0), :])
                jax.lax.fori_loop(0, 2, lambda j, z: (a_step(c, j), z)[1], 0)

                @pl.when(c >= 2)
                def _():
                    out_copy(2 * (c - 2), 2).start()

            r = ffn()
            t0 = 2 * (c - 1)
            s0 = jnp.where(c == 0, 0, n_seg - 4)
            for i in range(4):
                dst = jnp.where(edge, s0 + i, t0 + i // 2 + (4 if i % 2 == 0 else 0))
                y_ref[segs(dst), :] = r[i * seg:(i + 1) * seg]
            return carry
        jax.lax.fori_loop(0, NC, step, 0)

        out_ref[segs(n_seg - 6, 6), :] = y_ref[segs(n_seg - 6, 6), :].astype(out_ref.dtype)
        out_copy(n_seg - 6, 6).start()
        for c in range(NC - 3):
            out_copy(2 * c, 2).wait()
        out_copy(n_seg - 6, 6).wait()

    @functools.partial(jax.jit, static_argnames=("A_seg_len",))
    def run(A_x, A_mem0, A_Wq, A_Wk, A_Wv, A_Wo, A_seg_len, B_x, B_w_gate, B_w_up, B_w_down):
        B, S, Dm = A_x.shape
        H, Dh = A_Wq.shape[1:]
        M = A_mem0.shape[1]
        seg = A_seg_len
        DF = B_w_gate.shape[1]
        hbm = pl.BlockSpec(memory_space=pl.ANY)
        out = pl.pallas_call(
            functools.partial(kernel, M=M, seg=seg, H=H, Dh=Dh, n_seg=cfg.get("ns", S // seg)),
            in_specs=[hbm, pl.BlockSpec(memory_space=pltpu.VMEM), hbm, hbm, hbm, hbm, hbm, hbm, hbm],
            out_specs=hbm,
            out_shape=jax.ShapeDtypeStruct((S, Dm), A_x.dtype),
            scratch_shapes=[
                pltpu.VMEM((Dm, H * Dh), BF16), pltpu.VMEM((Dm, H * Dh), BF16), pltpu.VMEM((Dm, H * Dh), BF16),
                pltpu.VMEM((H * Dh, Dm), BF16),
                pltpu.VMEM((Dm, DF), BF16), pltpu.VMEM((Dm, DF), BF16), pltpu.VMEM((DF, Dm), BF16),
                pltpu.VMEM((NS, RC * H, Dh), BF16),
                pltpu.VMEM((4 * seg, Dm), F32),
                pltpu.VMEM((2 * (M + seg), Dm), BF16),
                pltpu.VMEM((2 * seg, Dm), BF16),
                pltpu.VMEM((2 * seg, Dm), BF16),
                pltpu.VMEM((S, Dm), BF16),
                pltpu.VMEM((S, Dm), F32),
                pltpu.VMEM((S, Dm), A_x.dtype),
                pltpu.SemaphoreType.DMA((NS,)),
                pltpu.SemaphoreType.DMA((NO,)),
                pltpu.SemaphoreType.DMA((3 * (DF // FC),)),
                pltpu.SemaphoreType.DMA((2,)),
                pltpu.SemaphoreType.DMA(()),
            ],
            compiler_params=pltpu.CompilerParams(vmem_limit_bytes=110 * 1024 * 1024),
        )(A_x.reshape(S, Dm), A_mem0.reshape(M, Dm),
          A_Wq.reshape(Dm * H, Dh), A_Wk.reshape(Dm * H, Dh), A_Wv.reshape(Dm * H, Dh),
          A_Wo.reshape(H * Dh, Dm), B_w_gate, B_w_up, B_w_down)
        return out.reshape(B, S, Dm)
    return run


_run = build({})


@functools.partial(jax.jit, static_argnames=("A_seg_len",))
def pallas_interleave_layers__memory_aug_recurrent_mem_tr__glu_gated_geglu__prompt_kernel(
    A_x, A_mem0, A_Wq, A_Wk, A_Wv, A_Wo, A_seg_len, B_x, B_w_gate, B_w_up, B_w_down
):
    return _run(A_x, A_mem0, A_Wq, A_Wk, A_Wv, A_Wo, A_seg_len, B_x, B_w_gate, B_w_up, B_w_down)
```

```python
import functools
import jax
import jax.numpy as jnp
import numpy as np
import jax.experimental.pallas as pl
import jax.experimental.pallas.tpu as pltpu

F32 = jnp.float32
BF16 = jnp.bfloat16
U32 = jnp.uint32


def _ln(x):
    m = jnp.mean(x, axis=-1, keepdims=True)
    d = x - m
    v = jnp.mean(d * d, axis=-1, keepdims=True)
    return (d * jax.lax.rsqrt(v + 1e-5)).astype(BF16)


def _gelu(x):
    c = 0.7978845608028654
    return 0.5 * x * (1.0 + jnp.tanh(c * (x + 0.044715 * (x * x * x))))


def _dot(a, b):
    return jnp.dot(a, b, preferred_element_type=F32)


def build(cfg):
    G = cfg.get("G", 2)
    FC = cfg.get("FC", 512)
    RC = cfg.get("RC", 256)
    NS = cfg.get("NS", 2)
    LAG = cfg.get("lag", 2)
    NO = 8
    PK = cfg.get('pk', 1)
    PD = cfg.get('pd', 0)

    def kernel(x_h, mem0_ref, wq_h, wk_h, wv_h, wo_h, wg_h, wu_h, wd_h, o_h,
               wq_ref, wk_ref, wv_ref, wo_ref, wg_ref, wu_ref, wd_ref, stage_ref,
               xs_ref, hc_ref, x_ref, y_ref, out_ref,
               sem_s, sem_o, sem_f, sem_x, sem_out, *, M, seg, H, Dh, n_seg):
        if PD:
            wo_ref, wg_ref, wu_ref, wd_ref = (r.bitcast(BF16) for r in (wo_ref, wg_ref, wu_ref, wd_ref))
        Dm = xs_ref.shape[1]
        DF = wg_ref.shape[1]
        scale = Dh ** -0.5
        NG = H // G
        NF = DF // FC
        S2 = 2 * seg
        cs = lambda g: slice(g * G * Dh, (g + 1) * G * Dh)
        fs = lambda f: slice(f * FC, (f + 1) * FC)
        hsl = lambda i: slice(i * Dh, (i + 1) * Dh)

        def h_put(r, v):
            n = v.shape[0] // 2
            hc_ref[pl.ds(r // 2 if isinstance(r, int) else pl.multiple_of(r // 2, 8), n), :] = pltpu.bitcast(v, U32)

        def h_get(r, n):
            return pltpu.bitcast(hc_ref[pl.ds(r // 2 if isinstance(r, int) else pl.multiple_of(r // 2, 8), n // 2), :], BF16)

        def aligned(r, n):
            return pl.ds(r if isinstance(r, int) else pl.multiple_of(r, seg), n)

        NRC = Dm // RC
        raw = [(src, dst, r) for src, dst in ((wq_h, wq_ref), (wk_h, wk_ref), (wv_h, wv_ref)) for r in range(NRC)]
        nr = len(raw)
        OR = H * Dh // NO

        def raw_copy(i):
            src, _, r = raw[i]
            return pltpu.make_async_copy(src.at[pl.ds(r * RC * H, RC * H), :], stage_ref.at[i % NS], sem_s.at[i % NS])

        def wo_copy(i):
            return pltpu.make_async_copy(wo_h.at[pl.ds(i * OR, OR), :], wo_ref.at[pl.ds(i * OR, OR), :], sem_o.at[i])

        def ffn_copy(i):
            f, w = divmod(i, 3)
            if w == 0:
                return pltpu.make_async_copy(wg_h.at[:, fs(f)], wg_ref.at[:, fs(f)], sem_f.at[i])
            if w == 1:
                return pltpu.make_async_copy(wu_h.at[:, fs(f)], wu_ref.at[:, fs(f)], sem_f.at[i])
            return pltpu.make_async_copy(wd_h.at[fs(f), :], wd_ref.at[fs(f), :], sem_f.at[i])

        queue = [raw_copy(i) for i in range(nr)] + [wo_copy(i) for i in range(NO)] + [ffn_copy(i) for i in range(3 * NF)]
        started = [0]

        def start_upto(n):
            while started[0] < min(n, len(queue)):
                queue[started[0]].start()
                started[0] += 1

        def relayout(i):
            _, dst, r = raw[i]
            u = stage_ref.at[i % NS].bitcast(U32)
            HP = H // 2

            def body(b, carry):
                ub = u.at[pl.ds(pl.multiple_of(b * (16 * HP), 16 * HP), 16 * HP), :]
                rows = pl.ds(pl.multiple_of((r * RC // 2) + b * 8, 8), 8) if PK else pl.ds(pl.multiple_of(r * RC + b * 16, 16), 16)

                def pair(j, carry2):
                    a = ub[pl.ds(j, 8, stride=2 * HP), :]
                    bb = ub[pl.ds(HP + j, 8, stride=2 * HP), :]
                    ev = (a & 0xFFFF) | (bb << 16)
                    od = (a >> 16) | (bb & jnp.uint32(0xFFFF0000))
                    if PK:
                        dst[rows, hsl(2 * j)] = ev
                        dst[rows, hsl(2 * j + 1)] = od
                    else:
                        dst[rows, hsl(2 * j)] = pltpu.bitcast(ev, BF16)
                        dst[rows, hsl(2 * j + 1)] = pltpu.bitcast(od, BF16)
                    return carry2
                for j in range(HP):
                    pair(j, 0)
                return carry
            jax.lax.fori_loop(0, RC // 16, body, 0)

        def segs(t, n=1):
            return aligned(t * seg, n * seg)

        x_first = pltpu.make_async_copy(x_h.at[0:4 * seg, :], x_ref.at[0:4 * seg, :], sem_x.at[0])
        x_rest = pltpu.make_async_copy(x_h.at[4 * seg:n_seg * seg, :], x_ref.at[4 * seg:n_seg * seg, :], sem_x.at[1])

        def out_copy(t, n):
            return pltpu.make_async_copy(out_ref.at[segs(t, n), :], o_h.at[segs(t, n), :], sem_out)

        def attention(load_h, R, lays, wait_wo=None, order=cfg.get('order', 's0 q1 k1 v1 w-2 e0 p0'), G=G, fill_in={}):
            NG = H // G
            cs = lambda g: slice(g * G * Dh, (g + 1) * G * Dh)
            ri = jax.lax.broadcasted_iota(jnp.int32, (R, 128), 0)
            ci = jax.lax.broadcasted_iota(jnp.int32, (R, 128), 1)

            def layer_pos(i):
                tok = jnp.where(i >= 2 * M + seg, lays[-1], lays[0])
                lay = jnp.where(i < 2 * M, (i >= M).astype(jnp.int32), tok)
                pos = jnp.where(i < 2 * M, i - lay * M, i - M - (i >= 2 * M + seg).astype(jnp.int32) * seg)
                return lay, pos
            rl, rp = layer_pos(ri)
            cl, cp = layer_pos(ci)
            same = (rl == cl) & (ci < R)
            keep = same & ((rp < M) | (rp >= cp))
            fill = jnp.where(same, -1e9, -jnp.inf).astype(F32)
            z = jnp.zeros((128 - R, Dh), BF16)
            hv = [load_h()]
            proj = lambda w, g: _dot(hv[0], pltpu.bitcast(w[:, cs(g)], BF16) if PK else w[:, cs(g)]).astype(BF16)

            def qk(q, k):
                return [jax.lax.dot_general(q[:, hsl(i)], jnp.concatenate([k[:, hsl(i)], z], axis=0),
                                            (((1,), (1,)), ((), ())), preferred_element_type=F32) for i in range(G)]

            def softmax(ss):
                ps = []
                for s in ss:
                    s = jnp.where(keep, s * scale, fill)
                    m = jnp.max(s, axis=-1, keepdims=True)
                    e = jnp.exp(s - m)
                    l = jnp.sum(e, axis=-1, keepdims=True)
                    ps.append((e * pl.reciprocal(l, approx=False)).astype(BF16))
                return ps

            def pv(ps, v):
                return jnp.concatenate(
                    [_dot(ps[i], jnp.concatenate([v[:, hsl(i)], z], axis=0)).astype(BF16) for i in range(G)], axis=1)

            acc = [None]
            os = {}

            def wo(g):
                if g < 0:
                    return
                if g == 0 and wait_wo is not None:
                    wait_wo()
                t = _dot(os.pop(g), wo_ref[cs(g), :])
                acc[0] = t if acc[0] is None else acc[0] + t

            steps = [(w[0], int(w[1:])) for w in order.split()]
            q, k, v, sc = {}, {}, {}, {}
            for g in range(-max(o for _, o in steps), NG - min(o for _, o in steps)):
                if g in fill_in:
                    fill_in[g]()
                    hv[0] = load_h()
                for op, off in steps:
                    i = g + off
                    if not 0 <= i < NG:
                        continue
                    if op == "q":
                        q[i] = proj(wq_ref, i)
                    elif op == "k":
                        k[i] = proj(wk_ref, i)
                    elif op == "v":
                        v[i] = proj(wv_ref, i)
                    elif op == "s":
                        sc[i] = qk(q.pop(i), k.pop(i))
                    elif op == "e":
                        sc[i] = softmax(sc[i])
                    elif op == "p":
                        os[i] = pv(sc.pop(i), v.pop(i))
                    elif op == "w":
                        wo(i)
            return acc[0]

        R1 = 2 * M + seg
        R2 = 2 * M + 2 * seg
        NC = (n_seg - 4) // 2 + 2
        last = NC - 1

        def ffn():
            def hidden(hb, f):
                return (_gelu(_dot(hb, wg_ref[:, fs(f)])) * _dot(hb, wu_ref[:, fs(f)])).astype(BF16)
            ha = h_get(2 * R2, S2)
            hbb = _ln(xs_ref[S2:2 * S2, :])
            prev = jnp.concatenate([hidden(ha, 0), hidden(hbb, 0)], axis=0)
            hb = jnp.concatenate([ha, hbb], axis=0)
            acc = xs_ref[...]
            for f in range(1, NF):
                a = hidden(hb, f)
                acc = acc + _dot(prev, wd_ref[fs(f - 1), :])
                prev = a
            return acc + _dot(prev, wd_ref[fs(NF - 1), :])

        x_first.start()
        start_upto(NS)
        for i in range(nr):
            queue[i].wait()
            relayout(i)
            start_upto(i + NS + 1)
        start_upto(nr + NO)
        x_first.wait()

        def single_block(c):
            m0 = mem0_ref[...].astype(F32)

            @pl.when(c == 0)
            def _():
                h_put(0, jnp.concatenate([m0, m0], axis=0).astype(BF16))
                y_ref[0:4 * seg, :] = x_ref[0:4 * seg, :].astype(F32)

            @pl.when(c == last)
            def _():
                m2 = h_get(0, 2 * M).astype(F32)[M:2 * M]
                h_put(0, jnp.concatenate([m2, m2], axis=0).astype(BF16))

            s0 = jnp.where(c == 0, 0, n_seg - 4)

            def single(j, carry):
                first = (c == 0) & (j == 0)

                def wait_wo():
                    @pl.when(first)
                    def _():
                        for i in range(nr, nr + NO):
                            queue[i].wait()
                        for i in range(nr + NO, len(queue)):
                            queue[i].start()
                x = y_ref[segs(s0 + j), :]
                h = jnp.concatenate([h_get(0, 2 * M), _ln(x)], axis=0)
                acc = attention(lambda: h, R1, (0,), wait_wo, cfg.get('sorder', 's0 q1 k1 v1 e0 p0') + ' w-%d' % (2 * H), cfg.get('sG', 2))
                h_put(0, acc[0:2 * M].astype(BF16))
                xs_ref[segs(j), :] = x + acc[2 * M:R1]
                return carry
            jax.lax.fori_loop(0, 4, single, 0)
            h_put(2 * R2, _ln(xs_ref[0:S2, :]))

            @pl.when(c == 0)
            def _():
                m1 = h_get(0, 2 * M).astype(F32)[0:M]
                h_put(0, jnp.concatenate([m1, m0], axis=0).astype(BF16))
                for i in range(nr + NO, len(queue)):
                    queue[i].wait()
                x_rest.start()

        def a_step(c, j):
            t = 2 * (c - 1) + j
            cur = j * R2
            nxt = (1 - j) * R2

            def fill_x():
                h_put(nxt + 2 * M, _ln(x_ref[segs(jnp.minimum(t + 5, n_seg - 1)), :].astype(F32)))

            def fill_y():
                h_put(nxt + R1, _ln(y_ref[segs(t + 1), :]))

            def fill_b():
                h_put(2 * R2, _ln(xs_ref[0:S2, :]))

            def fill_o():
                done = jnp.maximum(t - 2, 0)
                out_ref[segs(done), :] = y_ref[segs(done), :].astype(out_ref.dtype)
            f0, f1 = cfg.get("f0", 2), cfg.get("f1", 3)
            acc = attention(lambda: h_get(cur, R2), R2, (0, 1),
                            fill_in={f0: fill_x, f0 + f1: fill_y, f0 + 2 * f1: fill_b, f0 + 3 * f1: fill_o})
            h_put(nxt, acc[0:2 * M].astype(BF16))
            xs_ref[segs(2 * j), :] = x_ref[segs(t + 4), :].astype(F32) + acc[2 * M:R1]
            xs_ref[segs(2 * j + 1), :] = y_ref[segs(t), :] + acc[R1:R2]

        def step(c, carry):
            edge = (c == 0) | (c == last)

            @pl.when(edge)
            def _():
                single_block(c)

            @pl.when(jnp.logical_not(edge))
            def _():
                @pl.when(c == 1)
                def _():
                    x_rest.wait()
                    h_put(2 * M, _ln(x_ref[segs(4), :].astype(F32)))
                    h_put(R1, _ln(y_ref[segs(0), :]))
                if not cfg.get('skipA'):
                    jax.lax.fori_loop(0, 2, lambda j, z: (a_step(c, j), z)[1], 0)

                @pl.when(c >= 2)
                def _():
                    out_copy(2 * (c - 2), 2).start()

            r = xs_ref[...] if cfg.get('skipB') else ffn()
            t0 = 2 * (c - 1)
            s0 = jnp.where(c == 0, 0, n_seg - 4)
            for i in range(4):
                dst = jnp.where(edge, s0 + i, t0 + i // 2 + (4 if i % 2 == 0 else 0))
                y_ref[segs(dst), :] = r[i * seg:(i + 1) * seg]
            return carry
        jax.lax.fori_loop(0, NC, step, 0)

        out_ref[segs(n_seg - 6, 6), :] = y_ref[segs(n_seg - 6, 6), :].astype(out_ref.dtype)
        out_copy(n_seg - 6, 6).start()
        for c in range(NC - 3):
            out_copy(2 * c, 2).wait()
        out_copy(n_seg - 6, 6).wait()

    @functools.partial(jax.jit, static_argnames=("A_seg_len",))
    def run(A_x, A_mem0, A_Wq, A_Wk, A_Wv, A_Wo, A_seg_len, B_x, B_w_gate, B_w_up, B_w_down):
        B, S, Dm = A_x.shape
        H, Dh = A_Wq.shape[1:]
        M = A_mem0.shape[1]
        seg = A_seg_len
        DF = B_w_gate.shape[1]
        hbm = pl.BlockSpec(memory_space=pl.ANY)
        wbuf = lambda r, c, pk: pltpu.VMEM((r // 2, c), U32) if pk else pltpu.VMEM((r, c), BF16)
        out = pl.pallas_call(
            functools.partial(kernel, M=M, seg=seg, H=H, Dh=Dh, n_seg=cfg.get("ns", S // seg)),
            in_specs=[hbm, pl.BlockSpec(memory_space=pltpu.VMEM), hbm, hbm, hbm, hbm, hbm, hbm, hbm],
            out_specs=hbm,
            out_shape=jax.ShapeDtypeStruct((S, Dm), A_x.dtype),
            scratch_shapes=[
                wbuf(Dm, H * Dh, PK), wbuf(Dm, H * Dh, PK), wbuf(Dm, H * Dh, PK),
                wbuf(H * Dh, Dm, PD), wbuf(Dm, DF, PD), wbuf(Dm, DF, PD), wbuf(DF, Dm, PD),
                pltpu.VMEM((NS, RC * H, Dh), BF16),
                pltpu.VMEM((4 * seg, Dm), F32),
                wbuf(4 * (M + seg) + 2 * seg, Dm, 1),
                pltpu.VMEM((S, Dm), BF16),
                pltpu.VMEM((S, Dm), F32),
                pltpu.VMEM((S, Dm), A_x.dtype),
                pltpu.SemaphoreType.DMA((NS,)),
                pltpu.SemaphoreType.DMA((NO,)),
                pltpu.SemaphoreType.DMA((3 * (DF // FC),)),
                pltpu.SemaphoreType.DMA((2,)),
                pltpu.SemaphoreType.DMA(()),
            ],
            compiler_params=pltpu.CompilerParams(vmem_limit_bytes=110 * 1024 * 1024),
        )(A_x.reshape(S, Dm), A_mem0.reshape(M, Dm),
          A_Wq.reshape(Dm * H, Dh), A_Wk.reshape(Dm * H, Dh), A_Wv.reshape(Dm * H, Dh),
          A_Wo.reshape(H * Dh, Dm), B_w_gate, B_w_up, B_w_down)
        return out.reshape(B, S, Dm)
    return run


_run = build({})


@functools.partial(jax.jit, static_argnames=("A_seg_len",))
def pallas_interleave_layers__memory_aug_recurrent_mem_tr__glu_gated_geglu__prompt_kernel(
    A_x, A_mem0, A_Wq, A_Wk, A_Wv, A_Wo, A_seg_len, B_x, B_w_gate, B_w_up, B_w_down
):
    return _run(A_x, A_mem0, A_Wq, A_Wk, A_Wv, A_Wo, A_seg_len, B_x, B_w_gate, B_w_up, B_w_down)
```

```python
import functools
import jax
import jax.numpy as jnp
import numpy as np
import jax.experimental.pallas as pl
import jax.experimental.pallas.tpu as pltpu

F32 = jnp.float32
BF16 = jnp.bfloat16
U32 = jnp.uint32


def _ln(x):
    m = jnp.mean(x, axis=-1, keepdims=True)
    d = x - m
    v = jnp.mean(d * d, axis=-1, keepdims=True)
    return (d * jax.lax.rsqrt(v + 1e-5)).astype(BF16)


def _gelu(x):
    c = 0.7978845608028654
    return 0.5 * x * (1.0 + jnp.tanh(c * (x + 0.044715 * (x * x * x))))


def _dot(a, b):
    return jnp.dot(a, b, preferred_element_type=F32)


def build(cfg):
    G = cfg.get("G", 2)
    FC = cfg.get("FC", 256)
    RC = cfg.get("RC", 256)
    NS = cfg.get("NS", 2)
    LAG = cfg.get("lag", 2)
    NO = 8
    PK = cfg.get('pk', 1)
    PD = cfg.get('pd', 0)

    def kernel(x_h, mem0_ref, wq_h, wk_h, wv_h, wo_h, wg_h, wu_h, wd_h, o_h,
               wq_ref, wk_ref, wv_ref, wo_ref, wg_ref, wu_ref, wd_ref, eu_ref, ed_ref, stage_ref,
               xs_ref, hc_ref, x_ref, y_ref, out_ref,
               sem_s, sem_o, sem_f, sem_x, sem_out, *, M, seg, H, Dh, n_seg):
        if PD:
            wo_ref, wg_ref, wu_ref, wd_ref, eu_ref, ed_ref = (r.bitcast(BF16) for r in (wo_ref, wg_ref, wu_ref, wd_ref, eu_ref, ed_ref))
        Dm = xs_ref.shape[1]
        DF = wg_ref.shape[1]
        scale = Dh ** -0.5
        NG = H // G
        NF = DF // FC
        S2 = 2 * seg
        cs = lambda g: slice(g * G * Dh, (g + 1) * G * Dh)
        fs = lambda f: slice(f * FC, (f + 1) * FC)
        hsl = lambda i: slice(i * Dh, (i + 1) * Dh)

        def h_put(r, v):
            n = v.shape[0] // 2
            hc_ref[pl.ds(r // 2 if isinstance(r, int) else pl.multiple_of(r // 2, 8), n), :] = pltpu.bitcast(v, U32)

        def h_get(r, n):
            return pltpu.bitcast(hc_ref[pl.ds(r // 2 if isinstance(r, int) else pl.multiple_of(r // 2, 8), n // 2), :], BF16)

        def aligned(r, n):
            return pl.ds(r if isinstance(r, int) else pl.multiple_of(r, seg), n)

        NRC = Dm // RC
        raw = [(src, dst, r) for src, dst in ((wq_h, wq_ref), (wk_h, wk_ref), (wv_h, wv_ref)) for r in range(NRC)]
        nr = len(raw)
        OR = H * Dh // NO

        def raw_copy(i):
            src, _, r = raw[i]
            return pltpu.make_async_copy(src.at[pl.ds(r * RC * H, RC * H), :], stage_ref.at[i % NS], sem_s.at[i % NS])

        def wo_copy(i):
            return pltpu.make_async_copy(wo_h.at[pl.ds(i * OR, OR), :], wo_ref.at[pl.ds(i * OR, OR), :], sem_o.at[i])

        def ffn_copy(i):
            src, dst = ((wg_h, wg_ref), (wu_h, wu_ref), (wd_h, wd_ref))[i]
            return pltpu.make_async_copy(src, dst, sem_f.at[i])

        queue = [raw_copy(i) for i in range(nr)] + [wo_copy(i) for i in range(NO)] + [ffn_copy(i) for i in range(3)]
        started = [0]

        def start_upto(n):
            while started[0] < min(n, len(queue)):
                queue[started[0]].start()
                started[0] += 1

        def relayout(i):
            _, dst, r = raw[i]
            u = stage_ref.at[i % NS].bitcast(U32)
            HP = H // 2

            def body(b, carry):
                ub = u.at[pl.ds(pl.multiple_of(b * (16 * HP), 16 * HP), 16 * HP), :]
                rows = pl.ds(pl.multiple_of((r * RC // 2) + b * 8, 8), 8) if PK else pl.ds(pl.multiple_of(r * RC + b * 16, 16), 16)

                def pair(j, carry2):
                    a = ub[pl.ds(j, 8, stride=2 * HP), :]
                    bb = ub[pl.ds(HP + j, 8, stride=2 * HP), :]
                    ev = (a & 0xFFFF) | (bb << 16)
                    od = (a >> 16) | (bb & jnp.uint32(0xFFFF0000))
                    if PK:
                        dst[rows, hsl(2 * j)] = ev
                        dst[rows, hsl(2 * j + 1)] = od
                    else:
                        dst[rows, hsl(2 * j)] = pltpu.bitcast(ev, BF16)
                        dst[rows, hsl(2 * j + 1)] = pltpu.bitcast(od, BF16)
                    return carry2
                for j in range(HP):
                    pair(j, 0)
                return carry
            jax.lax.fori_loop(0, RC // 16, body, 0)

        def segs(t, n=1):
            return aligned(t * seg, n * seg)

        x_first = pltpu.make_async_copy(x_h.at[0:4 * seg, :], x_ref.at[0:4 * seg, :], sem_x.at[0])
        x_rest = pltpu.make_async_copy(x_h.at[4 * seg:n_seg * seg, :], x_ref.at[4 * seg:n_seg * seg, :], sem_x.at[1])

        def out_copy(t, n):
            return pltpu.make_async_copy(out_ref.at[segs(t, n), :], o_h.at[segs(t, n), :], sem_out)

        def attention(load_h, R, lays, wait_wo=None, order=cfg.get('order', 's0 q1 k1 v1 w-2 e0 p0'), G=G, fill_in={}):
            NG = H // G
            cs = lambda g: slice(g * G * Dh, (g + 1) * G * Dh)
            ri = jax.lax.broadcasted_iota(jnp.int32, (R, 128), 0)
            ci = jax.lax.broadcasted_iota(jnp.int32, (R, 128), 1)

            def layer_pos(i):
                tok = jnp.where(i >= 2 * M + seg, lays[-1], lays[0])
                lay = jnp.where(i < 2 * M, (i >= M).astype(jnp.int32), tok)
                pos = jnp.where(i < 2 * M, i - lay * M, i - M - (i >= 2 * M + seg).astype(jnp.int32) * seg)
                return lay, pos
            rl, rp = layer_pos(ri)
            cl, cp = layer_pos(ci)
            same = (rl == cl) & (ci < R)
            keep = same & ((rp < M) | (rp >= cp))
            fill = jnp.where(same, -1e9, -jnp.inf).astype(F32)
            z = jnp.zeros((128 - R, Dh), BF16)
            hv = [load_h()]
            proj = lambda w, g: _dot(hv[0], pltpu.bitcast(w[:, cs(g)], BF16) if PK else w[:, cs(g)]).astype(BF16)

            def qk(q, k):
                return [jax.lax.dot_general(q[:, hsl(i)], jnp.concatenate([k[:, hsl(i)], z], axis=0),
                                            (((1,), (1,)), ((), ())), preferred_element_type=F32) for i in range(G)]

            def softmax(ss):
                ps = []
                for s in ss:
                    s = jnp.where(keep, s * scale, fill)
                    m = jnp.max(s, axis=-1, keepdims=True)
                    e = jnp.exp(s - m)
                    l = jnp.sum(e, axis=-1, keepdims=True)
                    ps.append((e * pl.reciprocal(l, approx=False)).astype(BF16))
                return ps

            def pv(ps, v):
                return jnp.concatenate(
                    [_dot(ps[i], jnp.concatenate([v[:, hsl(i)], z], axis=0)).astype(BF16) for i in range(G)], axis=1)

            acc = [None]
            os = {}

            def wo(g):
                if g < 0:
                    return
                if g == 0 and wait_wo is not None:
                    wait_wo()
                t = _dot(os.pop(g), wo_ref[cs(g), :])
                acc[0] = t if acc[0] is None else acc[0] + t

            steps = [(w[0], int(w[1:])) for w in order.split()]
            q, k, v, sc = {}, {}, {}, {}
            for g in range(-max(o for _, o in steps), NG - min(o for _, o in steps)):
                if g in fill_in:
                    fill_in[g]()
                    hv[0] = load_h()
                for op, off in steps:
                    i = g + off
                    if not 0 <= i < NG:
                        continue
                    if op == "q":
                        q[i] = proj(wq_ref, i)
                    elif op == "k":
                        k[i] = proj(wk_ref, i)
                    elif op == "v":
                        v[i] = proj(wv_ref, i)
                    elif op == "s":
                        sc[i] = qk(q.pop(i), k.pop(i))
                    elif op == "e":
                        sc[i] = softmax(sc[i])
                    elif op == "p":
                        os[i] = pv(sc.pop(i), v.pop(i))
                    elif op == "w":
                        wo(i)
            return acc[0]

        R1 = 2 * M + seg
        R2 = 2 * M + 2 * seg
        NC = (n_seg - 4) // 2 + 2
        last = NC - 1

        D2 = Dm // 2
        NP = NF // 2

        def strassen_lhs(a11, a12, a21, a22):
            return [(t).astype(BF16) for t in (a11 + a22, a21 + a22, a11, a22, a11 + a12, a21 - a11, a12 - a22)]

        def strassen_out(m):
            return (m[0] + m[3] - m[4] + m[6], m[2] + m[4], m[1] + m[3], m[0] - m[1] + m[2] + m[5])

        def strassen_rhs_prepare(b11, b12, b21, b22, e0, e1, e2):
            w11, w12, w21, w22 = (r[...].astype(F32) for r in (b11, b12, b21, b22))
            e0[...] = (w11 + w22).astype(BF16)
            e1[...] = (w11 + w12).astype(BF16)
            e2[...] = (w21 + w22).astype(BF16)
            b12[...] = (w12 - w22).astype(BF16)
            b21[...] = (w21 - w11).astype(BF16)

        def prepare_ffn():
            def up(b, carry):
                r = pl.multiple_of(b * 16, 16)
                top, bot = pl.ds(r, 16), pl.ds(pl.multiple_of(D2 + r, 16), 16)
                for f in range(NF):
                    strassen_rhs_prepare(wg_ref.at[top, fs(f)], wu_ref.at[top, fs(f)], wg_ref.at[bot, fs(f)], wu_ref.at[bot, fs(f)],
                                         *(eu_ref.at[i, top, fs(f)] for i in range(3)))
                return carry
            jax.lax.fori_loop(0, D2 // 16, up, 0)

            def down(b, carry):
                p, r = b // (FC // 64), (b % (FC // 64)) * 64
                for i in range(4):
                    r0 = pl.ds(pl.multiple_of(2 * p * FC + r + 16 * i, 16), 16)
                    r1 = pl.ds(pl.multiple_of((2 * p + 1) * FC + r + 16 * i, 16), 16)
                    re = pl.ds(pl.multiple_of(p * FC + r + 16 * i, 16), 16)
                    for cl, ch in ((slice(k, k + 128), slice(D2 + k, D2 + k + 128)) for k in range(0, D2, 128)):
                        strassen_rhs_prepare(wd_ref.at[r0, cl], wd_ref.at[r0, ch], wd_ref.at[r1, cl], wd_ref.at[r1, ch],
                                             *(ed_ref.at[i2, re, cl] for i2 in range(3)))
                return carry
            jax.lax.fori_loop(0, NP * (FC // 64), down, 0)

        def ffn():
            ha = h_get(2 * R2, S2).astype(F32)
            hb = _ln(xs_ref[S2:2 * S2, :]).astype(F32)
            lhs = strassen_lhs(ha[:, 0:D2], ha[:, D2:Dm], hb[:, 0:D2], hb[:, D2:Dm])

            def hidden(f):
                rhs = (eu_ref[0, :, fs(f)], wg_ref[0:D2, fs(f)], wu_ref[0:D2, fs(f)], wg_ref[D2:Dm, fs(f)],
                       wu_ref[D2:Dm, fs(f)], eu_ref[1, :, fs(f)], eu_ref[2, :, fs(f)])
                m = [None] * 7
                for i in cfg.get("mord", (2, 3, 1, 4, 0, 5, 6)):
                    m[i] = _dot(lhs[i], rhs[i])
                ga, ua, gb, ub = strassen_out(m)
                return tuple((_gelu(g) * u).astype(BF16).astype(F32) for g, u in ((ga, ua), (gb, ub)))

            acc = [xs_ref[0:S2, 0:D2], xs_ref[0:S2, D2:Dm], xs_ref[S2:2 * S2, 0:D2], xs_ref[S2:2 * S2, D2:Dm]]

            def down(p, h0, h1):
                f0, f1 = fs(2 * p), fs(2 * p + 1)
                dl = strassen_lhs(h0[0], h1[0], h0[1], h1[1])
                rhs = (ed_ref[0, fs(p), :], wd_ref[f0, 0:D2], wd_ref[f0, D2:Dm], wd_ref[f1, 0:D2],
                       wd_ref[f1, D2:Dm], ed_ref[1, fs(p), :], ed_ref[2, fs(p), :])
                m = [None] * 7
                for i in cfg.get("dord", (2, 3, 1, 4, 0, 5, 6)):
                    m[i] = _dot(dl[i], rhs[i])
                for i, t in enumerate(strassen_out(m)):
                    acc[i] = acc[i] + t

            dlag = cfg.get("dlag", 1)
            hs = []
            for f in range(NF + dlag):
                if f < NF:
                    hs.append(hidden(f))
                e = f - dlag
                if e >= 0 and e % 2 == 1:
                    down(e // 2, hs[e - 1], hs[e])
            return [jnp.concatenate([acc[2 * i], acc[2 * i + 1]], axis=1) for i in range(2)]

        x_first.start()
        start_upto(NS)
        for i in range(nr):
            queue[i].wait()
            relayout(i)
            start_upto(i + NS + 1)
        start_upto(nr + NO)
        x_first.wait()

        def single_block(c):
            m0 = mem0_ref[...].astype(F32)

            @pl.when(c == 0)
            def _():
                h_put(0, jnp.concatenate([m0, m0], axis=0).astype(BF16))
                y_ref[0:4 * seg, :] = x_ref[0:4 * seg, :].astype(F32)

            @pl.when(c == last)
            def _():
                m2 = h_get(0, 2 * M).astype(F32)[M:2 * M]
                h_put(0, jnp.concatenate([m2, m2], axis=0).astype(BF16))

            s0 = jnp.where(c == 0, 0, n_seg - 4)

            def single(j, carry):
                first = (c == 0) & (j == 0)

                def wait_wo():
                    @pl.when(first)
                    def _():
                        for i in range(nr, nr + NO):
                            queue[i].wait()
                        for i in range(nr + NO, len(queue)):
                            queue[i].start()
                x = y_ref[segs(s0 + j), :]
                h = jnp.concatenate([h_get(0, 2 * M), _ln(x)], axis=0)
                acc = attention(lambda: h, R1, (0,), wait_wo, cfg.get('sorder', 's0 q1 k1 v1 e0 p0') + ' w-%d' % (2 * H), cfg.get('sG', 2))
                h_put(0, acc[0:2 * M].astype(BF16))
                xs_ref[segs(j), :] = x + acc[2 * M:R1]
                return carry
            jax.lax.fori_loop(0, 4, single, 0)
            h_put(2 * R2, _ln(xs_ref[0:S2, :]))

            @pl.when(c == 0)
            def _():
                m1 = h_get(0, 2 * M).astype(F32)[0:M]
                h_put(0, jnp.concatenate([m1, m0], axis=0).astype(BF16))
                for i in range(nr + NO, len(queue)):
                    queue[i].wait()
                x_rest.start()
                prepare_ffn()

        def a_step(c, j):
            t = 2 * (c - 1) + j
            cur = j * R2
            nxt = (1 - j) * R2

            def fill_x():
                h_put(nxt + 2 * M, _ln(x_ref[segs(jnp.minimum(t + 5, n_seg - 1)), :].astype(F32)))

            def fill_y():
                h_put(nxt + R1, _ln(y_ref[segs(t + 1), :]))

            def fill_b():
                h_put(2 * R2, _ln(xs_ref[0:S2, :]))

            def fill_o():
                done = jnp.maximum(t - 2, 0)
                out_ref[segs(done), :] = y_ref[segs(done), :].astype(out_ref.dtype)
            f0, f1 = cfg.get("f0", 2), cfg.get("f1", 3)
            acc = attention(lambda: h_get(cur, R2), R2, (0, 1),
                            fill_in={f0: fill_x, f0 + f1: fill_y, f0 + 2 * f1: fill_b, f0 + 3 * f1: fill_o})
            h_put(nxt, acc[0:2 * M].astype(BF16))
            xs_ref[segs(2 * j), :] = x_ref[segs(t + 4), :].astype(F32) + acc[2 * M:R1]
            xs_ref[segs(2 * j + 1), :] = y_ref[segs(t), :] + acc[R1:R2]

        def step(c, carry):
            edge = (c == 0) | (c == last)

            @pl.when(edge)
            def _():
                single_block(c)

            @pl.when(jnp.logical_not(edge))
            def _():
                @pl.when(c == 1)
                def _():
                    x_rest.wait()
                    h_put(2 * M, _ln(x_ref[segs(4), :].astype(F32)))
                    h_put(R1, _ln(y_ref[segs(0), :]))
                if not cfg.get('skipA'):
                    jax.lax.fori_loop(0, 2, lambda j, z: (a_step(c, j), z)[1], 0)

                @pl.when(c >= 2)
                def _():
                    out_copy(2 * (c - 2), 2).start()

            r = xs_ref[...] if cfg.get('skipB') else ffn()
            t0 = 2 * (c - 1)
            s0 = jnp.where(c == 0, 0, n_seg - 4)
            for i in range(4):
                dst = jnp.where(edge, s0 + i, t0 + i // 2 + (4 if i % 2 == 0 else 0))
                y_ref[segs(dst), :] = r[i // 2][(i % 2) * seg:(i % 2 + 1) * seg]
            return carry
        jax.lax.fori_loop(0, NC, step, 0)

        out_ref[segs(n_seg - 6, 6), :] = y_ref[segs(n_seg - 6, 6), :].astype(out_ref.dtype)
        out_copy(n_seg - 6, 6).start()
        for c in range(NC - 3):
            out_copy(2 * c, 2).wait()
        out_copy(n_seg - 6, 6).wait()

    @functools.partial(jax.jit, static_argnames=("A_seg_len",))
    def run(A_x, A_mem0, A_Wq, A_Wk, A_Wv, A_Wo, A_seg_len, B_x, B_w_gate, B_w_up, B_w_down):
        B, S, Dm = A_x.shape
        H, Dh = A_Wq.shape[1:]
        M = A_mem0.shape[1]
        seg = A_seg_len
        DF = B_w_gate.shape[1]
        hbm = pl.BlockSpec(memory_space=pl.ANY)
        wbuf = lambda r, c, pk: pltpu.VMEM((r // 2, c), U32) if pk else pltpu.VMEM((r, c), BF16)
        out = pl.pallas_call(
            functools.partial(kernel, M=M, seg=seg, H=H, Dh=Dh, n_seg=cfg.get("ns", S // seg)),
            in_specs=[hbm, pl.BlockSpec(memory_space=pltpu.VMEM), hbm, hbm, hbm, hbm, hbm, hbm, hbm],
            out_specs=hbm,
            out_shape=jax.ShapeDtypeStruct((S, Dm), A_x.dtype),
            scratch_shapes=[
                wbuf(Dm, H * Dh, PK), wbuf(Dm, H * Dh, PK), wbuf(Dm, H * Dh, PK),
                wbuf(H * Dh, Dm, PD), wbuf(Dm, DF, PD), wbuf(Dm, DF, PD), wbuf(DF, Dm, PD),
                pltpu.VMEM((3, Dm // 4, DF), U32) if PD else pltpu.VMEM((3, Dm // 2, DF), BF16),
                pltpu.VMEM((3, DF // 4, Dm // 2), U32) if PD else pltpu.VMEM((3, DF // 2, Dm // 2), BF16),
                pltpu.VMEM((NS, RC * H, Dh), BF16),
                pltpu.VMEM((4 * seg, Dm), F32),
                wbuf(4 * (M + seg) + 2 * seg, Dm, 1),
                pltpu.VMEM((S, Dm), BF16),
                pltpu.VMEM((S, Dm), F32),
                pltpu.VMEM((S, Dm), A_x.dtype),
                pltpu.SemaphoreType.DMA((NS,)),
                pltpu.SemaphoreType.DMA((NO,)),
                pltpu.SemaphoreType.DMA((3,)),
                pltpu.SemaphoreType.DMA((2,)),
                pltpu.SemaphoreType.DMA(()),
            ],
            compiler_params=pltpu.CompilerParams(vmem_limit_bytes=120 * 1024 * 1024),
        )(A_x.reshape(S, Dm), A_mem0.reshape(M, Dm),
          A_Wq.reshape(Dm * H, Dh), A_Wk.reshape(Dm * H, Dh), A_Wv.reshape(Dm * H, Dh),
          A_Wo.reshape(H * Dh, Dm), B_w_gate, B_w_up, B_w_down)
        return out.reshape(B, S, Dm)
    return run


_run = build({"pd": 1, "FC": 896})


@functools.partial(jax.jit, static_argnames=("A_seg_len",))
def pallas_interleave_layers__memory_aug_recurrent_mem_tr__glu_gated_geglu__prompt_kernel(
    A_x, A_mem0, A_Wq, A_Wk, A_Wv, A_Wo, A_seg_len, B_x, B_w_gate, B_w_up, B_w_down
):
    return _run(A_x, A_mem0, A_Wq, A_Wk, A_Wv, A_Wo, A_seg_len, B_x, B_w_gate, B_w_up, B_w_down)
```

```python
import functools
import jax
import jax.numpy as jnp
import numpy as np
import jax.experimental.pallas as pl
import jax.experimental.pallas.tpu as pltpu

F32 = jnp.float32
BF16 = jnp.bfloat16
U32 = jnp.uint32


def _ln(x):
    m = jnp.mean(x, axis=-1, keepdims=True)
    d = x - m
    v = jnp.mean(d * d, axis=-1, keepdims=True)
    return (d * jax.lax.rsqrt(v + 1e-5)).astype(BF16)


def _gelu(x):
    c = 0.7978845608028654
    return 0.5 * x * (1.0 + jnp.tanh(c * (x + 0.044715 * (x * x * x))))


def _dot(a, b):
    return jnp.dot(a, b, preferred_element_type=F32)


def build(cfg):
    G = cfg.get("G", 2)
    FC = cfg.get("FC", 896)
    RC = cfg.get("RC", 256)
    NS = cfg.get("NS", 2)
    LAG = cfg.get("lag", 2)
    NO = 8
    PK = cfg.get('pk', 1)
    PD = cfg.get('pd', 1)

    def kernel(x_h, mem0_ref, wq_h, wk_h, wv_h, wo_h, wg_h, wu_h, wd_h, o_h,
               wq_ref, wk_ref, wv_ref, wo_ref, wg_ref, wu_ref, wd_ref, eu_ref, ed_ref, stage_ref,
               xs_ref, hc_ref, x_ref, y_ref, out_ref,
               sem_s, sem_o, sem_f, sem_x, sem_out, *, M, seg, H, Dh, n_seg):
        wg_p, wu_p, wd_p, eu_p, ed_p = wg_ref, wu_ref, wd_ref, eu_ref, ed_ref
        if PD:
            wo_ref, wg_ref, wu_ref, wd_ref, eu_ref, ed_ref = (r.bitcast(BF16) for r in (wo_ref, wg_ref, wu_ref, wd_ref, eu_ref, ed_ref))
        Dm = xs_ref.shape[1]
        DF = wg_ref.shape[1]
        scale = Dh ** -0.5
        NG = H // G
        NF = DF // FC
        S2 = 2 * seg
        cs = lambda g: slice(g * G * Dh, (g + 1) * G * Dh)
        fs = lambda f: slice(f * FC, (f + 1) * FC)
        hsl = lambda i: slice(i * Dh, (i + 1) * Dh)

        def h_put(r, v):
            n = v.shape[0] // 2
            hc_ref[pl.ds(r // 2 if isinstance(r, int) else pl.multiple_of(r // 2, 8), n), :] = pltpu.bitcast(v, U32)

        def h_get(r, n):
            return pltpu.bitcast(hc_ref[pl.ds(r // 2 if isinstance(r, int) else pl.multiple_of(r // 2, 8), n // 2), :], BF16)

        def aligned(r, n):
            return pl.ds(r if isinstance(r, int) else pl.multiple_of(r, seg), n)

        NRC = Dm // RC
        raw = [(src, dst, r) for src, dst in ((wq_h, wq_ref), (wk_h, wk_ref), (wv_h, wv_ref)) for r in range(NRC)]
        nr = len(raw)
        OR = H * Dh // NO

        def raw_copy(i):
            src, _, r = raw[i]
            return pltpu.make_async_copy(src.at[pl.ds(r * RC * H, RC * H), :], stage_ref.at[i % NS], sem_s.at[i % NS])

        def wo_copy(i):
            return pltpu.make_async_copy(wo_h.at[pl.ds(i * OR, OR), :], wo_ref.at[pl.ds(i * OR, OR), :], sem_o.at[i])

        def ffn_copy(i):
            src, dst = ((wg_h, wg_ref), (wu_h, wu_ref), (wd_h, wd_ref))[i]
            return pltpu.make_async_copy(src, dst, sem_f.at[i])

        queue = [raw_copy(i) for i in range(nr)] + [wo_copy(i) for i in range(NO)] + [ffn_copy(i) for i in range(3)]
        started = [0]

        def start_upto(n):
            while started[0] < min(n, len(queue)):
                queue[started[0]].start()
                started[0] += 1

        def relayout(i):
            _, dst, r = raw[i]
            u = stage_ref.at[i % NS].bitcast(U32)
            HP = H // 2

            def body(b, carry):
                ub = u.at[pl.ds(pl.multiple_of(b * (16 * HP), 16 * HP), 16 * HP), :]
                rows = pl.ds(pl.multiple_of((r * RC // 2) + b * 8, 8), 8) if PK else pl.ds(pl.multiple_of(r * RC + b * 16, 16), 16)

                def pair(j, carry2):
                    a = ub[pl.ds(j, 8, stride=2 * HP), :]
                    bb = ub[pl.ds(HP + j, 8, stride=2 * HP), :]
                    ev = (a & 0xFFFF) | (bb << 16)
                    od = (a >> 16) | (bb & jnp.uint32(0xFFFF0000))
                    if PK:
                        dst[rows, hsl(2 * j)] = ev
                        dst[rows, hsl(2 * j + 1)] = od
                    else:
                        dst[rows, hsl(2 * j)] = pltpu.bitcast(ev, BF16)
                        dst[rows, hsl(2 * j + 1)] = pltpu.bitcast(od, BF16)
                    return carry2
                for j in range(HP):
                    pair(j, 0)
                return carry
            jax.lax.fori_loop(0, RC // 16, body, 0)

        def segs(t, n=1):
            return aligned(t * seg, n * seg)

        x_first = pltpu.make_async_copy(x_h.at[0:4 * seg, :], x_ref.at[0:4 * seg, :], sem_x.at[0])
        x_rest = pltpu.make_async_copy(x_h.at[4 * seg:n_seg * seg, :], x_ref.at[4 * seg:n_seg * seg, :], sem_x.at[1])

        def out_copy(t, n):
            return pltpu.make_async_copy(out_ref.at[segs(t, n), :], o_h.at[segs(t, n), :], sem_out)

        def attention(load_h, R, lays, wait_wo=None, order=cfg.get('order', 's0 q1 k1 v1 w-2 e0 p0'), G=G, fill_in={}):
            NG = H // G
            cs = lambda g: slice(g * G * Dh, (g + 1) * G * Dh)
            ri = jax.lax.broadcasted_iota(jnp.int32, (R, 128), 0)
            ci = jax.lax.broadcasted_iota(jnp.int32, (R, 128), 1)

            def layer_pos(i):
                tok = jnp.where(i >= 2 * M + seg, lays[-1], lays[0])
                lay = jnp.where(i < 2 * M, (i >= M).astype(jnp.int32), tok)
                pos = jnp.where(i < 2 * M, i - lay * M, i - M - (i >= 2 * M + seg).astype(jnp.int32) * seg)
                return lay, pos
            rl, rp = layer_pos(ri)
            cl, cp = layer_pos(ci)
            same = (rl == cl) & (ci < R)
            keep = same & ((rp < M) | (rp >= cp))
            fill = jnp.where(same, -1e9, -jnp.inf).astype(F32)
            z = jnp.zeros((128 - R, Dh), BF16)
            hv = [load_h()]
            proj = lambda w, g: _dot(hv[0], pltpu.bitcast(w[:, cs(g)], BF16) if PK else w[:, cs(g)]).astype(BF16)

            def qk(q, k):
                return [jax.lax.dot_general(q[:, hsl(i)], jnp.concatenate([k[:, hsl(i)], z], axis=0),
                                            (((1,), (1,)), ((), ())), preferred_element_type=F32) for i in range(G)]

            def softmax(ss):
                ps = []
                for s in ss:
                    s = jnp.where(keep, s * scale, fill)
                    m = jnp.max(s, axis=-1, keepdims=True)
                    e = jnp.exp(s - m)
                    l = jnp.sum(e, axis=-1, keepdims=True)
                    ps.append((e * pl.reciprocal(l, approx=False)).astype(BF16))
                return ps

            def pv(ps, v):
                return jnp.concatenate(
                    [_dot(ps[i], jnp.concatenate([v[:, hsl(i)], z], axis=0)).astype(BF16) for i in range(G)], axis=1)

            acc = [None]
            os = {}

            def wo(g):
                if g < 0:
                    return
                if g == 0 and wait_wo is not None:
                    wait_wo()
                t = _dot(os.pop(g), wo_ref[cs(g), :])
                acc[0] = t if acc[0] is None else acc[0] + t

            steps = [(w[0], int(w[1:])) for w in order.split()]
            q, k, v, sc = {}, {}, {}, {}
            for g in range(-max(o for _, o in steps), NG - min(o for _, o in steps)):
                if g in fill_in:
                    fill_in[g]()
                    hv[0] = load_h()
                for op, off in steps:
                    i = g + off
                    if not 0 <= i < NG:
                        continue
                    if op == "q":
                        q[i] = proj(wq_ref, i)
                    elif op == "k":
                        k[i] = proj(wk_ref, i)
                    elif op == "v":
                        v[i] = proj(wv_ref, i)
                    elif op == "s":
                        sc[i] = qk(q.pop(i), k.pop(i))
                    elif op == "e":
                        sc[i] = softmax(sc[i])
                    elif op == "p":
                        os[i] = pv(sc.pop(i), v.pop(i))
                    elif op == "w":
                        wo(i)
            return acc[0]

        R1 = 2 * M + seg
        R2 = 2 * M + 2 * seg
        NC = (n_seg - 4) // 2 + 2
        last = NC - 1

        D2 = Dm // 2
        NP = NF // 2

        def strassen_lhs(a11, a12, a21, a22):
            return [(t).astype(BF16) for t in (a11 + a22, a21 + a22, a11, a22, a11 + a12, a21 - a11, a12 - a22)]

        def strassen_out(m):
            return (m[0] + m[3] - m[4] + m[6], m[2] + m[4], m[1] + m[3], m[0] - m[1] + m[2] + m[5])

        def strassen_rhs_prepare(b11, b12, b21, b22, e0, e1, e2):
            w = [r[...] for r in (b11, b12, b21, b22)]
            res = []
            for half in range(2):
                w11, w12, w21, w22 = (pltpu.unpack_elementwise(t, index=half, packed_dtype=BF16, unpacked_dtype=F32) for t in w)
                res.append((w11 + w22, w11 + w12, w21 + w22, w12 - w22, w21 - w11))
            for dst, lo, hi in zip((e0, e1, e2, b12, b21), *res):
                dst[...] = pltpu.pack_elementwise((lo, hi), packed_dtype=BF16).astype(U32)

        def prepare_ffn():
            def up(b, carry):
                r = pl.multiple_of(b * 8, 8)
                top, bot = pl.ds(r, 8), pl.ds(pl.multiple_of(D2 // 2 + r, 8), 8)
                for k in range(0, DF, 512):
                    c = slice(k, k + 512)
                    strassen_rhs_prepare(wg_p.at[top, c], wu_p.at[top, c], wg_p.at[bot, c], wu_p.at[bot, c],
                                         *(eu_p.at[i, top, c] for i in range(3)))
                return carry
            jax.lax.fori_loop(0, D2 // 16, up, 0)
            F2 = FC // 2
            nb = F2 // 56

            def down(b, carry):
                p, r = b // nb, (b % nb) * 56
                for i in range(7):
                    r0 = pl.ds(pl.multiple_of(2 * p * F2 + r + 8 * i, 8), 8)
                    r1 = pl.ds(pl.multiple_of((2 * p + 1) * F2 + r + 8 * i, 8), 8)
                    re = pl.ds(pl.multiple_of(p * F2 + r + 8 * i, 8), 8)
                    strassen_rhs_prepare(wd_p.at[r0, 0:D2], wd_p.at[r0, D2:Dm], wd_p.at[r1, 0:D2], wd_p.at[r1, D2:Dm],
                                         *(ed_p.at[i2, re, :] for i2 in range(3)))
                return carry
            jax.lax.fori_loop(0, NP * nb, down, 0)

        def ffn():
            ha = h_get(2 * R2, S2).astype(F32)
            hb = _ln(xs_ref[S2:2 * S2, :]).astype(F32)
            lhs = strassen_lhs(ha[:, 0:D2], ha[:, D2:Dm], hb[:, 0:D2], hb[:, D2:Dm])

            def hidden(f):
                rhs = (eu_ref[0, :, fs(f)], wg_ref[0:D2, fs(f)], wu_ref[0:D2, fs(f)], wg_ref[D2:Dm, fs(f)],
                       wu_ref[D2:Dm, fs(f)], eu_ref[1, :, fs(f)], eu_ref[2, :, fs(f)])
                m = [None] * 7
                for i in cfg.get("mord", (2, 3, 1, 4, 0, 5, 6)):
                    m[i] = _dot(lhs[i], rhs[i])
                ga, ua, gb, ub = strassen_out(m)
                return tuple((_gelu(g) * u).astype(BF16).astype(F32) for g, u in ((ga, ua), (gb, ub)))

            acc = [xs_ref[0:S2, 0:D2], xs_ref[0:S2, D2:Dm], xs_ref[S2:2 * S2, 0:D2], xs_ref[S2:2 * S2, D2:Dm]]

            def down(p, h0, h1):
                f0, f1 = fs(2 * p), fs(2 * p + 1)
                dl = strassen_lhs(h0[0], h1[0], h0[1], h1[1])
                rhs = (ed_ref[0, fs(p), :], wd_ref[f0, 0:D2], wd_ref[f0, D2:Dm], wd_ref[f1, 0:D2],
                       wd_ref[f1, D2:Dm], ed_ref[1, fs(p), :], ed_ref[2, fs(p), :])
                m = [None] * 7
                for i in cfg.get("dord", (0, 1, 3, 4, 6, 2, 5)):
                    m[i] = _dot(dl[i], rhs[i])
                for i, t in enumerate(strassen_out(m)):
                    acc[i] = acc[i] + t

            dlag = cfg.get("dlag", 1)
            hs = []
            for f in range(NF + dlag):
                if f < NF:
                    hs.append(hidden(f))
                e = f - dlag
                if e >= 0 and e % 2 == 1:
                    down(e // 2, hs[e - 1], hs[e])
            return [jnp.concatenate([acc[2 * i], acc[2 * i + 1]], axis=1) for i in range(2)]

        x_first.start()
        start_upto(NS)
        for i in range(nr):
            queue[i].wait()
            relayout(i)
            start_upto(i + NS + 1)
        start_upto(nr + NO)
        x_first.wait()

        def single_block(c):
            m0 = mem0_ref[...].astype(F32)

            @pl.when(c == 0)
            def _():
                h_put(0, jnp.concatenate([m0, m0], axis=0).astype(BF16))
                y_ref[0:4 * seg, :] = x_ref[0:4 * seg, :].astype(F32)

            @pl.when(c == last)
            def _():
                m2 = h_get(0, 2 * M).astype(F32)[M:2 * M]
                h_put(0, jnp.concatenate([m2, m2], axis=0).astype(BF16))

            s0 = jnp.where(c == 0, 0, n_seg - 4)

            def single(j, carry):
                first = (c == 0) & (j == 0)

                def wait_wo():
                    @pl.when(first)
                    def _():
                        for i in range(nr, nr + NO):
                            queue[i].wait()
                        for i in range(nr + NO, len(queue)):
                            queue[i].start()
                x = y_ref[segs(s0 + j), :]
                h = jnp.concatenate([h_get(0, 2 * M), _ln(x)], axis=0)
                acc = attention(lambda: h, R1, (0,), wait_wo, cfg.get('sorder', 's0 q1 k1 v1 e0 p0') + ' w-%d' % (2 * H), cfg.get('sG', 2))
                h_put(0, acc[0:2 * M].astype(BF16))
                xs_ref[segs(j), :] = x + acc[2 * M:R1]
                return carry
            jax.lax.fori_loop(0, 4, single, 0)
            h_put(2 * R2, _ln(xs_ref[0:S2, :]))

            @pl.when(c == 0)
            def _():
                m1 = h_get(0, 2 * M).astype(F32)[0:M]
                h_put(0, jnp.concatenate([m1, m0], axis=0).astype(BF16))
                for i in range(nr + NO, len(queue)):
                    queue[i].wait()
                x_rest.start()
                prepare_ffn()

        def a_step(c, j):
            t = 2 * (c - 1) + j
            cur = j * R2
            nxt = (1 - j) * R2

            def fill_x():
                h_put(nxt + 2 * M, _ln(x_ref[segs(jnp.minimum(t + 5, n_seg - 1)), :].astype(F32)))

            def fill_y():
                h_put(nxt + R1, _ln(y_ref[segs(t + 1), :]))

            def fill_b():
                h_put(2 * R2, _ln(xs_ref[0:S2, :]))

            def fill_o():
                done = jnp.maximum(t - 2, 0)
                out_ref[segs(done), :] = y_ref[segs(done), :].astype(out_ref.dtype)
            f0, f1 = cfg.get("f0", 2), cfg.get("f1", 3)
            acc = attention(lambda: h_get(cur, R2), R2, (0, 1),
                            fill_in={f0: fill_x, f0 + f1: fill_y, f0 + 2 * f1: fill_b, f0 + 3 * f1: fill_o})
            h_put(nxt, acc[0:2 * M].astype(BF16))
            xs_ref[segs(2 * j), :] = x_ref[segs(t + 4), :].astype(F32) + acc[2 * M:R1]
            xs_ref[segs(2 * j + 1), :] = y_ref[segs(t), :] + acc[R1:R2]

        def step(c, carry):
            edge = (c == 0) | (c == last)

            @pl.when(edge)
            def _():
                single_block(c)

            @pl.when(jnp.logical_not(edge))
            def _():
                @pl.when(c == 1)
                def _():
                    x_rest.wait()
                    h_put(2 * M, _ln(x_ref[segs(4), :].astype(F32)))
                    h_put(R1, _ln(y_ref[segs(0), :]))
                if not cfg.get('skipA'):
                    jax.lax.fori_loop(0, 2, lambda j, z: (a_step(c, j), z)[1], 0)

                @pl.when(c >= 2)
                def _():
                    out_copy(2 * (c - 2), 2).start()

            r = xs_ref[...] if cfg.get('skipB') else ffn()
            t0 = 2 * (c - 1)
            s0 = jnp.where(c == 0, 0, n_seg - 4)
            for i in range(4):
                dst = jnp.where(edge, s0 + i, t0 + i // 2 + (4 if i % 2 == 0 else 0))
                y_ref[segs(dst), :] = r[i // 2][(i % 2) * seg:(i % 2 + 1) * seg]
            return carry
        jax.lax.fori_loop(0, NC, step, 0)

        out_ref[segs(n_seg - 6, 6), :] = y_ref[segs(n_seg - 6, 6), :].astype(out_ref.dtype)
        out_copy(n_seg - 6, 6).start()
        for c in range(NC - 3):
            out_copy(2 * c, 2).wait()
        out_copy(n_seg - 6, 6).wait()

    @functools.partial(jax.jit, static_argnames=("A_seg_len",))
    def run(A_x, A_mem0, A_Wq, A_Wk, A_Wv, A_Wo, A_seg_len, B_x, B_w_gate, B_w_up, B_w_down):
        B, S, Dm = A_x.shape
        H, Dh = A_Wq.shape[1:]
        M = A_mem0.shape[1]
        seg = A_seg_len
        DF = B_w_gate.shape[1]
        hbm = pl.BlockSpec(memory_space=pl.ANY)
        wbuf = lambda r, c, pk: pltpu.VMEM((r // 2, c), U32) if pk else pltpu.VMEM((r, c), BF16)
        out = pl.pallas_call(
            functools.partial(kernel, M=M, seg=seg, H=H, Dh=Dh, n_seg=cfg.get("ns", S // seg)),
            in_specs=[hbm, pl.BlockSpec(memory_space=pltpu.VMEM), hbm, hbm, hbm, hbm, hbm, hbm, hbm],
            out_specs=hbm,
            out_shape=jax.ShapeDtypeStruct((S, Dm), A_x.dtype),
            scratch_shapes=[
                wbuf(Dm, H * Dh, PK), wbuf(Dm, H * Dh, PK), wbuf(Dm, H * Dh, PK),
                wbuf(H * Dh, Dm, PD), wbuf(Dm, DF, PD), wbuf(Dm, DF, PD), wbuf(DF, Dm, PD),
                pltpu.VMEM((3, Dm // 4, DF), U32) if PD else pltpu.VMEM((3, Dm // 2, DF), BF16),
                pltpu.VMEM((3, DF // 4, Dm // 2), U32) if PD else pltpu.VMEM((3, DF // 2, Dm // 2), BF16),
                pltpu.VMEM((NS, RC * H, Dh), BF16),
                pltpu.VMEM((4 * seg, Dm), F32),
                wbuf(4 * (M + seg) + 2 * seg, Dm, 1),
                pltpu.VMEM((S, Dm), BF16),
                pltpu.VMEM((S, Dm), F32),
                pltpu.VMEM((S, Dm), A_x.dtype),
                pltpu.SemaphoreType.DMA((NS,)),
                pltpu.SemaphoreType.DMA((NO,)),
                pltpu.SemaphoreType.DMA((3,)),
                pltpu.SemaphoreType.DMA((2,)),
                pltpu.SemaphoreType.DMA(()),
            ],
            compiler_params=pltpu.CompilerParams(vmem_limit_bytes=120 * 1024 * 1024),
        )(A_x.reshape(S, Dm), A_mem0.reshape(M, Dm),
          A_Wq.reshape(Dm * H, Dh), A_Wk.reshape(Dm * H, Dh), A_Wv.reshape(Dm * H, Dh),
          A_Wo.reshape(H * Dh, Dm), B_w_gate, B_w_up, B_w_down)
        return out.reshape(B, S, Dm)
    return run


_run = build({})


@functools.partial(jax.jit, static_argnames=("A_seg_len",))
def pallas_interleave_layers__memory_aug_recurrent_mem_tr__glu_gated_geglu__prompt_kernel(
    A_x, A_mem0, A_Wq, A_Wk, A_Wv, A_Wo, A_seg_len, B_x, B_w_gate, B_w_up, B_w_down
):
    return _run(A_x, A_mem0, A_Wq, A_Wk, A_Wv, A_Wo, A_seg_len, B_x, B_w_gate, B_w_up, B_w_down)
```

```python
import functools
import jax
import jax.numpy as jnp
import numpy as np
import jax.experimental.pallas as pl
import jax.experimental.pallas.tpu as pltpu

F32 = jnp.float32
BF16 = jnp.bfloat16
U32 = jnp.uint32


def _ln(x):
    m = jnp.mean(x, axis=-1, keepdims=True)
    d = x - m
    v = jnp.mean(d * d, axis=-1, keepdims=True)
    return d * jax.lax.rsqrt(v + 1e-5)


def _gelu(x):
    c = 0.7978845608028654
    return 0.5 * x * (1.0 + jnp.tanh(c * (x + 0.044715 * (x * x * x))))


def _dot(a, b):
    return jnp.dot(a, b, preferred_element_type=F32)


def build(cfg):
    G = cfg.get("G", 2)
    FC = cfg.get("FC", 896)
    RC = cfg.get("RC", 64)
    NS = cfg.get("NS", 3)
    LAG = cfg.get("lag", 2)
    NO = 8

    def kernel(x_h, mem0_ref, wq_h, wk_h, wv_h, wo_h, wg_h, wu_h, wd_h, o_h,
               wq_p, wk_p, wv_p, wo_p, wg_p, wu_p, wd_p, eo_p, eu_p, ed_p, stage_ref,
               xs_ref, hc_ref, x_ref, y_ref,
               sem_s, sem_o, sem_f, sem_x, sem_out, *, M, seg, H, Dh, n_seg):
        wo_ref, wg_ref, wu_ref, wd_ref, eo_ref, eu_ref, ed_ref = (
            r.bitcast(BF16) for r in (wo_p, wg_p, wu_p, wd_p, eo_p, eu_p, ed_p))
        out_ref = x_ref
        Dm = xs_ref.shape[1]
        DF = wg_ref.shape[1]
        scale = Dh ** -0.5
        NG = H // G
        NF = DF // FC
        S2 = 2 * seg
        cs = lambda g: slice(g * G * Dh, (g + 1) * G * Dh)
        fs = lambda f: slice(f * FC, (f + 1) * FC)
        hsl = lambda i: slice(i * Dh, (i + 1) * Dh)

        def h_rows(r, n):
            return pl.ds(r if isinstance(r, int) else pl.multiple_of(r, M), n)

        def aligned(r, n):
            return pl.ds(r if isinstance(r, int) else pl.multiple_of(r, seg), n)

        D2 = Dm // 2
        NRC = D2 // RC
        raw = [(src, dst, r) for src, dst in ((wq_h, wq_p), (wk_h, wk_p), (wv_h, wv_p)) for r in range(NRC)]
        nr = len(raw)
        OR = H * Dh // NO

        class Both:
            def __init__(self, i):
                src, _, r = raw[i]
                self.parts = [pltpu.make_async_copy(src.at[pl.ds((half * D2 + r * RC) * H, RC * H), :],
                                                    stage_ref.at[i % NS, half], sem_s.at[i % NS, half]) for half in range(2)]

            def start(self):
                for p in self.parts:
                    p.start()

            def wait(self):
                for p in self.parts:
                    p.wait()

        def wo_copy(i):
            return pltpu.make_async_copy(wo_h.at[pl.ds(i * OR, OR), :], wo_ref.at[pl.ds(i * OR, OR), :], sem_o.at[i])

        def ffn_copy(i):
            src, dst = ((wg_h, wg_ref), (wu_h, wu_ref), (wd_h, wd_ref))[i]
            return pltpu.make_async_copy(src, dst, sem_f.at[i])

        queue = [Both(i) for i in range(nr)] + [wo_copy(i) for i in range(NO)] + [ffn_copy(i) for i in range(3)]
        started = [0]

        def start_upto(n):
            while started[0] < min(n, len(queue)):
                queue[started[0]].start()
                started[0] += 1

        def unpack(t):
            return [pltpu.unpack_elementwise(t, index=i, packed_dtype=BF16, unpacked_dtype=F32) for i in range(2)]

        def pack(lo, hi):
            return pltpu.pack_elementwise((lo, hi), packed_dtype=BF16).astype(U32)

        def strassen_rhs(b11, b12, b21, b22):
            return (b11 + b22, b11, b12 - b22, b21 - b11, b22, b11 + b12, b21 + b22)

        def relayout(i):
            _, dst, r = raw[i]
            u = [stage_ref.at[i % NS, half].bitcast(U32) for half in range(2)]
            HP = H // 2

            def body(b, carry):
                ub = [t.at[pl.ds(pl.multiple_of(b * (16 * HP), 16 * HP), 16 * HP), :] for t in u]
                rows = pl.ds(pl.multiple_of((r * RC // 2) + b * 8, 8), 8)
                for j in range(HP):
                    res = []
                    for par in range(2):
                        top, bot = (unpack(t[pl.ds(par * HP + j, 8, stride=2 * HP), :]) for t in ub)
                        res.append(strassen_rhs(top[0], top[1], bot[0], bot[1]))
                    for n in range(7):
                        dst[n, rows, hsl(j)] = pack(res[0][n], res[1][n])
                return carry
            jax.lax.fori_loop(0, RC // 16, body, 0)

        def segs(t, n=1):
            return aligned(t * seg, n * seg)

        x_first = pltpu.make_async_copy(x_h.at[0:4 * seg, :], x_ref.at[0:4 * seg, :], sem_x.at[0])
        x_rest = pltpu.make_async_copy(x_h.at[4 * seg:n_seg * seg, :], x_ref.at[4 * seg:n_seg * seg, :], sem_x.at[1])

        def out_copy(t, n):
            return pltpu.make_async_copy(out_ref.at[segs(t, n), :], o_h.at[segs(t, n), :], sem_out)

        def strassen_lhs(a11, a12, a21, a22):
            return (a11 + a22, a21 + a22, a11, a22, a11 + a12, a21 - a11, a12 - a22)

        def strassen_out(m):
            return (m[0] + m[3] - m[4] + m[6], m[2] + m[4], m[1] + m[3], m[0] - m[1] + m[2] + m[5])

        def product(lhs, rhs):
            m = [None] * 7
            if len(lhs) == 7:
                for n in cfg.get("aord", (2, 3, 1, 4, 0, 5, 6)):
                    m[n] = _dot(lhs[n], rhs(n))
                return strassen_out(m)
            a11, a12 = lhs
            both = a11 + a12
            right = _dot(a11, rhs(2))
            left = _dot(a12, rhs(3))
            return left + _dot(both, rhs(1)), right + _dot(both, rhs(4))

        def operands(hs, lo, hi):
            quads = [t for h in hs for t in (h[:, lo], h[:, hi])]
            return strassen_lhs(*quads) if len(hs) == 2 else quads

        L = M + seg

        def attention(hs, order, G, wait_wo=None, fill_in={}):
            nl = len(hs)
            R = nl * L
            NG = H // G
            ri = jax.lax.broadcasted_iota(jnp.int32, (R, 128), 0)
            ci = jax.lax.broadcasted_iota(jnp.int32, (R, 128), 1)
            rl, cl = (ri >= L).astype(jnp.int32), (ci >= L).astype(jnp.int32)
            rp, cp = ri - rl * L, ci - cl * L
            same = (rl == cl) & (ci < R)
            keep = same & ((rp < M) | (rp >= cp))
            fill = jnp.where(same, -1e9, -jnp.inf).astype(F32)
            z = jnp.zeros((128 - R, Dh), F32)
            lhs = operands(hs, slice(0, D2), slice(D2, Dm))

            def proj(w, g):
                c = product(lhs, lambda n: pltpu.bitcast(w[n, :, g * (G // 2) * Dh:(g + 1) * (G // 2) * Dh], BF16))
                return [jnp.concatenate([c[2 * l + i % 2][:, hsl(i // 2)] for l in range(nl)], axis=0) for i in range(G)]

            def as_rhs(t):
                return jnp.concatenate([t, z], axis=0).astype(BF16)

            def softmax(s):
                s = jnp.where(keep, s * scale, fill)
                e = jnp.exp(s - jnp.max(s, axis=-1, keepdims=True))
                return e * pl.reciprocal(jnp.sum(e, axis=-1, keepdims=True), approx=False)

            acc = []
            os = {}

            def wo(g):
                if g == 0 and wait_wo is not None:
                    wait_wo()
                o = os.pop(g)
                ol = operands([jnp.concatenate([t[l * L:(l + 1) * L] for t in o[0::2] + o[1::2]], axis=1) for l in range(nl)],
                              slice(0, G // 2 * Dh), slice(G // 2 * Dh, G * Dh))
                pairs = range(g * G // 2, (g + 1) * G // 2)

                def rhs(n):
                    if n in (0, 5, 6):
                        return eo_ref[{0: 0, 5: 1, 6: 2}[n], pairs[0] * Dh:(pairs[-1] + 1) * Dh, :]
                    odd, cols = {1: (0, slice(0, D2)), 2: (0, slice(D2, Dm)), 3: (1, slice(0, D2)), 4: (1, slice(D2, Dm))}[n]
                    parts = [wo_ref[(2 * p + odd) * Dh:(2 * p + odd + 1) * Dh, cols] for p in pairs]
                    return parts[0] if len(parts) == 1 else jnp.concatenate(parts, axis=0)
                c = product(ol, rhs)
                acc[:] = list(c) if not acc else [x + y for x, y in zip(acc, c)]

            steps = [(w[0], int(w[1:])) for w in order.split()]
            q, k, v, sc = {}, {}, {}, {}
            for g in range(-max(o for _, o in steps), NG - min(o for _, o in steps)):
                if g in fill_in:
                    fill_in[g]()
                for op, off in steps:
                    i = g + off
                    if not 0 <= i < NG:
                        continue
                    if op == "q":
                        q[i] = proj(wq_p, i)
                    elif op == "k":
                        k[i] = [as_rhs(t) for t in proj(wk_p, i)]
                    elif op == "v":
                        v[i] = [as_rhs(t) for t in proj(wv_p, i)]
                    elif op == "s":
                        sc[i] = [jax.lax.dot_general(a, b, (((1,), (1,)), ((), ())), preferred_element_type=F32)
                                 for a, b in zip(q.pop(i), k.pop(i))]
                    elif op == "e":
                        sc[i] = [softmax(t) for t in sc[i]]
                    elif op == "p":
                        os[i] = [_dot(a, b) for a, b in zip(sc.pop(i), v.pop(i))]
                    elif op == "w":
                        wo(i)
            return [jnp.concatenate(acc[2 * l:2 * l + 2], axis=1) for l in range(nl)]

        R2 = 2 * L
        NC = (n_seg - 4) // 2 + 2
        last = NC - 1

        NP = NF // 2

        def strassen_rhs_prepare(b11, b12, b21, b22, e0, e1, e2):
            res = [strassen_rhs(*t) for t in zip(*(unpack(r[...]) for r in (b11, b12, b21, b22)))]
            for dst, n in ((e0, 0), (e1, 5), (e2, 6), (b12, 2), (b21, 3)):
                dst[...] = pack(res[0][n], res[1][n])

        def prepare_wo(i):
            ppc = OR // (2 * Dh)

            def body(b, carry):
                p, r = i * ppc + b // 4, (b % 4) * 16
                for n in range(2):
                    r0, r1, re = (pl.ds(pl.multiple_of(row * (Dh // 2) + r + 8 * n, 8), 8) for row in (2 * p, 2 * p + 1, p))
                    strassen_rhs_prepare(wo_p.at[r0, 0:D2], wo_p.at[r0, D2:Dm], wo_p.at[r1, 0:D2], wo_p.at[r1, D2:Dm],
                                         *(eo_p.at[n2, re, :] for n2 in range(3)))
                return carry
            jax.lax.fori_loop(0, ppc * 4, body, 0)

        def prepare_ffn():
            def up(b, carry):
                r = pl.multiple_of(b * 8, 8)
                top, bot = pl.ds(r, 8), pl.ds(pl.multiple_of(D2 // 2 + r, 8), 8)
                for k in range(0, DF, 512):
                    c = slice(k, k + 512)
                    strassen_rhs_prepare(wg_p.at[top, c], wu_p.at[top, c], wg_p.at[bot, c], wu_p.at[bot, c],
                                         *(eu_p.at[i, top, c] for i in range(3)))
                return carry
            jax.lax.fori_loop(0, D2 // 16, up, 0)
            F2 = FC // 2
            nb = F2 // 56

            def down(b, carry):
                p, r = b // nb, (b % nb) * 56
                for i in range(7):
                    r0 = pl.ds(pl.multiple_of(2 * p * F2 + r + 8 * i, 8), 8)
                    r1 = pl.ds(pl.multiple_of((2 * p + 1) * F2 + r + 8 * i, 8), 8)
                    re = pl.ds(pl.multiple_of(p * F2 + r + 8 * i, 8), 8)
                    strassen_rhs_prepare(wd_p.at[r0, 0:D2], wd_p.at[r0, D2:Dm], wd_p.at[r1, 0:D2], wd_p.at[r1, D2:Dm],
                                         *(ed_p.at[i2, re, :] for i2 in range(3)))
                return carry
            jax.lax.fori_loop(0, NP * nb, down, 0)

        def ffn():
            ha = hc_ref[2 * R2:2 * R2 + S2, :]
            hb = _ln(xs_ref[S2:2 * S2, :])
            lhs = [t.astype(BF16) for t in operands((ha, hb), slice(0, D2), slice(D2, Dm))]

            def hidden(f):
                rhs = (eu_ref[0, :, fs(f)], wg_ref[0:D2, fs(f)], wu_ref[0:D2, fs(f)], wg_ref[D2:Dm, fs(f)],
                       wu_ref[D2:Dm, fs(f)], eu_ref[1, :, fs(f)], eu_ref[2, :, fs(f)])
                m = [None] * 7
                for i in cfg.get("mord", (2, 3, 1, 4, 0, 5, 6)):
                    m[i] = _dot(lhs[i], rhs[i])
                ga, ua, gb, ub = strassen_out(m)
                return _gelu(ga) * ua, _gelu(gb) * ub

            acc = [xs_ref[0:S2, 0:D2], xs_ref[0:S2, D2:Dm], xs_ref[S2:2 * S2, 0:D2], xs_ref[S2:2 * S2, D2:Dm]]

            def down(p, h0, h1):
                f0, f1 = fs(2 * p), fs(2 * p + 1)
                dl = [t.astype(BF16) for t in strassen_lhs(h0[0], h1[0], h0[1], h1[1])]
                rhs = (ed_ref[0, fs(p), :], wd_ref[f0, 0:D2], wd_ref[f0, D2:Dm], wd_ref[f1, 0:D2],
                       wd_ref[f1, D2:Dm], ed_ref[1, fs(p), :], ed_ref[2, fs(p), :])
                m = [None] * 7
                for i in cfg.get("dord", (0, 1, 3, 4, 6, 2, 5)):
                    m[i] = _dot(dl[i], rhs[i])
                for i, t in enumerate(strassen_out(m)):
                    acc[i] = acc[i] + t

            dlag = cfg.get("dlag", 1)
            hs = []
            for f in range(NF + dlag):
                if f < NF:
                    hs.append(hidden(f))
                e = f - dlag
                if e >= 0 and e % 2 == 1:
                    down(e // 2, hs[e - 1], hs[e])
            return [jnp.concatenate([acc[2 * i], acc[2 * i + 1]], axis=1) for i in range(2)]

        x_first.start()
        start_upto(NS)
        for i in range(nr):
            queue[i].wait()
            relayout(i)
            start_upto(i + NS + 1)
        start_upto(nr + NO)
        x_first.wait()

        def single_block(c):
            @pl.when(c == 0)
            def _():
                hc_ref[0:M, :] = mem0_ref[...].astype(F32)
                y_ref[0:4 * seg, :] = x_ref[0:4 * seg, :].astype(F32)

            @pl.when(c == last)
            def _():
                hc_ref[0:M, :] = hc_ref[L:L + M, :]

            s0 = jnp.where(c == 0, 0, n_seg - 4)

            def single(j, carry):
                def wait_wo():
                    @pl.when((c == 0) & (j == 0))
                    def _():
                        for i in range(NO):
                            queue[nr + i].wait()
                            if i == 0:
                                for n in range(nr + NO, len(queue)):
                                    queue[n].start()
                            prepare_wo(i)
                x = y_ref[segs(s0 + j), :]
                h = jnp.concatenate([hc_ref[0:M, :], _ln(x)], axis=0)
                acc, = attention([h], cfg.get('sorder', 's0 q1 k1 v1 e0 p0') + ' w-%d' % (2 * H), cfg.get('sG', 2), wait_wo)
                hc_ref[0:M, :] = acc[0:M]
                xs_ref[segs(j), :] = x + acc[M:L]
                return carry
            jax.lax.fori_loop(0, 4, single, 0)
            hc_ref[2 * R2:2 * R2 + S2, :] = _ln(xs_ref[0:S2, :])

            @pl.when(c == 0)
            def _():
                hc_ref[L:L + M, :] = mem0_ref[...].astype(F32)
                for i in range(nr + NO, len(queue)):
                    queue[i].wait()
                x_rest.start()
                prepare_ffn()

        def a_step(c, j):
            t = 2 * (c - 1) + j
            cur = j * R2
            nxt = (1 - j) * R2

            def fill_x():
                hc_ref[h_rows(nxt + M, seg), :] = _ln(x_ref[segs(jnp.minimum(t + 5, n_seg - 1)), :].astype(F32))

            def fill_y():
                hc_ref[h_rows(nxt + L + M, seg), :] = _ln(y_ref[segs(t + 1), :])

            def fill_b():
                hc_ref[2 * R2:2 * R2 + S2, :] = _ln(xs_ref[0:S2, :])

            def fill_o():
                done = jnp.maximum(t - 2, 0)
                out_ref[segs(done), :] = y_ref[segs(done), :].astype(out_ref.dtype)
            f0, f1 = cfg.get("f0", 2), cfg.get("f1", 3)
            x1, x2 = x_ref[segs(t + 4), :].astype(F32), y_ref[segs(t), :]
            acc = attention([hc_ref[h_rows(cur + l * L, L), :] for l in range(2)],
                            cfg.get('order', 's0 q1 k1 v1 w-2 e0 p0'), G,
                            fill_in={f0: fill_x, f0 + f1: fill_y, f0 + 2 * f1: fill_b, f0 + 3 * f1: fill_o})
            for l, res in enumerate((x1, x2)):
                hc_ref[h_rows(nxt + l * L, M), :] = acc[l][0:M]
                xs_ref[segs(2 * j + l), :] = res + acc[l][M:L]

        def step(c, carry):
            edge = (c == 0) | (c == last)

            @pl.when(edge)
            def _():
                single_block(c)

            @pl.when(jnp.logical_not(edge))
            def _():
                @pl.when(c == 1)
                def _():
                    x_rest.wait()
                    hc_ref[M:L, :] = _ln(x_ref[segs(4), :].astype(F32))
                    hc_ref[L + M:R2, :] = _ln(y_ref[segs(0), :])
                if not cfg.get('skipA'):
                    jax.lax.fori_loop(0, 2, lambda j, z: (a_step(c, j), z)[1], 0)

                @pl.when(c >= 2)
                def _():
                    out_copy(2 * (c - 2), 2).start()

            r = xs_ref[...] if cfg.get('skipB') else ffn()
            t0 = 2 * (c - 1)
            s0 = jnp.where(c == 0, 0, n_seg - 4)
            for i in range(4):
                dst = jnp.where(edge, s0 + i, t0 + i // 2 + (4 if i % 2 == 0 else 0))
                y_ref[segs(dst), :] = r[i // 2][(i % 2) * seg:(i % 2 + 1) * seg]
            return carry
        jax.lax.fori_loop(0, NC, step, 0)

        out_ref[segs(n_seg - 6, 6), :] = y_ref[segs(n_seg - 6, 6), :].astype(out_ref.dtype)
        out_copy(n_seg - 6, 6).start()
        for c in range(NC - 3):
            out_copy(2 * c, 2).wait()
        out_copy(n_seg - 6, 6).wait()

    @functools.partial(jax.jit, static_argnames=("A_seg_len",))
    def run(A_x, A_mem0, A_Wq, A_Wk, A_Wv, A_Wo, A_seg_len, B_x, B_w_gate, B_w_up, B_w_down):
        B, S, Dm = A_x.shape
        H, Dh = A_Wq.shape[1:]
        M = A_mem0.shape[1]
        seg = A_seg_len
        DF = B_w_gate.shape[1]
        hbm = pl.BlockSpec(memory_space=pl.ANY)
        packed = lambda r, c: pltpu.VMEM((r // 2, c), U32)
        proj = pltpu.VMEM((7, Dm // 4, H * Dh // 2), U32)
        out = pl.pallas_call(
            functools.partial(kernel, M=M, seg=seg, H=H, Dh=Dh, n_seg=cfg.get("ns", S // seg)),
            in_specs=[hbm, pl.BlockSpec(memory_space=pltpu.VMEM), hbm, hbm, hbm, hbm, hbm, hbm, hbm],
            out_specs=hbm,
            out_shape=jax.ShapeDtypeStruct((S, Dm), A_x.dtype),
            scratch_shapes=[
                proj, proj, proj,
                packed(H * Dh, Dm), packed(Dm, DF), packed(Dm, DF), packed(DF, Dm),
                pltpu.VMEM((3, H * Dh // 4, Dm // 2), U32),
                pltpu.VMEM((3, Dm // 4, DF), U32),
                pltpu.VMEM((3, DF // 4, Dm // 2), U32),
                pltpu.VMEM((NS, 2, RC * H, Dh), BF16),
                pltpu.VMEM((4 * seg, Dm), F32),
                pltpu.VMEM((4 * (M + seg) + 2 * seg, Dm), F32),
                pltpu.VMEM((S, Dm), BF16),
                pltpu.VMEM((S, Dm), F32),
                pltpu.SemaphoreType.DMA((NS, 2)),
                pltpu.SemaphoreType.DMA((NO,)),
                pltpu.SemaphoreType.DMA((3,)),
                pltpu.SemaphoreType.DMA((2,)),
                pltpu.SemaphoreType.DMA(()),
            ],
            compiler_params=pltpu.CompilerParams(vmem_limit_bytes=126 * 1024 * 1024),
        )(A_x.reshape(S, Dm), A_mem0.reshape(M, Dm),
          A_Wq.reshape(Dm * H, Dh), A_Wk.reshape(Dm * H, Dh), A_Wv.reshape(Dm * H, Dh),
          A_Wo.reshape(H * Dh, Dm), B_w_gate, B_w_up, B_w_down)
        return out.reshape(B, S, Dm)
    return run


_run = build({})


@functools.partial(jax.jit, static_argnames=("A_seg_len",))
def pallas_interleave_layers__memory_aug_recurrent_mem_tr__glu_gated_geglu__prompt_kernel(
    A_x, A_mem0, A_Wq, A_Wk, A_Wv, A_Wo, A_seg_len, B_x, B_w_gate, B_w_up, B_w_down
):
    return _run(A_x, A_mem0, A_Wq, A_Wk, A_Wv, A_Wo, A_seg_len, B_x, B_w_gate, B_w_up, B_w_down)
```

```python
import functools
import jax
import jax.numpy as jnp
import numpy as np
import jax.experimental.pallas as pl
import jax.experimental.pallas.tpu as pltpu

F32 = jnp.float32
BF16 = jnp.bfloat16
U32 = jnp.uint32


def _ln(x):
    m = jnp.mean(x, axis=-1, keepdims=True)
    d = x - m
    v = jnp.mean(d * d, axis=-1, keepdims=True)
    return d * jax.lax.rsqrt(v + 1e-5)


def _gelu(x):
    c = 0.7978845608028654
    return 0.5 * x * (1.0 + jnp.tanh(c * (x + 0.044715 * (x * x * x))))


def _dot(a, b):
    return jnp.dot(a, b, preferred_element_type=F32)


def build(cfg):
    G = cfg.get("G", 2)
    FC = cfg.get("FC", 896)
    RC = cfg.get("RC", 64)
    NS = cfg.get("NS", 3)
    LAG = cfg.get("lag", 2)
    NO = 8

    def kernel(x_h, mem0_ref, wq_h, wk_h, wv_h, wo_h, wg_h, wu_h, wd_h, o_h,
               wq_p, wk_p, wv_p, wo_p, wg_p, wu_p, wd_p, eo_p, eu_p, ed_p, stage_ref,
               xs_ref, hc_ref, x_ref, y_ref,
               sem_s, sem_o, sem_f, sem_x, sem_out, *, M, seg, H, Dh, n_seg):
        wo_ref, wg_ref, wu_ref, wd_ref, eo_ref, eu_ref, ed_ref = (
            r.bitcast(BF16) for r in (wo_p, wg_p, wu_p, wd_p, eo_p, eu_p, ed_p))
        out_ref = x_ref
        Dm = xs_ref.shape[1]
        DF = wg_ref.shape[1]
        scale = Dh ** -0.5
        NG = H // G
        NF = DF // FC
        S2 = 2 * seg
        cs = lambda g: slice(g * G * Dh, (g + 1) * G * Dh)
        fs = lambda f: slice(f * FC, (f + 1) * FC)
        hsl = lambda i: slice(i * Dh, (i + 1) * Dh)

        def h_rows(r, n):
            return pl.ds(r if isinstance(r, int) else pl.multiple_of(r, M), n)

        def aligned(r, n):
            return pl.ds(r if isinstance(r, int) else pl.multiple_of(r, seg), n)

        D2 = Dm // 2
        NRC = D2 // RC
        raw = [(src, dst, r) for src, dst in ((wq_h, wq_p), (wk_h, wk_p), (wv_h, wv_p)) for r in range(NRC)]
        nr = len(raw)
        OR = H * Dh // NO

        class Both:
            def __init__(self, i):
                src, _, r = raw[i]
                self.parts = [pltpu.make_async_copy(src.at[pl.ds((half * D2 + r * RC) * H, RC * H), :],
                                                    stage_ref.at[i % NS, half], sem_s.at[i % NS, half]) for half in range(2)]

            def start(self):
                for p in self.parts:
                    p.start()

            def wait(self):
                for p in self.parts:
                    p.wait()

        def wo_copy(i):
            return pltpu.make_async_copy(wo_h.at[pl.ds(i * OR, OR), :], wo_ref.at[pl.ds(i * OR, OR), :], sem_o.at[i])

        def ffn_copy(i):
            src, dst = ((wg_h, wg_ref), (wu_h, wu_ref), (wd_h, wd_ref))[i]
            return pltpu.make_async_copy(src, dst, sem_f.at[i])

        queue = [Both(i) for i in range(nr)] + [wo_copy(i) for i in range(NO)] + [ffn_copy(i) for i in range(3)]
        gate, up, down_copy = queue[nr + NO:]
        started = [0]

        def start_upto(n):
            while started[0] < min(n, len(queue)):
                queue[started[0]].start()
                started[0] += 1

        def unpack(t):
            return [pltpu.unpack_elementwise(t, index=i, packed_dtype=BF16, unpacked_dtype=F32) for i in range(2)]

        def pack(lo, hi):
            return pltpu.pack_elementwise((lo, hi), packed_dtype=BF16).astype(U32)

        def strassen_rhs(b11, b12, b21, b22):
            return (b11 + b22, b11, b12 - b22, b21 - b11, b22, b11 + b12, b21 + b22)

        def relayout(i):
            _, dst, r = raw[i]
            u = [stage_ref.at[i % NS, half].bitcast(U32) for half in range(2)]
            HP = H // 2

            def body(b, carry):
                ub = [t.at[pl.ds(pl.multiple_of(b * (16 * HP), 16 * HP), 16 * HP), :] for t in u]
                rows = pl.ds(pl.multiple_of((r * RC // 2) + b * 8, 8), 8)
                for j in range(HP):
                    res = []
                    for par in range(2):
                        top, bot = (unpack(t[pl.ds(par * HP + j, 8, stride=2 * HP), :]) for t in ub)
                        res.append(strassen_rhs(top[0], top[1], bot[0], bot[1]))
                    for n in range(7):
                        dst[n, rows, hsl(j)] = pack(res[0][n], res[1][n])
                return carry
            jax.lax.fori_loop(0, RC // 16, body, 0)

        def segs(t, n=1):
            return aligned(t * seg, n * seg)

        x_first = pltpu.make_async_copy(x_h.at[0:4 * seg, :], x_ref.at[0:4 * seg, :], sem_x.at[0])
        x_rest = pltpu.make_async_copy(x_h.at[4 * seg:n_seg * seg, :], x_ref.at[4 * seg:n_seg * seg, :], sem_x.at[1])

        def out_copy(t, n):
            return pltpu.make_async_copy(out_ref.at[segs(t, n), :], o_h.at[segs(t, n), :], sem_out)

        def strassen_lhs(a11, a12, a21, a22):
            return (a11 + a22, a21 + a22, a11, a22, a11 + a12, a21 - a11, a12 - a22)

        def strassen_out(m):
            return ((m[3] - m[4]) + m[0] + m[6], m[2] + m[4], m[1] + m[3], (m[2] - m[1]) + m[0] + m[5])

        def product(lhs, rhs):
            m = [None] * 7
            if len(lhs) == 7:
                for n in cfg.get("aord", (2, 3, 1, 4, 0, 5, 6)):
                    m[n] = _dot(lhs[n], rhs(n))
                return strassen_out(m)
            a11, a12 = lhs
            both = a11 + a12
            right = _dot(a11, rhs(2))
            left = _dot(a12, rhs(3))
            return left + _dot(both, rhs(1)), right + _dot(both, rhs(4))

        def operands(hs, lo, hi):
            quads = [t for h in hs for t in (h[:, lo], h[:, hi])]
            return strassen_lhs(*quads) if len(hs) == 2 else quads

        L = M + seg

        def attention(hs, order, G, WG, wait_wo=None, fill_in={}):
            nl = len(hs)
            R = nl * L
            NG = H // G
            ri = jax.lax.broadcasted_iota(jnp.int32, (R, 128), 0)
            ci = jax.lax.broadcasted_iota(jnp.int32, (R, 128), 1)
            rl, cl = (ri >= L).astype(jnp.int32), (ci >= L).astype(jnp.int32)
            rp, cp = ri - rl * L, ci - cl * L
            same = (rl == cl) & (ci < R)
            keep = same & ((rp < M) | (rp >= cp))
            fill = jnp.where(same, -1e9, -jnp.inf).astype(F32)
            z = jnp.zeros((128 - R, Dh), F32)
            lhs = operands(hs, slice(0, D2), slice(D2, Dm))

            def proj(w, g):
                c = product(lhs, lambda n: pltpu.bitcast(w[n, :, g * (G // 2) * Dh:(g + 1) * (G // 2) * Dh], BF16))
                return [jnp.concatenate([c[2 * l + i % 2][:, hsl(i // 2)] for l in range(nl)], axis=0) for i in range(G)]

            def as_rhs(t):
                return jnp.concatenate([t, z], axis=0).astype(BF16)

            def softmax(s):
                s = jnp.where(keep, s * scale, fill)
                e = jnp.exp(s - jnp.max(s, axis=-1, keepdims=True))
                return e * pl.reciprocal(jnp.sum(e, axis=-1, keepdims=True), approx=False)

            acc = []
            os = {}

            def wo(g):
                if g == 0 and wait_wo is not None:
                    wait_wo()
                if (g + 1) % WG and not (cfg.get("split", 1) and g == NG - 2):
                    return
                o = [t for i in sorted(os) if i <= g for t in os.pop(i)]
                n2 = len(o) // 2
                ol = operands([jnp.concatenate([t[l * L:(l + 1) * L] for t in o[0::2] + o[1::2]], axis=1) for l in range(nl)],
                              slice(0, n2 * Dh), slice(n2 * Dh, 2 * n2 * Dh))
                pairs = range((g + 1) * G // 2 - n2, (g + 1) * G // 2)

                def rhs(n):
                    if n in (0, 5, 6):
                        return eo_ref[{0: 0, 5: 1, 6: 2}[n], pairs[0] * Dh:(pairs[-1] + 1) * Dh, :]
                    odd, cols = {1: (0, slice(0, D2)), 2: (0, slice(D2, Dm)), 3: (1, slice(0, D2)), 4: (1, slice(D2, Dm))}[n]
                    parts = [wo_ref[(2 * p + odd) * Dh:(2 * p + odd + 1) * Dh, cols] for p in pairs]
                    return parts[0] if len(parts) == 1 else jnp.concatenate(parts, axis=0)
                if nl == 2 and cfg.get("wacc", 1):
                    c = [_dot(ol[n], rhs(n)) for n in range(7)]
                else:
                    c = product(ol, rhs)
                acc[:] = list(c) if not acc else [x + y for x, y in zip(acc, c)]

            steps = [(w[0], int(w[1:])) for w in order.split()]
            q, k, v, sc = {}, {}, {}, {}
            for g in range(-max(o for _, o in steps), NG - min(o for _, o in steps)):
                if g in fill_in:
                    fill_in[g]()
                for op, off in steps:
                    i = g + off
                    if not 0 <= i < NG:
                        continue
                    if op == "q":
                        q[i] = proj(wq_p, i)
                    elif op == "k":
                        k[i] = [as_rhs(t) for t in proj(wk_p, i)]
                    elif op == "v":
                        v[i] = [as_rhs(t) for t in proj(wv_p, i)]
                    elif op == "s":
                        sc[i] = [jax.lax.dot_general(a, b, (((1,), (1,)), ((), ())), preferred_element_type=F32)
                                 for a, b in zip(q.pop(i), k.pop(i))]
                    elif op == "e":
                        sc[i] = [softmax(t) for t in sc[i]]
                    elif op == "p":
                        os[i] = [_dot(a, b) for a, b in zip(sc.pop(i), v.pop(i))]
                    elif op == "w":
                        wo(i)
            if len(acc) == 7:
                acc = strassen_out(acc)
            return [jnp.concatenate(acc[2 * l:2 * l + 2], axis=1) for l in range(nl)]

        R2 = 2 * L
        NC = (n_seg - 4) // 2 + 2
        last = NC - 1

        NP = NF // 2

        def strassen_rhs_prepare(b11, b12, b21, b22, e0, e1, e2):
            res = [strassen_rhs(*t) for t in zip(*(unpack(r[...]) for r in (b11, b12, b21, b22)))]
            for dst, n in ((e0, 0), (e1, 5), (e2, 6), (b12, 2), (b21, 3)):
                dst[...] = pack(res[0][n], res[1][n])

        def prepare_wo(i):
            ppc = OR // (2 * Dh)

            def body(b, carry):
                p, r = i * ppc + b // 4, (b % 4) * 16
                for n in range(2):
                    r0, r1, re = (pl.ds(pl.multiple_of(row * (Dh // 2) + r + 8 * n, 8), 8) for row in (2 * p, 2 * p + 1, p))
                    strassen_rhs_prepare(wo_p.at[r0, 0:D2], wo_p.at[r0, D2:Dm], wo_p.at[r1, 0:D2], wo_p.at[r1, D2:Dm],
                                         *(eo_p.at[n2, re, :] for n2 in range(3)))
                return carry
            jax.lax.fori_loop(0, ppc * 4, body, 0)

        def prepare_up():
            def body(b, carry):
                r = pl.multiple_of(b * 8, 8)
                top, bot = pl.ds(r, 8), pl.ds(pl.multiple_of(D2 // 2 + r, 8), 8)
                for k in range(0, DF, 512):
                    c = slice(k, k + 512)
                    strassen_rhs_prepare(wg_p.at[top, c], wu_p.at[top, c], wg_p.at[bot, c], wu_p.at[bot, c],
                                         *(eu_p.at[i, top, c] for i in range(3)))
                return carry
            jax.lax.fori_loop(0, D2 // 16, body, 0)

        def prepare_down():
            F2 = FC // 2
            nb = F2 // 56

            def body(b, carry):
                p, r = b // nb, (b % nb) * 56
                for i in range(7):
                    r0 = pl.ds(pl.multiple_of(2 * p * F2 + r + 8 * i, 8), 8)
                    r1 = pl.ds(pl.multiple_of((2 * p + 1) * F2 + r + 8 * i, 8), 8)
                    re = pl.ds(pl.multiple_of(p * F2 + r + 8 * i, 8), 8)
                    strassen_rhs_prepare(wd_p.at[r0, 0:D2], wd_p.at[r0, D2:Dm], wd_p.at[r1, 0:D2], wd_p.at[r1, D2:Dm],
                                         *(ed_p.at[i2, re, :] for i2 in range(3)))
                return carry
            jax.lax.fori_loop(0, NP * nb, body, 0)

        def ffn():
            ha = hc_ref[2 * R2:2 * R2 + S2, :]
            hb = _ln(xs_ref[S2:2 * S2, :])
            lhs = [t.astype(BF16) for t in operands((ha, hb), slice(0, D2), slice(D2, Dm))]

            def hidden(f):
                rhs = (eu_ref[0, :, fs(f)], wg_ref[0:D2, fs(f)], wu_ref[0:D2, fs(f)], wg_ref[D2:Dm, fs(f)],
                       wu_ref[D2:Dm, fs(f)], eu_ref[1, :, fs(f)], eu_ref[2, :, fs(f)])
                m = [None] * 7
                for i in cfg.get("mord", (2, 3, 1, 4, 0, 5, 6)):
                    m[i] = _dot(lhs[i], rhs[i])
                ga, ua, gb, ub = strassen_out(m)
                return _gelu(ga) * ua, _gelu(gb) * ub

            acc = [xs_ref[0:S2, 0:D2], xs_ref[0:S2, D2:Dm], xs_ref[S2:2 * S2, 0:D2], xs_ref[S2:2 * S2, D2:Dm]]

            def down(p, h0, h1):
                f0, f1 = fs(2 * p), fs(2 * p + 1)
                dl = [t.astype(BF16) for t in strassen_lhs(h0[0], h1[0], h0[1], h1[1])]
                rhs = (ed_ref[0, fs(p), :], wd_ref[f0, 0:D2], wd_ref[f0, D2:Dm], wd_ref[f1, 0:D2],
                       wd_ref[f1, D2:Dm], ed_ref[1, fs(p), :], ed_ref[2, fs(p), :])
                m = [None] * 7
                for i in cfg.get("dord", (0, 1, 3, 4, 6, 2, 5)):
                    m[i] = _dot(dl[i], rhs[i])
                for i, t in enumerate(strassen_out(m)):
                    acc[i] = acc[i] + t

            dlag = cfg.get("dlag", 1)
            hs = []
            for f in range(NF + dlag):
                if f < NF:
                    hs.append(hidden(f))
                e = f - dlag
                if e >= 0 and e % 2 == 1:
                    down(e // 2, hs[e - 1], hs[e])
            return [jnp.concatenate([acc[2 * i], acc[2 * i + 1]], axis=1) for i in range(2)]

        x_first.start()
        start_upto(NS)
        for i in range(nr):
            queue[i].wait()
            relayout(i)
            start_upto(i + NS + 1)
        start_upto(nr + NO)
        x_first.wait()

        def single_block(c):
            @pl.when(c == 0)
            def _():
                hc_ref[0:M, :] = mem0_ref[...].astype(F32)
                y_ref[0:4 * seg, :] = x_ref[0:4 * seg, :].astype(F32)

            @pl.when(c == last)
            def _():
                hc_ref[0:M, :] = hc_ref[L:L + M, :]

            s0 = jnp.where(c == 0, 0, n_seg - 4)

            def single(j, carry):
                def wait_wo():
                    @pl.when(c == 0)
                    def _():
                        @pl.when(j == 0)
                        def _():
                            for i in range(NO):
                                queue[nr + i].wait()
                                if i == 0:
                                    gate.start()
                                    up.start()
                                prepare_wo(i)

                        @pl.when(j == 2)
                        def _():
                            down_copy.start()
                x = y_ref[segs(s0 + j), :]
                h = jnp.concatenate([hc_ref[0:M, :], _ln(x)], axis=0)
                acc, = attention([h], cfg.get('sorder', 's0 q1 k1 v1 e0 p0') + ' w-%d' % (2 * H), cfg.get('sG', 2), cfg.get('sWG', 2), wait_wo)
                hc_ref[0:M, :] = acc[0:M]
                xs_ref[segs(j), :] = x + acc[M:L]
                return carry
            jax.lax.fori_loop(0, 4, single, 0)
            hc_ref[2 * R2:2 * R2 + S2, :] = _ln(xs_ref[0:S2, :])

            @pl.when(c == 0)
            def _():
                hc_ref[L:L + M, :] = mem0_ref[...].astype(F32)
                gate.wait()
                up.wait()
                prepare_up()
                down_copy.wait()
                x_rest.start()
                prepare_down()

        def a_step(c, j):
            t = 2 * (c - 1) + j
            cur = j * R2
            nxt = (1 - j) * R2

            def fill_x():
                hc_ref[h_rows(nxt + M, seg), :] = _ln(x_ref[segs(jnp.minimum(t + 5, n_seg - 1)), :].astype(F32))

            def fill_y():
                hc_ref[h_rows(nxt + L + M, seg), :] = _ln(y_ref[segs(t + 1), :])

            def fill_b():
                hc_ref[2 * R2:2 * R2 + S2, :] = _ln(xs_ref[0:S2, :])

            def fill_o():
                done = jnp.maximum(t - 2, 0)
                out_ref[segs(done), :] = y_ref[segs(done), :].astype(out_ref.dtype)
            f0, f1 = cfg.get("f0", 2), cfg.get("f1", 3)
            x1, x2 = x_ref[segs(t + 4), :].astype(F32), y_ref[segs(t), :]
            acc = attention([hc_ref[h_rows(cur + l * L, L), :] for l in range(2)],
                            cfg.get('order', 's0 q1 k1 v1 w-2 e0 p0'), G, cfg.get('WG', 2),
                            fill_in={f0: fill_x, f0 + f1: fill_y, f0 + 2 * f1: fill_b, f0 + 3 * f1: fill_o})
            for l, res in enumerate((x1, x2)):
                hc_ref[h_rows(nxt + l * L, M), :] = acc[l][0:M]
                xs_ref[segs(2 * j + l), :] = res + acc[l][M:L]

        def step(c, carry):
            edge = (c == 0) | (c == last)

            @pl.when(edge)
            def _():
                single_block(c)

            @pl.when(jnp.logical_not(edge))
            def _():
                @pl.when(c == 1)
                def _():
                    x_rest.wait()
                    hc_ref[M:L, :] = _ln(x_ref[segs(4), :].astype(F32))
                    hc_ref[L + M:R2, :] = _ln(y_ref[segs(0), :])
                if not cfg.get('skipA'):
                    jax.lax.fori_loop(0, 2, lambda j, z: (a_step(c, j), z)[1], 0)

                @pl.when(c >= 2)
                def _():
                    out_copy(2 * (c - 2), 2).start()

            r = xs_ref[...] if cfg.get('skipB') else ffn()
            t0 = 2 * (c - 1)
            s0 = jnp.where(c == 0, 0, n_seg - 4)
            for i in range(4):
                dst = jnp.where(edge, s0 + i, t0 + i // 2 + (4 if i % 2 == 0 else 0))
                y_ref[segs(dst), :] = r[i // 2][(i % 2) * seg:(i % 2 + 1) * seg]
            return carry
        jax.lax.fori_loop(0, NC, step, 0)

        out_ref[segs(n_seg - 6, 6), :] = y_ref[segs(n_seg - 6, 6), :].astype(out_ref.dtype)
        out_copy(n_seg - 6, 6).start()
        for c in range(NC - 3):
            out_copy(2 * c, 2).wait()
        out_copy(n_seg - 6, 6).wait()

    @functools.partial(jax.jit, static_argnames=("A_seg_len",))
    def run(A_x, A_mem0, A_Wq, A_Wk, A_Wv, A_Wo, A_seg_len, B_x, B_w_gate, B_w_up, B_w_down):
        B, S, Dm = A_x.shape
        H, Dh = A_Wq.shape[1:]
        M = A_mem0.shape[1]
        seg = A_seg_len
        DF = B_w_gate.shape[1]
        hbm = pl.BlockSpec(memory_space=pl.ANY)
        packed = lambda r, c: pltpu.VMEM((r // 2, c), U32)
        proj = pltpu.VMEM((7, Dm // 4, H * Dh // 2), U32)
        out = pl.pallas_call(
            functools.partial(kernel, M=M, seg=seg, H=H, Dh=Dh, n_seg=cfg.get("ns", S // seg)),
            in_specs=[hbm, pl.BlockSpec(memory_space=pltpu.VMEM), hbm, hbm, hbm, hbm, hbm, hbm, hbm],
            out_specs=hbm,
            out_shape=jax.ShapeDtypeStruct((S, Dm), A_x.dtype),
            scratch_shapes=[
                proj, proj, proj,
                packed(H * Dh, Dm), packed(Dm, DF), packed(Dm, DF), packed(DF, Dm),
                pltpu.VMEM((3, H * Dh // 4, Dm // 2), U32),
                pltpu.VMEM((3, Dm // 4, DF), U32),
                pltpu.VMEM((3, DF // 4, Dm // 2), U32),
                pltpu.VMEM((NS, 2, RC * H, Dh), BF16),
                pltpu.VMEM((4 * seg, Dm), F32),
                pltpu.VMEM((4 * (M + seg) + 2 * seg, Dm), F32),
                pltpu.VMEM((S, Dm), BF16),
                pltpu.VMEM((S, Dm), F32),
                pltpu.SemaphoreType.DMA((NS, 2)),
                pltpu.SemaphoreType.DMA((NO,)),
                pltpu.SemaphoreType.DMA((3,)),
                pltpu.SemaphoreType.DMA((2,)),
                pltpu.SemaphoreType.DMA(()),
            ],
            compiler_params=pltpu.CompilerParams(vmem_limit_bytes=126 * 1024 * 1024),
        )(A_x.reshape(S, Dm), A_mem0.reshape(M, Dm),
          A_Wq.reshape(Dm * H, Dh), A_Wk.reshape(Dm * H, Dh), A_Wv.reshape(Dm * H, Dh),
          A_Wo.reshape(H * Dh, Dm), B_w_gate, B_w_up, B_w_down)
        return out.reshape(B, S, Dm)
    return run


_run = build({})


@functools.partial(jax.jit, static_argnames=("A_seg_len",))
def pallas_interleave_layers__memory_aug_recurrent_mem_tr__glu_gated_geglu__prompt_kernel(
    A_x, A_mem0, A_Wq, A_Wk, A_Wv, A_Wo, A_seg_len, B_x, B_w_gate, B_w_up, B_w_down
):
    return _run(A_x, A_mem0, A_Wq, A_Wk, A_Wv, A_Wo, A_seg_len, B_x, B_w_gate, B_w_up, B_w_down)
```

```python
import functools
import jax
import jax.numpy as jnp
import numpy as np
import jax.experimental.pallas as pl
import jax.experimental.pallas.tpu as pltpu

F32 = jnp.float32
BF16 = jnp.bfloat16
U32 = jnp.uint32


def _ln(x):
    m = jnp.mean(x, axis=-1, keepdims=True)
    d = x - m
    v = jnp.mean(d * d, axis=-1, keepdims=True)
    return d * jax.lax.rsqrt(v + 1e-5)


def _gelu(x):
    c = 0.7978845608028654
    return 0.5 * x * (1.0 + jnp.tanh(c * (x + 0.044715 * (x * x * x))))


def _dot(a, b):
    return jnp.dot(a, b, preferred_element_type=F32)


def build(cfg):
    G = cfg.get("G", 2)
    FC = cfg.get("FC", 896)
    RC = cfg.get("RC", 64)
    NS = cfg.get("NS", 3)
    LAG = cfg.get("lag", 2)
    NO = 8

    def kernel(x_h, mem0_ref, wq_h, wk_h, wv_h, wo_h, wg_h, wu_h, wd_h, o_h,
               wq_p, wk_p, wv_p, wo_p, wg_p, wu_p, wd_p, eo_p, eu_p, ed_p, stage_ref,
               xs_ref, hc_ref, x_ref, y_ref,
               sem_s, sem_o, sem_f, sem_x, sem_out, *, M, seg, H, Dh, n_seg):
        wo_ref, wg_ref, wu_ref, wd_ref, eo_ref, eu_ref, ed_ref = (
            r.bitcast(BF16) for r in (wo_p, wg_p, wu_p, wd_p, eo_p, eu_p, ed_p))
        out_ref = x_ref
        Dm = xs_ref.shape[1]
        DF = wg_ref.shape[1]
        scale = Dh ** -0.5
        NG = H // G
        NF = DF // FC
        S2 = 2 * seg
        cs = lambda g: slice(g * G * Dh, (g + 1) * G * Dh)
        fs = lambda f: slice(f * FC, (f + 1) * FC)
        hsl = lambda i: slice(i * Dh, (i + 1) * Dh)

        def h_rows(r, n):
            return pl.ds(r if isinstance(r, int) else pl.multiple_of(r, M), n)

        def aligned(r, n):
            return pl.ds(r if isinstance(r, int) else pl.multiple_of(r, seg), n)

        D2 = Dm // 2
        NRC = D2 // RC
        raw = [(src, dst, r) for src, dst in ((wq_h, wq_p), (wk_h, wk_p), (wv_h, wv_p)) for r in range(NRC)]
        nr = len(raw)
        OR = H * Dh // NO

        class Both:
            def __init__(self, i):
                src, _, r = raw[i]
                self.parts = [pltpu.make_async_copy(src.at[pl.ds((half * D2 + r * RC) * H, RC * H), :],
                                                    stage_ref.at[i % NS, half], sem_s.at[i % NS, half]) for half in range(2)]

            def start(self):
                for p in self.parts:
                    p.start()

            def wait(self):
                for p in self.parts:
                    p.wait()

        def wo_copy(i):
            return pltpu.make_async_copy(wo_h.at[pl.ds(i * OR, OR), :], wo_ref.at[pl.ds(i * OR, OR), :], sem_o.at[i])

        def ffn_copy(i):
            src, dst = ((wg_h, wg_ref), (wu_h, wu_ref), (wd_h, wd_ref))[i]
            return pltpu.make_async_copy(src, dst, sem_f.at[i])

        queue = [Both(i) for i in range(nr)] + [wo_copy(i) for i in range(NO)] + [ffn_copy(i) for i in range(3)]
        gate, up, down_copy = queue[nr + NO:]
        started = [0]

        def start_upto(n):
            while started[0] < min(n, len(queue)):
                queue[started[0]].start()
                started[0] += 1

        def unpack(t):
            return [pltpu.unpack_elementwise(t, index=i, packed_dtype=BF16, unpacked_dtype=F32) for i in range(2)]

        def pack(lo, hi):
            return pltpu.pack_elementwise((lo, hi), packed_dtype=BF16).astype(U32)

        def strassen_rhs(b11, b12, b21, b22):
            return (b11 + b22, b11, b12 - b22, b21 - b11, b22, b11 + b12, b21 + b22)

        def relayout(i):
            _, dst, r = raw[i]
            u = [stage_ref.at[i % NS, half].bitcast(U32) for half in range(2)]
            HP = H // 2

            def body(b, carry):
                ub = [t.at[pl.ds(pl.multiple_of(b * (16 * HP), 16 * HP), 16 * HP), :] for t in u]
                rows = pl.ds(pl.multiple_of((r * RC // 2) + b * 8, 8), 8)
                for j in range(HP):
                    res = []
                    for par in range(2):
                        top, bot = (unpack(t[pl.ds(par * HP + j, 8, stride=2 * HP), :]) for t in ub)
                        res.append(strassen_rhs(top[0], top[1], bot[0], bot[1]))
                    for n in range(7):
                        dst[n, rows, hsl(j)] = pack(res[0][n], res[1][n])
                return carry
            jax.lax.fori_loop(0, RC // 16, body, 0)

        def segs(t, n=1):
            return aligned(t * seg, n * seg)

        x_first = pltpu.make_async_copy(x_h.at[0:4 * seg, :], x_ref.at[0:4 * seg, :], sem_x.at[0])
        x_rest = pltpu.make_async_copy(x_h.at[4 * seg:n_seg * seg, :], x_ref.at[4 * seg:n_seg * seg, :], sem_x.at[1])

        def out_copy(t, n):
            return pltpu.make_async_copy(out_ref.at[segs(t, n), :], o_h.at[segs(t, n), :], sem_out)

        def strassen_lhs(a11, a12, a21, a22):
            return (a11 + a22, a21 + a22, a11, a22, a11 + a12, a21 - a11, a12 - a22)

        def strassen_out(m):
            return ((m[3] - m[4]) + m[0] + m[6], m[2] + m[4], m[1] + m[3], (m[2] - m[1]) + m[0] + m[5])

        def product(lhs, rhs):
            m = [None] * 7
            if len(lhs) == 7:
                for n in cfg.get("aord", (2, 3, 1, 4, 0, 5, 6)):
                    m[n] = _dot(lhs[n], rhs(n))
                return strassen_out(m)
            a11, a12 = lhs
            both = a11 + a12
            right = _dot(a11, rhs(2))
            left = _dot(a12, rhs(3))
            return left + _dot(both, rhs(1)), right + _dot(both, rhs(4))

        def operands(hs, lo, hi):
            quads = [t for h in hs for t in (h[:, lo], h[:, hi])]
            return strassen_lhs(*quads) if len(hs) == 2 else quads

        L = M + seg
        halves = (slice(0, D2), slice(D2, Dm))

        def attention(load_hs, order, G, WG, wait_wo=None, fill_in={}, residual=None):
            hs = load_hs()
            nl = len(hs)
            R = nl * L
            NG = H // G
            ri = jax.lax.broadcasted_iota(jnp.int32, (R, 128), 0)
            ci = jax.lax.broadcasted_iota(jnp.int32, (R, 128), 1)
            rl, cl = (ri >= L).astype(jnp.int32), (ci >= L).astype(jnp.int32)
            rp, cp = ri - rl * L, ci - cl * L
            same = (rl == cl) & (ci < R)
            keep = same & ((rp < M) | (rp >= cp))
            fill = jnp.where(same, -1e9, -jnp.inf).astype(F32)
            z = jnp.zeros((128 - R, Dh), F32)
            lhs = list(operands(hs, slice(0, D2), slice(D2, Dm)))

            def proj(w, g):
                c = product(lhs, lambda n: pltpu.bitcast(w[n, :, g * (G // 2) * Dh:(g + 1) * (G // 2) * Dh], BF16))
                return [jnp.concatenate([c[2 * l + i % 2][:, hsl(i // 2)] for l in range(nl)], axis=0) for i in range(G)]

            def as_rhs(t):
                return jnp.concatenate([t, z], axis=0).astype(BF16)

            def softmax(s):
                s = jnp.where(keep, s * scale, fill)
                e = jnp.exp(s - jnp.max(s, axis=-1, keepdims=True))
                return e * pl.reciprocal(jnp.sum(e, axis=-1, keepdims=True), approx=False)

            acc = []
            os = {}

            def wo(g):
                if g == 0 and wait_wo is not None:
                    wait_wo()
                if (g + 1) % WG and not (cfg.get("split", 1) and g == NG - 2):
                    return
                o = [t for i in sorted(os) if i <= g for t in os.pop(i)]
                n2 = len(o) // 2
                ol = operands([jnp.concatenate([t[l * L:(l + 1) * L] for t in o[0::2] + o[1::2]], axis=1) for l in range(nl)],
                              slice(0, n2 * Dh), slice(n2 * Dh, 2 * n2 * Dh))
                pairs = range((g + 1) * G // 2 - n2, (g + 1) * G // 2)

                def rhs(n):
                    if n in (0, 5, 6):
                        return eo_ref[{0: 0, 5: 1, 6: 2}[n], pairs[0] * Dh:(pairs[-1] + 1) * Dh, :]
                    odd, cols = {1: (0, slice(0, D2)), 2: (0, slice(D2, Dm)), 3: (1, slice(0, D2)), 4: (1, slice(D2, Dm))}[n]
                    parts = [wo_ref[(2 * p + odd) * Dh:(2 * p + odd + 1) * Dh, cols] for p in pairs]
                    return parts[0] if len(parts) == 1 else jnp.concatenate(parts, axis=0)
                if nl == 2 and g == NG - 1:
                    out = [t + r for t, r in zip(strassen_out(acc), residual())]
                    for n, plus, minus in ((0, (0, 3), ()), (3, (0, 2), ()), (4, (1,), (0,)), (1, (2,), (3,)),
                                           (2, (1, 3), ()), (5, (3,), ()), (6, (0,), ())):
                        t = _dot(ol[n], rhs(n))
                        for i in plus:
                            out[i] = out[i] + t
                        for i in minus:
                            out[i] = out[i] - t
                    acc[:] = out
                    return
                if nl == 2:
                    c = [_dot(ol[n], rhs(n)) for n in range(7)]
                else:
                    c = product(ol, rhs)
                acc[:] = list(c) if not acc else [x + y for x, y in zip(acc, c)]

            steps = [(w[0], int(w[1:])) for w in order.split()]
            q, k, v, sc = {}, {}, {}, {}
            for g in range(-max(o for _, o in steps), NG - min(o for _, o in steps)):
                if g in fill_in:
                    fill_in[g]()
                    if cfg.get('reload', 1):
                        lhs[2] = load_hs()[0][:, 0:D2]
                for op, off in steps:
                    i = g + off
                    if not 0 <= i < NG:
                        continue
                    if op == "q":
                        q[i] = proj(wq_p, i)
                    elif op == "k":
                        k[i] = [as_rhs(t) for t in proj(wk_p, i)]
                    elif op == "v":
                        v[i] = [as_rhs(t) for t in proj(wv_p, i)]
                    elif op == "s":
                        sc[i] = [jax.lax.dot_general(a, b, (((1,), (1,)), ((), ())), preferred_element_type=F32)
                                 for a, b in zip(q.pop(i), k.pop(i))]
                    elif op == "e":
                        sc[i] = [softmax(t) for t in sc[i]]
                    elif op == "p":
                        os[i] = [_dot(a, b) for a, b in zip(sc.pop(i), v.pop(i))]
                    elif op == "w":
                        wo(i)
            return acc

        R2 = 2 * L
        NC = (n_seg - 4) // 2 + 2
        last = NC - 1

        NP = NF // 2

        def strassen_rhs_prepare(b11, b12, b21, b22, e0, e1, e2):
            res = [strassen_rhs(*t) for t in zip(*(unpack(r[...]) for r in (b11, b12, b21, b22)))]
            for dst, n in ((e0, 0), (e1, 5), (e2, 6), (b12, 2), (b21, 3)):
                dst[...] = pack(res[0][n], res[1][n])

        def prepare_wo(i):
            ppc = OR // (2 * Dh)

            def body(b, carry):
                p, r = i * ppc + b // 4, (b % 4) * 16
                for n in range(2):
                    r0, r1, re = (pl.ds(pl.multiple_of(row * (Dh // 2) + r + 8 * n, 8), 8) for row in (2 * p, 2 * p + 1, p))
                    strassen_rhs_prepare(wo_p.at[r0, 0:D2], wo_p.at[r0, D2:Dm], wo_p.at[r1, 0:D2], wo_p.at[r1, D2:Dm],
                                         *(eo_p.at[n2, re, :] for n2 in range(3)))
                return carry
            jax.lax.fori_loop(0, ppc * 4, body, 0)

        def prepare_up():
            def body(b, carry):
                r = pl.multiple_of(b * 8, 8)
                top, bot = pl.ds(r, 8), pl.ds(pl.multiple_of(D2 // 2 + r, 8), 8)
                for k in range(0, DF, 512):
                    c = slice(k, k + 512)
                    strassen_rhs_prepare(wg_p.at[top, c], wu_p.at[top, c], wg_p.at[bot, c], wu_p.at[bot, c],
                                         *(eu_p.at[i, top, c] for i in range(3)))
                return carry
            jax.lax.fori_loop(0, D2 // 16, body, 0)

        def prepare_down():
            F2 = FC // 2
            nb = F2 // 56

            def body(b, carry):
                p, r = b // nb, (b % nb) * 56
                for i in range(7):
                    r0 = pl.ds(pl.multiple_of(2 * p * F2 + r + 8 * i, 8), 8)
                    r1 = pl.ds(pl.multiple_of((2 * p + 1) * F2 + r + 8 * i, 8), 8)
                    re = pl.ds(pl.multiple_of(p * F2 + r + 8 * i, 8), 8)
                    strassen_rhs_prepare(wd_p.at[r0, 0:D2], wd_p.at[r0, D2:Dm], wd_p.at[r1, 0:D2], wd_p.at[r1, D2:Dm],
                                         *(ed_p.at[i2, re, :] for i2 in range(3)))
                return carry
            jax.lax.fori_loop(0, NP * nb, body, 0)

        def ffn():
            ha = hc_ref[2 * R2:2 * R2 + S2, :]
            hb = _ln(xs_ref[S2:2 * S2, :])
            lhs = [t.astype(BF16) for t in operands((ha, hb), slice(0, D2), slice(D2, Dm))]

            def hidden(f):
                rhs = (eu_ref[0, :, fs(f)], wg_ref[0:D2, fs(f)], wu_ref[0:D2, fs(f)], wg_ref[D2:Dm, fs(f)],
                       wu_ref[D2:Dm, fs(f)], eu_ref[1, :, fs(f)], eu_ref[2, :, fs(f)])
                m = [None] * 7
                for i in cfg.get("mord", (2, 3, 1, 4, 0, 5, 6)):
                    m[i] = _dot(lhs[i], rhs[i])
                ga, ua, gb, ub = strassen_out(m)
                return _gelu(ga) * ua, _gelu(gb) * ub

            acc = [xs_ref[0:S2, 0:D2], xs_ref[0:S2, D2:Dm], xs_ref[S2:2 * S2, 0:D2], xs_ref[S2:2 * S2, D2:Dm]]

            def down(p, h0, h1):
                f0, f1 = fs(2 * p), fs(2 * p + 1)
                dl = [t.astype(BF16) for t in strassen_lhs(h0[0], h1[0], h0[1], h1[1])]
                rhs = (ed_ref[0, fs(p), :], wd_ref[f0, 0:D2], wd_ref[f0, D2:Dm], wd_ref[f1, 0:D2],
                       wd_ref[f1, D2:Dm], ed_ref[1, fs(p), :], ed_ref[2, fs(p), :])
                m = [None] * 7
                for i in cfg.get("dord", (0, 1, 3, 4, 6, 2, 5)):
                    m[i] = _dot(dl[i], rhs[i])
                acc[0] = acc[0] + m[0] + m[3] - m[4] + m[6]
                acc[1] = acc[1] + m[4] + m[2]
                acc[2] = acc[2] + m[1] + m[3]
                acc[3] = acc[3] + m[0] - m[1] + m[2] + m[5]

            dlag = cfg.get("dlag", 1)
            hs = []
            for f in range(NF + dlag):
                if f < NF:
                    hs.append(hidden(f))
                e = f - dlag
                if e >= 0 and e % 2 == 1:
                    down(e // 2, hs[e - 1], hs[e])
            return acc

        x_first.start()
        start_upto(NS)
        for i in range(nr):
            queue[i].wait()
            relayout(i)
            start_upto(i + NS + 1)
        start_upto(nr + NO)
        x_first.wait()

        def single_block(c):
            @pl.when(c == 0)
            def _():
                hc_ref[0:M, :] = mem0_ref[...].astype(F32)
                y_ref[0:4 * seg, :] = x_ref[0:4 * seg, :].astype(F32)

            @pl.when(c == last)
            def _():
                hc_ref[0:M, :] = hc_ref[L:L + M, :]

            s0 = jnp.where(c == 0, 0, n_seg - 4)

            def single(j, carry):
                def wait_wo():
                    @pl.when(c == 0)
                    def _():
                        @pl.when(j == 0)
                        def _():
                            for i in range(NO):
                                queue[nr + i].wait()
                                if i == 0:
                                    gate.start()
                                    up.start()
                                prepare_wo(i)

                        @pl.when(j == 2)
                        def _():
                            down_copy.start()
                x = y_ref[segs(s0 + j), :]
                h = jnp.concatenate([hc_ref[0:M, :], _ln(x)], axis=0)
                acc = jnp.concatenate(attention(lambda: [h], cfg.get('sorder', 's0 q1 k1 v1 e0 p0') + ' w-%d' % (2 * H), cfg.get('sG', 2), cfg.get('sWG', 2), wait_wo), axis=1)
                hc_ref[0:M, :] = acc[0:M]
                xs_ref[segs(j), :] = x + acc[M:L]
                return carry
            jax.lax.fori_loop(0, 4, single, 0)
            hc_ref[2 * R2:2 * R2 + S2, :] = _ln(xs_ref[0:S2, :])

            @pl.when(c == 0)
            def _():
                hc_ref[L:L + M, :] = mem0_ref[...].astype(F32)
                gate.wait()
                up.wait()
                prepare_up()
                down_copy.wait()
                x_rest.start()
                prepare_down()

        def a_step(c, j):
            t = 2 * (c - 1) + j
            cur = j * R2
            nxt = (1 - j) * R2

            def fill_x():
                hc_ref[h_rows(nxt + M, seg), :] = _ln(x_ref[segs(jnp.minimum(t + 5, n_seg - 1)), :].astype(F32))

            def fill_y():
                hc_ref[h_rows(nxt + L + M, seg), :] = _ln(y_ref[segs(t + 1), :])

            def fill_b():
                hc_ref[2 * R2:2 * R2 + S2, :] = _ln(xs_ref[0:S2, :])

            def fill_o():
                done = jnp.maximum(t - 2, 0)
                out_ref[segs(done), :] = y_ref[segs(done), :].astype(out_ref.dtype)
            f0, f1 = cfg.get("f0", 1), cfg.get("f1", 1)

            def residual():
                zero = jnp.zeros((M, Dm), F32)
                rows = [jnp.concatenate([zero, r], axis=0) for r in (x_ref[segs(t + 4), :].astype(F32), y_ref[segs(t), :])]
                return [r[:, cols] for r in rows for cols in halves]
            acc = attention(lambda: [hc_ref[h_rows(cur + l * L, L), :] for l in range(2)],
                            cfg.get('order', 's0 q1 k1 v1 w-2 e0 p0'), G, cfg.get('WG', 2),
                            fill_in={f0: fill_o, f0 + f1: fill_x, f0 + 2 * f1: fill_y, f0 + 3 * f1: fill_b},
                            residual=residual)
            for i in (2, 1, 3, 0):
                l, cols = i // 2, halves[i % 2]
                hc_ref[h_rows(nxt + l * L, M), cols] = acc[i][0:M]
                xs_ref[segs(2 * j + l), cols] = acc[i][M:L]

        def step(c, carry):
            edge = (c == 0) | (c == last)

            @pl.when(edge)
            def _():
                single_block(c)

            @pl.when(jnp.logical_not(edge))
            def _():
                @pl.when(c == 1)
                def _():
                    x_rest.wait()
                    hc_ref[M:L, :] = _ln(x_ref[segs(4), :].astype(F32))
                    hc_ref[L + M:R2, :] = _ln(y_ref[segs(0), :])
                if not cfg.get('skipA'):
                    jax.lax.fori_loop(0, 2, lambda j, z: (a_step(c, j), z)[1], 0)

                @pl.when(c >= 2)
                def _():
                    out_copy(2 * (c - 2), 2).start()

            r = xs_ref[...] if cfg.get('skipB') else ffn()
            t0 = 2 * (c - 1)
            s0 = jnp.where(c == 0, 0, n_seg - 4)
            dst = [jnp.where(edge, s0 + i, t0 + i // 2 + (4 if i % 2 == 0 else 0)) for i in range(4)]
            for i in (0, 2, 1, 3):
                for n in range(2):
                    y_ref[segs(dst[2 * (i // 2) + n]), halves[i % 2]] = r[i][n * seg:(n + 1) * seg]
            return carry
        jax.lax.fori_loop(0, NC, step, 0)

        out_ref[segs(n_seg - 6, 6), :] = y_ref[segs(n_seg - 6, 6), :].astype(out_ref.dtype)
        out_copy(n_seg - 6, 6).start()
        for c in range(NC - 3):
            out_copy(2 * c, 2).wait()
        out_copy(n_seg - 6, 6).wait()

    @functools.partial(jax.jit, static_argnames=("A_seg_len",))
    def run(A_x, A_mem0, A_Wq, A_Wk, A_Wv, A_Wo, A_seg_len, B_x, B_w_gate, B_w_up, B_w_down):
        B, S, Dm = A_x.shape
        H, Dh = A_Wq.shape[1:]
        M = A_mem0.shape[1]
        seg = A_seg_len
        DF = B_w_gate.shape[1]
        hbm = pl.BlockSpec(memory_space=pl.ANY)
        packed = lambda r, c: pltpu.VMEM((r // 2, c), U32)
        proj = pltpu.VMEM((7, Dm // 4, H * Dh // 2), U32)
        out = pl.pallas_call(
            functools.partial(kernel, M=M, seg=seg, H=H, Dh=Dh, n_seg=cfg.get("ns", S // seg)),
            in_specs=[hbm, pl.BlockSpec(memory_space=pltpu.VMEM), hbm, hbm, hbm, hbm, hbm, hbm, hbm],
            out_specs=hbm,
            out_shape=jax.ShapeDtypeStruct((S, Dm), A_x.dtype),
            scratch_shapes=[
                proj, proj, proj,
                packed(H * Dh, Dm), packed(Dm, DF), packed(Dm, DF), packed(DF, Dm),
                pltpu.VMEM((3, H * Dh // 4, Dm // 2), U32),
                pltpu.VMEM((3, Dm // 4, DF), U32),
                pltpu.VMEM((3, DF // 4, Dm // 2), U32),
                pltpu.VMEM((NS, 2, RC * H, Dh), BF16),
                pltpu.VMEM((4 * seg, Dm), F32),
                pltpu.VMEM((4 * (M + seg) + 2 * seg, Dm), F32),
                pltpu.VMEM((S, Dm), BF16),
                pltpu.VMEM((S, Dm), F32),
                pltpu.SemaphoreType.DMA((NS, 2)),
                pltpu.SemaphoreType.DMA((NO,)),
                pltpu.SemaphoreType.DMA((3,)),
                pltpu.SemaphoreType.DMA((2,)),
                pltpu.SemaphoreType.DMA(()),
            ],
            compiler_params=pltpu.CompilerParams(vmem_limit_bytes=126 * 1024 * 1024),
        )(A_x.reshape(S, Dm), A_mem0.reshape(M, Dm),
          A_Wq.reshape(Dm * H, Dh), A_Wk.reshape(Dm * H, Dh), A_Wv.reshape(Dm * H, Dh),
          A_Wo.reshape(H * Dh, Dm), B_w_gate, B_w_up, B_w_down)
        return out.reshape(B, S, Dm)
    return run


_run = build({})


@functools.partial(jax.jit, static_argnames=("A_seg_len",))
def pallas_interleave_layers__memory_aug_recurrent_mem_tr__glu_gated_geglu__prompt_kernel(
    A_x, A_mem0, A_Wq, A_Wk, A_Wv, A_Wo, A_seg_len, B_x, B_w_gate, B_w_up, B_w_down
):
    return _run(A_x, A_mem0, A_Wq, A_Wk, A_Wv, A_Wo, A_seg_len, B_x, B_w_gate, B_w_up, B_w_down)
```

```python
import functools
import jax
import jax.numpy as jnp
import numpy as np
import jax.experimental.pallas as pl
import jax.experimental.pallas.tpu as pltpu

F32 = jnp.float32
BF16 = jnp.bfloat16
U32 = jnp.uint32


def _ln(x):
    m = jnp.mean(x, axis=-1, keepdims=True)
    d = x - m
    v = jnp.mean(d * d, axis=-1, keepdims=True)
    return d * jax.lax.rsqrt(v + 1e-5)


def _gelu(x):
    c = 0.7978845608028654
    return 0.5 * x * (1.0 + jnp.tanh(c * (x + 0.044715 * (x * x * x))))


def _dot(a, b):
    return jnp.dot(a, b, preferred_element_type=F32)


def build(cfg):
    G = cfg.get("G", 2)
    FC = cfg.get("FC", 896)
    RC = cfg.get("RC", 64)
    NS = cfg.get("NS", 3)
    LAG = cfg.get("lag", 2)
    NO = 8

    def kernel(x_h, mem0_ref, wq_h, wk_h, wv_h, wo_h, wg_h, wu_h, wd_h, o_h,
               wq_p, wk_p, wv_p, wo_p, wg_p, wu_p, wd_p, eo_p, eu_p, ed_p, stage_ref,
               xs_ref, hc_ref, x_ref, y_ref,
               sem_s, sem_o, sem_f, sem_x, sem_out, *, M, seg, H, Dh, n_seg):
        wo_ref, wg_ref, wu_ref, wd_ref, eo_ref, eu_ref, ed_ref = (
            r.bitcast(BF16) for r in (wo_p, wg_p, wu_p, wd_p, eo_p, eu_p, ed_p))
        out_ref = x_ref
        Dm = xs_ref.shape[1]
        DF = wg_ref.shape[1]
        scale = Dh ** -0.5
        NG = H // G
        NF = DF // FC
        S2 = 2 * seg
        cs = lambda g: slice(g * G * Dh, (g + 1) * G * Dh)
        fs = lambda f: slice(f * FC, (f + 1) * FC)
        hsl = lambda i: slice(i * Dh, (i + 1) * Dh)

        def h_rows(r, n):
            return pl.ds(r if isinstance(r, int) else pl.multiple_of(r, M), n)

        def aligned(r, n):
            return pl.ds(r if isinstance(r, int) else pl.multiple_of(r, seg), n)

        D2 = Dm // 2
        NRC = D2 // RC
        assert NS <= NRC
        proj_w = ((wq_h, wq_p), (wk_h, wk_p), (wv_h, wv_p))
        OR = H * Dh // NO

        def raw_copies(w, r):
            slot = (w * NRC + r) % NS
            return [pltpu.make_async_copy(proj_w[w][0].at[pl.ds(pl.multiple_of((half * D2 + r * RC) * H, RC * H), RC * H), :],
                                          stage_ref.at[slot, half], sem_s.at[slot, half]) for half in range(2)]

        def wo_copy(i):
            return pltpu.make_async_copy(wo_h.at[pl.ds(i * OR, OR), :], wo_ref.at[pl.ds(i * OR, OR), :], sem_o.at[i])

        def ffn_copy(i):
            src, dst = ((wg_h, wg_ref), (wu_h, wu_ref), (wd_h, wd_ref))[i]
            return pltpu.make_async_copy(src, dst, sem_f.at[i])

        wo_copies = [wo_copy(i) for i in range(NO)]
        gate, up, down_copy = (ffn_copy(i) for i in range(3))

        def unpack(t):
            return [pltpu.unpack_elementwise(t, index=i, packed_dtype=BF16, unpacked_dtype=F32) for i in range(2)]

        def pack(lo, hi):
            return pltpu.pack_elementwise((lo, hi), packed_dtype=BF16).astype(U32)

        def strassen_rhs(b11, b12, b21, b22):
            return (b11 + b22, b11, b12 - b22, b21 - b11, b22, b11 + b12, b21 + b22)

        def relayout(w, r):
            dst = proj_w[w][1]
            u = [stage_ref.at[(w * NRC + r) % NS, half].bitcast(U32) for half in range(2)]
            HP = H // 2

            def body(b, carry):
                ub = [t.at[pl.ds(pl.multiple_of(b * (16 * HP), 16 * HP), 16 * HP), :] for t in u]
                rows = pl.ds(pl.multiple_of(r * (RC // 2) + b * 8, 8), 8)
                for j in range(HP):
                    res = []
                    for par in range(2):
                        top, bot = (unpack(t[pl.ds(par * HP + j, 8, stride=2 * HP), :]) for t in ub)
                        res.append(strassen_rhs(top[0], top[1], bot[0], bot[1]))
                    for n in range(7):
                        dst[n, rows, hsl(j)] = pack(res[0][n], res[1][n])
                return carry
            jax.lax.fori_loop(0, RC // 16, body, 0)

        def segs(t, n=1):
            return aligned(t * seg, n * seg)

        x_first = pltpu.make_async_copy(x_h.at[0:4 * seg, :], x_ref.at[0:4 * seg, :], sem_x.at[0])
        x_rest = pltpu.make_async_copy(x_h.at[4 * seg:n_seg * seg, :], x_ref.at[4 * seg:n_seg * seg, :], sem_x.at[1])

        def out_copy(t, n):
            return pltpu.make_async_copy(out_ref.at[segs(t, n), :], o_h.at[segs(t, n), :], sem_out)

        def strassen_lhs(a11, a12, a21, a22):
            return (a11 + a22, a21 + a22, a11, a22, a11 + a12, a21 - a11, a12 - a22)

        def strassen_out(m):
            return ((m[3] - m[4]) + m[0] + m[6], m[2] + m[4], m[1] + m[3], (m[2] - m[1]) + m[0] + m[5])

        def product(lhs, rhs):
            m = [None] * 7
            if len(lhs) == 7:
                for n in cfg.get("aord", (2, 3, 1, 4, 0, 5, 6)):
                    m[n] = _dot(lhs[n], rhs(n))
                return strassen_out(m)
            a11, a12 = lhs
            both = a11 + a12
            right = _dot(a11, rhs(2))
            left = _dot(a12, rhs(3))
            return left + _dot(both, rhs(1)), right + _dot(both, rhs(4))

        def operands(hs, lo, hi):
            quads = [t for h in hs for t in (h[:, lo], h[:, hi])]
            return strassen_lhs(*quads) if len(hs) == 2 else quads

        L = M + seg
        halves = (slice(0, D2), slice(D2, Dm))

        def attention(load_hs, order, G, WG, wait_wo=None, fill_in={}, residual=None):
            hs = load_hs()
            nl = len(hs)
            R = nl * L
            NG = H // G
            ri = jax.lax.broadcasted_iota(jnp.int32, (R, 128), 0)
            ci = jax.lax.broadcasted_iota(jnp.int32, (R, 128), 1)
            rl, cl = (ri >= L).astype(jnp.int32), (ci >= L).astype(jnp.int32)
            rp, cp = ri - rl * L, ci - cl * L
            same = (rl == cl) & (ci < R)
            keep = same & ((rp < M) | (rp >= cp))
            fill = jnp.where(same, -1e9, -jnp.inf).astype(F32)
            z = jnp.zeros((128 - R, Dh), F32)
            lhs = list(operands(hs, slice(0, D2), slice(D2, Dm)))

            def proj(w, g):
                c = product(lhs, lambda n: pltpu.bitcast(w[n, :, g * (G // 2) * Dh:(g + 1) * (G // 2) * Dh], BF16))
                return [jnp.concatenate([c[2 * l + i % 2][:, hsl(i // 2)] for l in range(nl)], axis=0) for i in range(G)]

            def as_rhs(t):
                return jnp.concatenate([t, z], axis=0).astype(BF16)

            def softmax(s):
                s = jnp.where(keep, s * scale, fill)
                e = jnp.exp(s - jnp.max(s, axis=-1, keepdims=True))
                return e * pl.reciprocal(jnp.sum(e, axis=-1, keepdims=True), approx=False)

            acc = []
            os = {}

            def wo(g):
                if g == 0 and wait_wo is not None:
                    wait_wo()
                if (g + 1) % WG and not (cfg.get("split", 1) and g == NG - 2):
                    return
                o = [t for i in sorted(os) if i <= g for t in os.pop(i)]
                n2 = len(o) // 2
                ol = operands([jnp.concatenate([t[l * L:(l + 1) * L] for t in o[0::2] + o[1::2]], axis=1) for l in range(nl)],
                              slice(0, n2 * Dh), slice(n2 * Dh, 2 * n2 * Dh))
                pairs = range((g + 1) * G // 2 - n2, (g + 1) * G // 2)

                def rhs(n):
                    if n in (0, 5, 6):
                        return eo_ref[{0: 0, 5: 1, 6: 2}[n], pairs[0] * Dh:(pairs[-1] + 1) * Dh, :]
                    odd, cols = {1: (0, slice(0, D2)), 2: (0, slice(D2, Dm)), 3: (1, slice(0, D2)), 4: (1, slice(D2, Dm))}[n]
                    parts = [wo_ref[(2 * p + odd) * Dh:(2 * p + odd + 1) * Dh, cols] for p in pairs]
                    return parts[0] if len(parts) == 1 else jnp.concatenate(parts, axis=0)
                if nl == 2 and g == NG - 1:
                    out = [t + r for t, r in zip(strassen_out(acc), residual())]
                    for n, plus, minus in ((0, (0, 3), ()), (3, (0, 2), ()), (4, (1,), (0,)), (1, (2,), (3,)),
                                           (2, (1, 3), ()), (5, (3,), ()), (6, (0,), ())):
                        t = _dot(ol[n], rhs(n))
                        for i in plus:
                            out[i] = out[i] + t
                        for i in minus:
                            out[i] = out[i] - t
                    acc[:] = out
                    return
                if nl == 2:
                    c = [_dot(ol[n], rhs(n)) for n in range(7)]
                else:
                    c = product(ol, rhs)
                acc[:] = list(c) if not acc else [x + y for x, y in zip(acc, c)]

            steps = [(w[0], int(w[1:])) for w in order.split()]
            q, k, v, sc = {}, {}, {}, {}
            for g in range(-max(o for _, o in steps), NG - min(o for _, o in steps)):
                if g in fill_in:
                    fill_in[g]()
                    if cfg.get('reload', 1):
                        lhs[2] = load_hs()[0][:, 0:D2]
                for op, off in steps:
                    i = g + off
                    if not 0 <= i < NG:
                        continue
                    if op == "q":
                        q[i] = proj(wq_p, i)
                    elif op == "k":
                        k[i] = [as_rhs(t) for t in proj(wk_p, i)]
                    elif op == "v":
                        v[i] = [as_rhs(t) for t in proj(wv_p, i)]
                    elif op == "s":
                        sc[i] = [jax.lax.dot_general(a, b, (((1,), (1,)), ((), ())), preferred_element_type=F32)
                                 for a, b in zip(q.pop(i), k.pop(i))]
                    elif op == "e":
                        sc[i] = [softmax(t) for t in sc[i]]
                    elif op == "p":
                        os[i] = [_dot(a, b) for a, b in zip(sc.pop(i), v.pop(i))]
                    elif op == "w":
                        wo(i)
            return acc

        R2 = 2 * L
        NC = (n_seg - 4) // 2 + 2
        last = NC - 1

        NP = NF // 2

        def strassen_rhs_prepare(b11, b12, b21, b22, e0, e1, e2):
            res = [strassen_rhs(*t) for t in zip(*(unpack(r[...]) for r in (b11, b12, b21, b22)))]
            for dst, n in ((e0, 0), (e1, 5), (e2, 6), (b12, 2), (b21, 3)):
                dst[...] = pack(res[0][n], res[1][n])

        def prepare_wo(i):
            ppc = OR // (2 * Dh)

            def body(b, carry):
                p, r = i * ppc + b // 4, (b % 4) * 16
                for n in range(2):
                    r0, r1, re = (pl.ds(pl.multiple_of(row * (Dh // 2) + r + 8 * n, 8), 8) for row in (2 * p, 2 * p + 1, p))
                    strassen_rhs_prepare(wo_p.at[r0, 0:D2], wo_p.at[r0, D2:Dm], wo_p.at[r1, 0:D2], wo_p.at[r1, D2:Dm],
                                         *(eo_p.at[n2, re, :] for n2 in range(3)))
                return carry
            jax.lax.fori_loop(0, ppc * 4, body, 0, unroll=4)

        def prepare_up():
            def body(b, carry):
                r = pl.multiple_of(b * 8, 8)
                top, bot = pl.ds(r, 8), pl.ds(pl.multiple_of(D2 // 2 + r, 8), 8)
                for k in range(0, DF, 512):
                    c = slice(k, k + 512)
                    strassen_rhs_prepare(wg_p.at[top, c], wu_p.at[top, c], wg_p.at[bot, c], wu_p.at[bot, c],
                                         *(eu_p.at[i, top, c] for i in range(3)))
                return carry
            jax.lax.fori_loop(0, D2 // 16, body, 0, unroll=cfg.get('pu', 2))

        def prepare_down():
            F2 = FC // 2
            nb = F2 // 56

            def body(b, carry):
                p, r = b // nb, (b % nb) * 56
                for i in range(7):
                    r0 = pl.ds(pl.multiple_of(2 * p * F2 + r + 8 * i, 8), 8)
                    r1 = pl.ds(pl.multiple_of((2 * p + 1) * F2 + r + 8 * i, 8), 8)
                    re = pl.ds(pl.multiple_of(p * F2 + r + 8 * i, 8), 8)
                    strassen_rhs_prepare(wd_p.at[r0, 0:D2], wd_p.at[r0, D2:Dm], wd_p.at[r1, 0:D2], wd_p.at[r1, D2:Dm],
                                         *(ed_p.at[i2, re, :] for i2 in range(3)))
                return carry
            jax.lax.fori_loop(0, NP * nb, body, 0, unroll=cfg.get('pu', 2))

        def ffn():
            ha = hc_ref[2 * R2:2 * R2 + S2, :]
            hb = _ln(xs_ref[S2:2 * S2, :])
            lhs = [t.astype(BF16) for t in operands((ha, hb), slice(0, D2), slice(D2, Dm))]

            def hidden(f):
                rhs = (eu_ref[0, :, fs(f)], wg_ref[0:D2, fs(f)], wu_ref[0:D2, fs(f)], wg_ref[D2:Dm, fs(f)],
                       wu_ref[D2:Dm, fs(f)], eu_ref[1, :, fs(f)], eu_ref[2, :, fs(f)])
                m = [None] * 7
                for i in cfg.get("mord", (2, 3, 1, 4, 0, 5, 6)):
                    m[i] = _dot(lhs[i], rhs[i])
                ga, ua, gb, ub = strassen_out(m)
                return _gelu(ga) * ua, _gelu(gb) * ub

            acc = [xs_ref[0:S2, 0:D2], xs_ref[0:S2, D2:Dm], xs_ref[S2:2 * S2, 0:D2], xs_ref[S2:2 * S2, D2:Dm]]

            def down(p, h0, h1):
                f0, f1 = fs(2 * p), fs(2 * p + 1)
                dl = [t.astype(BF16) for t in strassen_lhs(h0[0], h1[0], h0[1], h1[1])]
                rhs = (ed_ref[0, fs(p), :], wd_ref[f0, 0:D2], wd_ref[f0, D2:Dm], wd_ref[f1, 0:D2],
                       wd_ref[f1, D2:Dm], ed_ref[1, fs(p), :], ed_ref[2, fs(p), :])
                m = [None] * 7
                for i in cfg.get("dord", (0, 1, 3, 4, 6, 2, 5)):
                    m[i] = _dot(dl[i], rhs[i])
                acc[0] = acc[0] + m[0] + m[3] - m[4] + m[6]
                acc[1] = acc[1] + m[4] + m[2]
                acc[2] = acc[2] + m[1] + m[3]
                acc[3] = acc[3] + m[0] - m[1] + m[2] + m[5]

            dlag = cfg.get("dlag", 1)
            hs = []
            for f in range(NF + dlag):
                if f < NF:
                    hs.append(hidden(f))
                e = f - dlag
                if e >= 0 and e % 2 == 1:
                    down(e // 2, hs[e - 1], hs[e])
            return acc

        x_first.start()
        for r in range(NS):
            for cp in raw_copies(0, r):
                cp.start()
        for w in range(3):
            def load(r, carry):
                for cp in raw_copies(w, r):
                    cp.wait()
                relayout(w, r)

                @pl.when(r + NS < NRC)
                def _():
                    for cp in raw_copies(w, r + NS):
                        cp.start()

                @pl.when(r + NS >= NRC)
                def _():
                    if w < 2:
                        for cp in raw_copies(w + 1, r + NS - NRC):
                            cp.start()
                    else:
                        i = r + NS - NRC
                        pltpu.make_async_copy(wo_h.at[pl.ds(pl.multiple_of(i * OR, OR), OR), :],
                                              wo_ref.at[pl.ds(pl.multiple_of(i * OR, OR), OR), :], sem_o.at[i]).start()
                return carry
            jax.lax.fori_loop(0, NRC, load, 0)
        for i in range(NS, NO):
            wo_copies[i].start()
        x_first.wait()

        def single_block(c):
            @pl.when(c == 0)
            def _():
                hc_ref[0:M, :] = mem0_ref[...].astype(F32)
                y_ref[0:4 * seg, :] = x_ref[0:4 * seg, :].astype(F32)

            @pl.when(c == last)
            def _():
                hc_ref[0:M, :] = hc_ref[L:L + M, :]
                out_ref[segs(n_seg - 6, 2), :] = y_ref[segs(n_seg - 6, 2), :].astype(out_ref.dtype)
                out_copy(n_seg - 6, 2).start()

            s0 = jnp.where(c == 0, 0, n_seg - 4)
            hc_ref[R2:R2 + 4 * seg, :] = _ln(y_ref[segs(s0, 4), :])

            def single(j, carry):
                def wait_wo():
                    @pl.when(c == 0)
                    def _():
                        @pl.when(j == 0)
                        def _():
                            for i in range(NO):
                                wo_copies[i].wait()
                                if i == 0:
                                    gate.start()
                                    up.start()
                                prepare_wo(i)

                        @pl.when(j == 2)
                        def _():
                            down_copy.start()
                h = jnp.concatenate([hc_ref[0:M, :], hc_ref[h_rows(R2 + j * seg, seg), :]], axis=0)
                acc = jnp.concatenate(attention(lambda: [h], cfg.get('sorder', 's0 q1 k1 v1 e0 p0') + ' w-%d' % (2 * H), cfg.get('sG', 4), cfg.get('sWG', 2), wait_wo), axis=1)
                hc_ref[0:M, :] = acc[0:M]
                xs_ref[segs(j), :] = y_ref[segs(s0 + j), :] + acc[M:L]
                return carry
            jax.lax.fori_loop(0, 4, single, 0)
            hc_ref[2 * R2:2 * R2 + S2, :] = _ln(xs_ref[0:S2, :])

            @pl.when(c == 0)
            def _():
                hc_ref[L:L + M, :] = mem0_ref[...].astype(F32)
                gate.wait()
                up.wait()
                prepare_up()
                down_copy.wait()
                x_rest.start()
                prepare_down()

        def a_step(c, j):
            t = 2 * (c - 1) + j
            cur = j * R2
            nxt = (1 - j) * R2

            def fill_x():
                hc_ref[h_rows(nxt + M, seg), :] = _ln(x_ref[segs(jnp.minimum(t + 5, n_seg - 1)), :].astype(F32))

            def fill_y():
                hc_ref[h_rows(nxt + L + M, seg), :] = _ln(y_ref[segs(t + 1), :])

            def fill_b():
                hc_ref[2 * R2:2 * R2 + S2, :] = _ln(xs_ref[0:S2, :])

            def fill_o():
                done = jnp.maximum(t - 2, 0)
                out_ref[segs(done), :] = y_ref[segs(done), :].astype(out_ref.dtype)
            f0, f1 = cfg.get("f0", 1), cfg.get("f1", 1)

            def residual():
                zero = jnp.zeros((M, Dm), F32)
                rows = [jnp.concatenate([zero, r], axis=0) for r in (x_ref[segs(t + 4), :].astype(F32), y_ref[segs(t), :])]
                return [r[:, cols] for r in rows for cols in halves]
            acc = attention(lambda: [hc_ref[h_rows(cur + l * L, L), :] for l in range(2)],
                            cfg.get('order', 's0 q1 k1 v1 w-2 e0 p0'), G, cfg.get('WG', 2),
                            fill_in={f0: fill_o, f0 + f1: fill_x, f0 + 2 * f1: fill_y, f0 + 3 * f1: fill_b},
                            residual=residual)
            for i in (2, 1, 3, 0):
                l, cols = i // 2, halves[i % 2]
                hc_ref[h_rows(nxt + l * L, M), cols] = acc[i][0:M]
                xs_ref[segs(2 * j + l), cols] = acc[i][M:L]

        def step(c, carry):
            edge = (c == 0) | (c == last)

            @pl.when(edge)
            def _():
                single_block(c)

            @pl.when(jnp.logical_not(edge))
            def _():
                @pl.when(c == 1)
                def _():
                    x_rest.wait()
                    hc_ref[M:L, :] = _ln(x_ref[segs(4), :].astype(F32))
                    hc_ref[L + M:R2, :] = _ln(y_ref[segs(0), :])
                if cfg.get("unroll", 0):
                    a_step(c, 0)
                    a_step(c, 1)
                else:
                    jax.lax.fori_loop(0, 2, lambda j, z: (a_step(c, j), z)[1], 0)

                @pl.when(c >= 2)
                def _():
                    out_copy(2 * (c - 2), 2).start()

            r = ffn()
            t0 = 2 * (c - 1)
            s0 = jnp.where(c == 0, 0, n_seg - 4)
            dst = [jnp.where(edge, s0 + i, t0 + i // 2 + (4 if i % 2 == 0 else 0)) for i in range(4)]
            for i in (0, 2, 1, 3):
                for n in range(2):
                    y_ref[segs(dst[2 * (i // 2) + n]), halves[i % 2]] = r[i][n * seg:(n + 1) * seg]
            return carry
        jax.lax.fori_loop(0, NC, step, 0)

        out_ref[segs(n_seg - 4, 4), :] = y_ref[segs(n_seg - 4, 4), :].astype(out_ref.dtype)
        out_copy(n_seg - 4, 4).start()
        for c in range(NC - 2):
            out_copy(2 * c, 2).wait()
        out_copy(n_seg - 4, 4).wait()

    @functools.partial(jax.jit, static_argnames=("A_seg_len",))
    def run(A_x, A_mem0, A_Wq, A_Wk, A_Wv, A_Wo, A_seg_len, B_x, B_w_gate, B_w_up, B_w_down):
        B, S, Dm = A_x.shape
        H, Dh = A_Wq.shape[1:]
        M = A_mem0.shape[1]
        seg = A_seg_len
        DF = B_w_gate.shape[1]
        hbm = pl.BlockSpec(memory_space=pl.ANY)
        packed = lambda r, c: pltpu.VMEM((r // 2, c), U32)
        proj = pltpu.VMEM((7, Dm // 4, H * Dh // 2), U32)
        out = pl.pallas_call(
            functools.partial(kernel, M=M, seg=seg, H=H, Dh=Dh, n_seg=cfg.get("ns", S // seg)),
            in_specs=[hbm, pl.BlockSpec(memory_space=pltpu.VMEM), hbm, hbm, hbm, hbm, hbm, hbm, hbm],
            out_specs=hbm,
            out_shape=jax.ShapeDtypeStruct((S, Dm), A_x.dtype),
            scratch_shapes=[
                proj, proj, proj,
                packed(H * Dh, Dm), packed(Dm, DF), packed(Dm, DF), packed(DF, Dm),
                pltpu.VMEM((3, H * Dh // 4, Dm // 2), U32),
                pltpu.VMEM((3, Dm // 4, DF), U32),
                pltpu.VMEM((3, DF // 4, Dm // 2), U32),
                pltpu.VMEM((NS, 2, RC * H, Dh), BF16),
                pltpu.VMEM((4 * seg, Dm), F32),
                pltpu.VMEM((4 * (M + seg) + 2 * seg, Dm), F32),
                pltpu.VMEM((S, Dm), BF16),
                pltpu.VMEM((S, Dm), F32),
                pltpu.SemaphoreType.DMA((NS, 2)),
                pltpu.SemaphoreType.DMA((NO,)),
                pltpu.SemaphoreType.DMA((3,)),
                pltpu.SemaphoreType.DMA((2,)),
                pltpu.SemaphoreType.DMA(()),
            ],
            compiler_params=pltpu.CompilerParams(vmem_limit_bytes=126 * 1024 * 1024),
        )(A_x.reshape(S, Dm), A_mem0.reshape(M, Dm),
          A_Wq.reshape(Dm * H, Dh), A_Wk.reshape(Dm * H, Dh), A_Wv.reshape(Dm * H, Dh),
          A_Wo.reshape(H * Dh, Dm), B_w_gate, B_w_up, B_w_down)
        return out.reshape(B, S, Dm)
    return run


_run = build({})


@functools.partial(jax.jit, static_argnames=("A_seg_len",))
def pallas_interleave_layers__memory_aug_recurrent_mem_tr__glu_gated_geglu__prompt_kernel(
    A_x, A_mem0, A_Wq, A_Wk, A_Wv, A_Wo, A_seg_len, B_x, B_w_gate, B_w_up, B_w_down
):
    return _run(A_x, A_mem0, A_Wq, A_Wk, A_Wv, A_Wo, A_seg_len, B_x, B_w_gate, B_w_up, B_w_down)
```

```python
import functools
import jax
import jax.numpy as jnp
import numpy as np
import jax.experimental.pallas as pl
import jax.experimental.pallas.tpu as pltpu

F32 = jnp.float32
BF16 = jnp.bfloat16
U32 = jnp.uint32


def _ln(x):
    m = jnp.mean(x, axis=-1, keepdims=True)
    d = x - m
    v = jnp.mean(d * d, axis=-1, keepdims=True)
    return d * jax.lax.rsqrt(v + 1e-5)


def _gelu(x):
    c = 0.7978845608028654
    return 0.5 * x * (1.0 + jnp.tanh(c * (x + 0.044715 * (x * x * x))))


def _dot(a, b):
    return jnp.dot(a, b, preferred_element_type=F32)


def build(cfg):
    G = cfg.get("G", 2)
    FC = cfg.get("FC", 896)
    RC = cfg.get("RC", 64)
    NS = cfg.get("NS", 3)
    LAG = cfg.get("lag", 2)
    NO = 8

    def kernel(x_h, mem0_h, wq_h, wk_h, wv_h, wo_h, wg_h, wu_h, wd_h, o_h,
               wq_p, wk_p, wv_p, wo_p, wg_p, wu_p, wd_p, eo_p, eu_p, ed_p, stage_ref,
               xs_ref, hc_ref, x_ref, y_ref, mem0_ref,
               sem_s, sem_o, sem_f, sem_x, sem_out, *, M, seg, H, Dh, n_seg):
        wo_ref, wg_ref, wu_ref, wd_ref, eo_ref, eu_ref, ed_ref = (
            r.bitcast(BF16) for r in (wo_p, wg_p, wu_p, wd_p, eo_p, eu_p, ed_p))
        out_ref = x_ref
        Dm = xs_ref.shape[1]
        DF = wg_ref.shape[1]
        scale = Dh ** -0.5
        NG = H // G
        NF = DF // FC
        S2 = 2 * seg
        cs = lambda g: slice(g * G * Dh, (g + 1) * G * Dh)
        fs = lambda f: slice(f * FC, (f + 1) * FC)
        hsl = lambda i: slice(i * Dh, (i + 1) * Dh)

        def h_rows(r, n):
            return pl.ds(r if isinstance(r, int) else pl.multiple_of(r, M), n)

        def aligned(r, n):
            return pl.ds(r if isinstance(r, int) else pl.multiple_of(r, seg), n)

        D2 = Dm // 2
        NRC = D2 // RC
        assert NS <= NRC
        proj_w = ((wq_h, wq_p), (wk_h, wk_p), (wv_h, wv_p))
        OR = H * Dh // NO

        def raw_copies(w, r):
            slot = (w * NRC + r) % NS
            return [pltpu.make_async_copy(proj_w[w][0].at[pl.ds(pl.multiple_of((half * D2 + r * RC) * H, RC * H), RC * H), :],
                                          stage_ref.at[slot, half], sem_s.at[slot, half]) for half in range(2)]

        def wo_copy(i):
            return pltpu.make_async_copy(wo_h.at[pl.ds(i * OR, OR), :], wo_ref.at[pl.ds(i * OR, OR), :], sem_o.at[i])

        def ffn_copy(i):
            src, dst = ((wg_h, wg_ref), (wu_h, wu_ref), (wd_h, wd_ref))[i]
            return pltpu.make_async_copy(src, dst, sem_f.at[i])

        wo_copies = [wo_copy(i) for i in range(NO)]
        gate, up, down_copy = (ffn_copy(i) for i in range(3))

        def unpack(t):
            return [pltpu.unpack_elementwise(t, index=i, packed_dtype=BF16, unpacked_dtype=F32) for i in range(2)]

        def pack(lo, hi):
            return pltpu.pack_elementwise((lo, hi), packed_dtype=BF16).astype(U32)

        def strassen_rhs(b11, b12, b21, b22):
            return (b11 + b22, b11, b12 - b22, b21 - b11, b22, b11 + b12, b21 + b22)

        def relayout(w, r):
            dst = proj_w[w][1]
            u = [stage_ref.at[(w * NRC + r) % NS, half].bitcast(U32) for half in range(2)]
            HP = H // 2

            def body(b, carry):
                ub = [t.at[pl.ds(pl.multiple_of(b * (16 * HP), 16 * HP), 16 * HP), :] for t in u]
                rows = pl.ds(pl.multiple_of(r * (RC // 2) + b * 8, 8), 8)
                for j in range(HP):
                    res = []
                    for par in range(2):
                        top, bot = (unpack(t[pl.ds(par * HP + j, 8, stride=2 * HP), :]) for t in ub)
                        res.append(strassen_rhs(top[0], top[1], bot[0], bot[1]))
                    for n in range(7):
                        dst[n, rows, hsl(j)] = pack(res[0][n], res[1][n])
                return carry
            jax.lax.fori_loop(0, RC // 16, body, 0)

        def segs(t, n=1):
            return aligned(t * seg, n * seg)

        x_first = pltpu.make_async_copy(x_h.at[0:4 * seg, :], x_ref.at[0:4 * seg, :], sem_x.at[0])
        x_rest = pltpu.make_async_copy(x_h.at[4 * seg:n_seg * seg, :], x_ref.at[4 * seg:n_seg * seg, :], sem_x.at[1])

        mem_copy = pltpu.make_async_copy(mem0_h, mem0_ref, sem_x.at[2])

        def out_copy(t, n):
            return pltpu.make_async_copy(out_ref.at[segs(t, n), :], o_h.at[segs(t, n), :], sem_out)

        def strassen_lhs(a11, a12, a21, a22):
            return (a11 + a22, a21 + a22, a11, a22, a11 + a12, a21 - a11, a12 - a22)

        def strassen_out(m):
            return ((m[3] - m[4]) + m[0] + m[6], m[2] + m[4], m[1] + m[3], (m[2] - m[1]) + m[0] + m[5])

        def product(lhs, rhs):
            m = [None] * 7
            if len(lhs) == 7:
                for n in cfg.get("aord", (2, 3, 1, 4, 0, 5, 6)):
                    m[n] = _dot(lhs[n], rhs(n))
                return strassen_out(m)
            a11, a12 = lhs
            both = a11 + a12
            right = _dot(a11, rhs(2))
            left = _dot(a12, rhs(3))
            return left + _dot(both, rhs(1)), right + _dot(both, rhs(4))

        def operands(hs, lo, hi):
            quads = [t for h in hs for t in (h[:, lo], h[:, hi])]
            return strassen_lhs(*quads) if len(hs) == 2 else quads

        L = M + seg
        halves = (slice(0, D2), slice(D2, Dm))

        def attention(load_hs, order, G, WG, wait_wo=None, fill_in={}, residual=None):
            hs = load_hs()
            nl = len(hs)
            R = nl * L
            NG = H // G
            ri = jax.lax.broadcasted_iota(jnp.int32, (R, 128), 0)
            ci = jax.lax.broadcasted_iota(jnp.int32, (R, 128), 1)
            rl, cl = (ri >= L).astype(jnp.int32), (ci >= L).astype(jnp.int32)
            rp, cp = ri - rl * L, ci - cl * L
            same = (rl == cl) & (ci < R)
            keep = same & ((rp < M) | (rp >= cp))
            fill = jnp.where(same, -1e9, -jnp.inf).astype(F32)
            z = jnp.zeros((128 - R, Dh), F32)
            lhs = list(operands(hs, slice(0, D2), slice(D2, Dm)))

            def proj(w, g):
                c = product(lhs, lambda n: pltpu.bitcast(w[n, :, g * (G // 2) * Dh:(g + 1) * (G // 2) * Dh], BF16))
                return [jnp.concatenate([c[2 * l + i % 2][:, hsl(i // 2)] for l in range(nl)], axis=0) for i in range(G)]

            def as_rhs(t):
                return jnp.concatenate([t, z], axis=0).astype(BF16)

            def softmax(s):
                s = jnp.where(keep, s * scale, fill)
                e = jnp.exp(s - jnp.max(s, axis=-1, keepdims=True))
                p = e * pl.reciprocal(jnp.sum(e, axis=-1, keepdims=True), approx=False)
                return p.astype(BF16) if nl == 2 else p

            acc = []
            os = {}

            def wo(g):
                if g == 0 and wait_wo is not None:
                    wait_wo()
                if (g + 1) % WG and not (cfg.get("split", 1) and g == NG - 2):
                    return
                o = [t for i in sorted(os) if i <= g for t in os.pop(i)]
                n2 = len(o) // 2
                ol = operands([jnp.concatenate([t[l * L:(l + 1) * L] for t in o[0::2] + o[1::2]], axis=1) for l in range(nl)],
                              slice(0, n2 * Dh), slice(n2 * Dh, 2 * n2 * Dh))
                pairs = range((g + 1) * G // 2 - n2, (g + 1) * G // 2)

                def rhs(n):
                    if n in (0, 5, 6):
                        return eo_ref[{0: 0, 5: 1, 6: 2}[n], pairs[0] * Dh:(pairs[-1] + 1) * Dh, :]
                    odd, cols = {1: (0, slice(0, D2)), 2: (0, slice(D2, Dm)), 3: (1, slice(0, D2)), 4: (1, slice(D2, Dm))}[n]
                    parts = [wo_ref[(2 * p + odd) * Dh:(2 * p + odd + 1) * Dh, cols] for p in pairs]
                    return parts[0] if len(parts) == 1 else jnp.concatenate(parts, axis=0)
                if nl == 2 and g == NG - 1:
                    out = [t + r for t, r in zip(strassen_out(acc), residual())]
                    for n, plus, minus in ((0, (0, 3), ()), (3, (0, 2), ()), (4, (1,), (0,)), (1, (2,), (3,)),
                                           (2, (1, 3), ()), (5, (3,), ()), (6, (0,), ())):
                        t = _dot(ol[n], rhs(n))
                        for i in plus:
                            out[i] = out[i] + t
                        for i in minus:
                            out[i] = out[i] - t
                    acc[:] = out
                    return
                if nl == 2:
                    c = [_dot(ol[n], rhs(n)) for n in range(7)]
                else:
                    c = product(ol, rhs)
                acc[:] = list(c) if not acc else [x + y for x, y in zip(acc, c)]

            steps = [(w[0], int(w[1:])) for w in order.split()]
            q, k, v, sc = {}, {}, {}, {}
            for g in range(-max(o for _, o in steps), NG - min(o for _, o in steps)):
                if g in fill_in:
                    fill_in[g]()
                    if cfg.get('reload', 1):
                        lhs[2] = load_hs()[0][:, 0:D2]
                for op, off in steps:
                    i = g + off
                    if not 0 <= i < NG:
                        continue
                    if op == "q":
                        q[i] = proj(wq_p, i)
                    elif op == "k":
                        k[i] = [as_rhs(t) for t in proj(wk_p, i)]
                    elif op == "v":
                        v[i] = [as_rhs(t) for t in proj(wv_p, i)]
                    elif op == "s":
                        sc[i] = [jax.lax.dot_general(a, b, (((1,), (1,)), ((), ())), preferred_element_type=F32)
                                 for a, b in zip(q.pop(i), k.pop(i))]
                    elif op == "e":
                        sc[i] = [softmax(t) for t in sc[i]]
                    elif op == "p":
                        os[i] = [_dot(a, b) for a, b in zip(sc.pop(i), v.pop(i))]
                    elif op == "w":
                        wo(i)
            return acc

        R2 = 2 * L
        NC = (n_seg - 4) // 2 + 2
        last = NC - 1

        NP = NF // 2

        def strassen_rhs_prepare(b11, b12, b21, b22, e0, e1, e2):
            res = [strassen_rhs(*t) for t in zip(*(unpack(r[...]) for r in (b11, b12, b21, b22)))]
            for dst, n in ((e0, 0), (e1, 5), (e2, 6), (b12, 2), (b21, 3)):
                dst[...] = pack(res[0][n], res[1][n])

        def prepare_wo(i):
            ppc = OR // (2 * Dh)

            def body(b, carry):
                p, r = i * ppc + b // 4, (b % 4) * 16
                for n in range(2):
                    r0, r1, re = (pl.ds(pl.multiple_of(row * (Dh // 2) + r + 8 * n, 8), 8) for row in (2 * p, 2 * p + 1, p))
                    strassen_rhs_prepare(wo_p.at[r0, 0:D2], wo_p.at[r0, D2:Dm], wo_p.at[r1, 0:D2], wo_p.at[r1, D2:Dm],
                                         *(eo_p.at[n2, re, :] for n2 in range(3)))
                return carry
            jax.lax.fori_loop(0, ppc * 4, body, 0, unroll=4)

        def prepare_up():
            def body(b, carry):
                r = pl.multiple_of(b * 8, 8)
                top, bot = pl.ds(r, 8), pl.ds(pl.multiple_of(D2 // 2 + r, 8), 8)
                for k in range(0, DF, 512):
                    c = slice(k, k + 512)
                    strassen_rhs_prepare(wg_p.at[top, c], wu_p.at[top, c], wg_p.at[bot, c], wu_p.at[bot, c],
                                         *(eu_p.at[i, top, c] for i in range(3)))
                return carry
            jax.lax.fori_loop(0, D2 // 16, body, 0, unroll=cfg.get('pu', 2))

        def prepare_down():
            F2 = FC // 2
            nb = F2 // 56

            def body(b, carry):
                p, r = b // nb, (b % nb) * 56
                for i in range(7):
                    r0 = pl.ds(pl.multiple_of(2 * p * F2 + r + 8 * i, 8), 8)
                    r1 = pl.ds(pl.multiple_of((2 * p + 1) * F2 + r + 8 * i, 8), 8)
                    re = pl.ds(pl.multiple_of(p * F2 + r + 8 * i, 8), 8)
                    strassen_rhs_prepare(wd_p.at[r0, 0:D2], wd_p.at[r0, D2:Dm], wd_p.at[r1, 0:D2], wd_p.at[r1, D2:Dm],
                                         *(ed_p.at[i2, re, :] for i2 in range(3)))
                return carry
            jax.lax.fori_loop(0, NP * nb, body, 0, unroll=cfg.get('pu', 2))

        def ffn():
            ha = hc_ref[2 * R2:2 * R2 + S2, :]
            hb = _ln(xs_ref[S2:2 * S2, :])
            lhs = [t.astype(BF16) for t in operands((ha, hb), slice(0, D2), slice(D2, Dm))]

            def hidden(f):
                rhs = (eu_ref[0, :, fs(f)], wg_ref[0:D2, fs(f)], wu_ref[0:D2, fs(f)], wg_ref[D2:Dm, fs(f)],
                       wu_ref[D2:Dm, fs(f)], eu_ref[1, :, fs(f)], eu_ref[2, :, fs(f)])
                m = [None] * 7
                for i in cfg.get("mord", (2, 3, 1, 4, 0, 5, 6)):
                    m[i] = _dot(lhs[i], rhs[i])
                ga, ua, gb, ub = strassen_out(m)
                return _gelu(ga) * ua, _gelu(gb) * ub

            acc = [xs_ref[0:S2, 0:D2], xs_ref[0:S2, D2:Dm], xs_ref[S2:2 * S2, 0:D2], xs_ref[S2:2 * S2, D2:Dm]]

            def down(p, h0, h1):
                f0, f1 = fs(2 * p), fs(2 * p + 1)
                dl = [t.astype(BF16) for t in strassen_lhs(h0[0], h1[0], h0[1], h1[1])]
                rhs = (ed_ref[0, fs(p), :], wd_ref[f0, 0:D2], wd_ref[f0, D2:Dm], wd_ref[f1, 0:D2],
                       wd_ref[f1, D2:Dm], ed_ref[1, fs(p), :], ed_ref[2, fs(p), :])
                m = [None] * 7
                for i in cfg.get("dord", (0, 1, 3, 4, 6, 2, 5)):
                    m[i] = _dot(dl[i], rhs[i])
                acc[0] = acc[0] + m[0] + m[3] - m[4] + m[6]
                acc[1] = acc[1] + m[4] + m[2]
                acc[2] = acc[2] + m[1] + m[3]
                acc[3] = acc[3] + m[0] - m[1] + m[2] + m[5]

            dlag = cfg.get("dlag", 1)
            hs = []
            for f in range(NF + dlag):
                if f < NF:
                    hs.append(hidden(f))
                e = f - dlag
                if e >= 0 and e % 2 == 1:
                    down(e // 2, hs[e - 1], hs[e])
            return acc

        for r in range(NS):
            for cp in raw_copies(0, r):
                cp.start()
        x_first.start()
        mem_copy.start()
        for w in range(3):
            def load(r, carry):
                for cp in raw_copies(w, r):
                    cp.wait()
                relayout(w, r)

                @pl.when(r + NS < NRC)
                def _():
                    for cp in raw_copies(w, r + NS):
                        cp.start()

                @pl.when(r + NS >= NRC)
                def _():
                    if w < 2:
                        for cp in raw_copies(w + 1, r + NS - NRC):
                            cp.start()
                    else:
                        i = r + NS - NRC
                        pltpu.make_async_copy(wo_h.at[pl.ds(pl.multiple_of(i * OR, OR), OR), :],
                                              wo_ref.at[pl.ds(pl.multiple_of(i * OR, OR), OR), :], sem_o.at[i]).start()
                return carry
            jax.lax.fori_loop(0, NRC, load, 0)
        for i in range(NS, NO):
            wo_copies[i].start()
        x_first.wait()
        mem_copy.wait()

        def single_block(c):
            @pl.when(c == 0)
            def _():
                hc_ref[0:M, :] = mem0_ref[...].astype(F32)
                y_ref[0:4 * seg, :] = x_ref[0:4 * seg, :].astype(F32)

            @pl.when(c == last)
            def _():
                hc_ref[0:M, :] = hc_ref[L:L + M, :]
                out_ref[segs(n_seg - 6, 2), :] = y_ref[segs(n_seg - 6, 2), :].astype(out_ref.dtype)
                out_copy(n_seg - 6, 2).start()

            s0 = jnp.where(c == 0, 0, n_seg - 4)
            hc_ref[R2:R2 + 4 * seg, :] = _ln(y_ref[segs(s0, 4), :])

            def single(j, carry):
                def wait_wo():
                    @pl.when(c == 0)
                    def _():
                        @pl.when(j == 0)
                        def _():
                            for i in range(NO):
                                wo_copies[i].wait()
                                if i == 0:
                                    gate.start()
                                    up.start()
                                prepare_wo(i)

                        @pl.when(j == cfg.get('dj', 2))
                        def _():
                            down_copy.start()
                h = jnp.concatenate([hc_ref[0:M, :], hc_ref[h_rows(R2 + j * seg, seg), :]], axis=0)
                acc = jnp.concatenate(attention(lambda: [h], cfg.get('sorder', 's0 q1 k1 v1 e0 p0') + ' w-%d' % (2 * H), cfg.get('sG', 4), cfg.get('sWG', 2), wait_wo), axis=1)
                hc_ref[0:M, :] = acc[0:M]
                xs_ref[segs(j), :] = y_ref[segs(s0 + j), :] + acc[M:L]
                return carry
            jax.lax.fori_loop(0, 4, single, 0)
            hc_ref[2 * R2:2 * R2 + S2, :] = _ln(xs_ref[0:S2, :])

            @pl.when(c == 0)
            def _():
                hc_ref[L:L + M, :] = mem0_ref[...].astype(F32)
                gate.wait()
                up.wait()
                prepare_up()
                down_copy.wait()
                x_rest.start()
                prepare_down()

        def a_step(c, j):
            t = 2 * (c - 1) + j
            cur = j * R2
            nxt = (1 - j) * R2

            def fill_x():
                hc_ref[h_rows(nxt + M, seg), :] = _ln(x_ref[segs(jnp.minimum(t + 5, n_seg - 1)), :].astype(F32))

            def fill_y():
                hc_ref[h_rows(nxt + L + M, seg), :] = _ln(y_ref[segs(t + 1), :])

            def fill_b():
                hc_ref[2 * R2:2 * R2 + S2, :] = _ln(xs_ref[0:S2, :])

            def fill_o():
                done = jnp.maximum(t - 2, 0)
                out_ref[segs(done), :] = y_ref[segs(done), :].astype(out_ref.dtype)
            f0, f1 = cfg.get("f0", 1), cfg.get("f1", 1)

            def residual():
                zero = jnp.zeros((M, Dm), F32)
                rows = [jnp.concatenate([zero, r], axis=0) for r in (x_ref[segs(t + 4), :].astype(F32), y_ref[segs(t), :])]
                return [r[:, cols] for r in rows for cols in halves]
            acc = attention(lambda: [hc_ref[h_rows(cur + l * L, L), :] for l in range(2)],
                            cfg.get('order', 's0 q1 k1 v1 w-2 e0 p0'), G, cfg.get('WG', 2),
                            fill_in={f0: fill_o, f0 + f1: fill_x, f0 + 2 * f1: fill_y, f0 + 3 * f1: fill_b},
                            residual=residual)
            for i in (2, 1, 3, 0):
                l, cols = i // 2, halves[i % 2]
                hc_ref[h_rows(nxt + l * L, M), cols] = acc[i][0:M]
                xs_ref[segs(2 * j + l), cols] = acc[i][M:L]

        def step(c, carry):
            edge = (c == 0) | (c == last)

            @pl.when(edge)
            def _():
                single_block(c)

            @pl.when(jnp.logical_not(edge))
            def _():
                @pl.when(c == 1)
                def _():
                    x_rest.wait()
                    hc_ref[M:L, :] = _ln(x_ref[segs(4), :].astype(F32))
                    hc_ref[L + M:R2, :] = _ln(y_ref[segs(0), :])
                if cfg.get("unroll", 0):
                    a_step(c, 0)
                    a_step(c, 1)
                else:
                    jax.lax.fori_loop(0, 2, lambda j, z: (a_step(c, j), z)[1], 0)

                @pl.when(c >= 2)
                def _():
                    out_copy(2 * (c - 2), 2).start()

            r = ffn()
            t0 = 2 * (c - 1)
            s0 = jnp.where(c == 0, 0, n_seg - 4)
            dst = [jnp.where(edge, s0 + i, t0 + i // 2 + (4 if i % 2 == 0 else 0)) for i in range(4)]
            for i in (0, 2, 1, 3):
                for n in range(2):
                    y_ref[segs(dst[2 * (i // 2) + n]), halves[i % 2]] = r[i][n * seg:(n + 1) * seg]
            return carry
        jax.lax.fori_loop(0, NC, step, 0)

        out_ref[segs(n_seg - 4, 4), :] = y_ref[segs(n_seg - 4, 4), :].astype(out_ref.dtype)
        out_copy(n_seg - 4, 4).start()
        for c in range(NC - 2):
            out_copy(2 * c, 2).wait()
        out_copy(n_seg - 4, 4).wait()

    @functools.partial(jax.jit, static_argnames=("A_seg_len",))
    def run(A_x, A_mem0, A_Wq, A_Wk, A_Wv, A_Wo, A_seg_len, B_x, B_w_gate, B_w_up, B_w_down):
        B, S, Dm = A_x.shape
        H, Dh = A_Wq.shape[1:]
        M = A_mem0.shape[1]
        seg = A_seg_len
        DF = B_w_gate.shape[1]
        hbm = pl.BlockSpec(memory_space=pl.ANY)
        packed = lambda r, c: pltpu.VMEM((r // 2, c), U32)
        proj = pltpu.VMEM((7, Dm // 4, H * Dh // 2), U32)
        out = pl.pallas_call(
            functools.partial(kernel, M=M, seg=seg, H=H, Dh=Dh, n_seg=cfg.get("ns", S // seg)),
            in_specs=[hbm] * 9,
            out_specs=hbm,
            out_shape=jax.ShapeDtypeStruct((S, Dm), A_x.dtype),
            scratch_shapes=[
                proj, proj, proj,
                packed(H * Dh, Dm), packed(Dm, DF), packed(Dm, DF), packed(DF, Dm),
                pltpu.VMEM((3, H * Dh // 4, Dm // 2), U32),
                pltpu.VMEM((3, Dm // 4, DF), U32),
                pltpu.VMEM((3, DF // 4, Dm // 2), U32),
                pltpu.VMEM((NS, 2, RC * H, Dh), BF16),
                pltpu.VMEM((4 * seg, Dm), F32),
                pltpu.VMEM((4 * (M + seg) + 2 * seg, Dm), F32),
                pltpu.VMEM((S, Dm), BF16),
                pltpu.VMEM((S, Dm), F32),
                pltpu.VMEM((M, Dm), BF16),
                pltpu.SemaphoreType.DMA((NS, 2)),
                pltpu.SemaphoreType.DMA((NO,)),
                pltpu.SemaphoreType.DMA((3,)),
                pltpu.SemaphoreType.DMA((3,)),
                pltpu.SemaphoreType.DMA(()),
            ],
            compiler_params=pltpu.CompilerParams(vmem_limit_bytes=126 * 1024 * 1024, flags={k: True for k in cfg.get("flags", ())} or None),
        )(A_x.reshape(S, Dm), A_mem0.reshape(M, Dm),
          A_Wq.reshape(Dm * H, Dh), A_Wk.reshape(Dm * H, Dh), A_Wv.reshape(Dm * H, Dh),
          A_Wo.reshape(H * Dh, Dm), B_w_gate, B_w_up, B_w_down)
        return out.reshape(B, S, Dm)
    return run


_run = build({})


@functools.partial(jax.jit, static_argnames=("A_seg_len",))
def pallas_interleave_layers__memory_aug_recurrent_mem_tr__glu_gated_geglu__prompt_kernel(
    A_x, A_mem0, A_Wq, A_Wk, A_Wv, A_Wo, A_seg_len, B_x, B_w_gate, B_w_up, B_w_down
):
    return _run(A_x, A_mem0, A_Wq, A_Wk, A_Wv, A_Wo, A_seg_len, B_x, B_w_gate, B_w_up, B_w_down)
```

```python
import functools
import jax
import jax.numpy as jnp
import numpy as np
import jax.experimental.pallas as pl
import jax.experimental.pallas.tpu as pltpu

F32 = jnp.float32
BF16 = jnp.bfloat16
U32 = jnp.uint32


def _ln(x):
    m = jnp.mean(x, axis=-1, keepdims=True)
    d = x - m
    v = jnp.mean(d * d, axis=-1, keepdims=True)
    return d * jax.lax.rsqrt(v + 1e-5)


def _gelu(x):
    c = 0.7978845608028654
    return 0.5 * x * (1.0 + jnp.tanh(c * (x + 0.044715 * (x * x * x))))


def _dot(a, b):
    return jnp.dot(a, b, preferred_element_type=F32)


NO = 8
NS = 3
RC = 64
FC = 896


def _build():
    def kernel(x_h, mem0_h, wq_h, wk_h, wv_h, wo_h, wg_h, wu_h, wd_h, o_h,
               wq_p, wk_p, wv_p, wo_p, wg_p, wu_p, wd_p, eo_p, eu_p, ed_p, stage_ref,
               xs_ref, hc_ref, x_ref, y_ref, mem0_ref,
               sem_s, sem_o, sem_f, sem_x, sem_out, *, M, seg, H, Dh, n_seg):
        wo_ref, wg_ref, wu_ref, wd_ref, eo_ref, eu_ref, ed_ref = (
            r.bitcast(BF16) for r in (wo_p, wg_p, wu_p, wd_p, eo_p, eu_p, ed_p))
        out_ref = x_ref
        Dm = xs_ref.shape[1]
        DF = wg_ref.shape[1]
        scale = Dh ** -0.5
        NF = DF // FC
        S2 = 2 * seg
        fs = lambda f: slice(f * FC, (f + 1) * FC)
        hsl = lambda i: slice(i * Dh, (i + 1) * Dh)

        def h_rows(r, n):
            return pl.ds(r if isinstance(r, int) else pl.multiple_of(r, M), n)

        def aligned(r, n):
            return pl.ds(r if isinstance(r, int) else pl.multiple_of(r, seg), n)

        D2 = Dm // 2
        NRC = D2 // RC
        assert NS <= NRC
        proj_w = ((wq_h, wq_p), (wk_h, wk_p), (wv_h, wv_p))
        OR = H * Dh // NO

        def raw_copies(w, r):
            slot = (w * NRC + r) % NS
            return [pltpu.make_async_copy(proj_w[w][0].at[pl.ds(pl.multiple_of((half * D2 + r * RC) * H, RC * H), RC * H), :],
                                          stage_ref.at[slot, half], sem_s.at[slot, half]) for half in range(2)]

        def wo_copy(i):
            return pltpu.make_async_copy(wo_h.at[pl.ds(i * OR, OR), :], wo_ref.at[pl.ds(i * OR, OR), :], sem_o.at[i])

        def ffn_copy(i):
            src, dst = ((wg_h, wg_ref), (wu_h, wu_ref), (wd_h, wd_ref))[i]
            return pltpu.make_async_copy(src, dst, sem_f.at[i])

        wo_copies = [wo_copy(i) for i in range(NO)]
        gate, up, down_copy = (ffn_copy(i) for i in range(3))

        def unpack(t):
            return [pltpu.unpack_elementwise(t, index=i, packed_dtype=BF16, unpacked_dtype=F32) for i in range(2)]

        def pack(lo, hi):
            return pltpu.pack_elementwise((lo, hi), packed_dtype=BF16).astype(U32)

        def strassen_rhs(b11, b12, b21, b22):
            return (b11 + b22, b11, b12 - b22, b21 - b11, b22, b11 + b12, b21 + b22)

        def relayout(w, r):
            dst = proj_w[w][1]
            u = [stage_ref.at[(w * NRC + r) % NS, half].bitcast(U32) for half in range(2)]
            HP = H // 2

            def body(b, carry):
                ub = [t.at[pl.ds(pl.multiple_of(b * (16 * HP), 16 * HP), 16 * HP), :] for t in u]
                rows = pl.ds(pl.multiple_of(r * (RC // 2) + b * 8, 8), 8)
                for j in range(HP):
                    res = []
                    for par in range(2):
                        top, bot = (unpack(t[pl.ds(par * HP + j, 8, stride=2 * HP), :]) for t in ub)
                        res.append(strassen_rhs(top[0], top[1], bot[0], bot[1]))
                    for n in range(7):
                        dst[n, rows, hsl(j)] = pack(res[0][n], res[1][n])
                return carry
            jax.lax.fori_loop(0, RC // 16, body, 0)

        def segs(t, n=1):
            return aligned(t * seg, n * seg)

        x_first = pltpu.make_async_copy(x_h.at[0:4 * seg, :], x_ref.at[0:4 * seg, :], sem_x.at[0])
        x_rest = pltpu.make_async_copy(x_h.at[4 * seg:n_seg * seg, :], x_ref.at[4 * seg:n_seg * seg, :], sem_x.at[1])

        mem_copy = pltpu.make_async_copy(mem0_h, mem0_ref, sem_x.at[2])

        def out_copy(t, n):
            return pltpu.make_async_copy(out_ref.at[segs(t, n), :], o_h.at[segs(t, n), :], sem_out)

        def strassen_lhs(a11, a12, a21, a22):
            return (a11 + a22, a21 + a22, a11, a22, a11 + a12, a21 - a11, a12 - a22)

        def strassen_out(m):
            return ((m[3] - m[4]) + m[0] + m[6], m[2] + m[4], m[1] + m[3], (m[2] - m[1]) + m[0] + m[5])

        def product(lhs, rhs):
            m = [None] * 7
            if len(lhs) == 7:
                for n in (2, 3, 1, 4, 0, 5, 6):
                    m[n] = _dot(lhs[n], rhs(n))
                return strassen_out(m)
            a11, a12 = lhs
            both = a11 + a12
            right = _dot(a11, rhs(2))
            left = _dot(a12, rhs(3))
            return left + _dot(both, rhs(1)), right + _dot(both, rhs(4))

        def operands(hs, lo, hi):
            quads = [t for h in hs for t in (h[:, lo], h[:, hi])]
            return strassen_lhs(*quads) if len(hs) == 2 else quads

        L = M + seg
        halves = (slice(0, D2), slice(D2, Dm))

        def attention(load_hs, order, G, WG, wait_wo=None, fill_in={}, residual=None):
            hs = load_hs()
            nl = len(hs)
            R = nl * L
            NG = H // G
            ri = jax.lax.broadcasted_iota(jnp.int32, (R, 128), 0)
            ci = jax.lax.broadcasted_iota(jnp.int32, (R, 128), 1)
            rl, cl = (ri >= L).astype(jnp.int32), (ci >= L).astype(jnp.int32)
            rp, cp = ri - rl * L, ci - cl * L
            same = (rl == cl) & (ci < R)
            keep = same & ((rp < M) | (rp >= cp))
            fill = jnp.where(same, -1e9, -jnp.inf).astype(F32)
            z = jnp.zeros((128 - R, Dh), F32)
            lhs = list(operands(hs, slice(0, D2), slice(D2, Dm)))

            def proj(w, g):
                c = product(lhs, lambda n: pltpu.bitcast(w[n, :, g * (G // 2) * Dh:(g + 1) * (G // 2) * Dh], BF16))
                return [jnp.concatenate([c[2 * l + i % 2][:, hsl(i // 2)] for l in range(nl)], axis=0) for i in range(G)]

            def as_rhs(t):
                return jnp.concatenate([t, z], axis=0).astype(BF16)

            def softmax(s):
                s = jnp.where(keep, s * scale, fill)
                e = jnp.exp(s - jnp.max(s, axis=-1, keepdims=True))
                p = e * pl.reciprocal(jnp.sum(e, axis=-1, keepdims=True), approx=False)
                return p.astype(BF16) if nl == 2 else p

            acc = []
            os = {}

            def wo(g):
                if g == 0 and wait_wo is not None:
                    wait_wo()
                if (g + 1) % WG and g != NG - 2:
                    return
                o = [t for i in sorted(os) if i <= g for t in os.pop(i)]
                n2 = len(o) // 2
                ol = operands([jnp.concatenate([t[l * L:(l + 1) * L] for t in o[0::2] + o[1::2]], axis=1) for l in range(nl)],
                              slice(0, n2 * Dh), slice(n2 * Dh, 2 * n2 * Dh))
                pairs = range((g + 1) * G // 2 - n2, (g + 1) * G // 2)

                def rhs(n):
                    if n in (0, 5, 6):
                        return eo_ref[{0: 0, 5: 1, 6: 2}[n], pairs[0] * Dh:(pairs[-1] + 1) * Dh, :]
                    odd, cols = {1: (0, slice(0, D2)), 2: (0, slice(D2, Dm)), 3: (1, slice(0, D2)), 4: (1, slice(D2, Dm))}[n]
                    parts = [wo_ref[(2 * p + odd) * Dh:(2 * p + odd + 1) * Dh, cols] for p in pairs]
                    return parts[0] if len(parts) == 1 else jnp.concatenate(parts, axis=0)
                if nl == 2 and g == NG - 1:
                    out = [t + r for t, r in zip(strassen_out(acc), residual())]
                    for n, plus, minus in ((0, (0, 3), ()), (3, (0, 2), ()), (4, (1,), (0,)), (1, (2,), (3,)),
                                           (2, (1, 3), ()), (5, (3,), ()), (6, (0,), ())):
                        t = _dot(ol[n], rhs(n))
                        for i in plus:
                            out[i] = out[i] + t
                        for i in minus:
                            out[i] = out[i] - t
                    acc[:] = out
                    return
                if nl == 2:
                    c = [_dot(ol[n], rhs(n)) for n in range(7)]
                else:
                    c = product(ol, rhs)
                acc[:] = list(c) if not acc else [x + y for x, y in zip(acc, c)]

            steps = [(w[0], int(w[1:])) for w in order.split()]
            q, k, v, sc = {}, {}, {}, {}
            for g in range(-max(o for _, o in steps), NG - min(o for _, o in steps)):
                if g in fill_in:
                    fill_in[g]()
                    lhs[2] = load_hs()[0][:, 0:D2]
                for op, off in steps:
                    i = g + off
                    if not 0 <= i < NG:
                        continue
                    if op == "q":
                        q[i] = proj(wq_p, i)
                    elif op == "k":
                        k[i] = [as_rhs(t) for t in proj(wk_p, i)]
                    elif op == "v":
                        v[i] = [as_rhs(t) for t in proj(wv_p, i)]
                    elif op == "s":
                        sc[i] = [jax.lax.dot_general(a, b, (((1,), (1,)), ((), ())), preferred_element_type=F32)
                                 for a, b in zip(q.pop(i), k.pop(i))]
                    elif op == "e":
                        sc[i] = [softmax(t) for t in sc[i]]
                    elif op == "p":
                        os[i] = [_dot(a, b) for a, b in zip(sc.pop(i), v.pop(i))]
                    elif op == "w":
                        wo(i)
            return acc

        R2 = 2 * L
        NC = (n_seg - 4) // 2 + 2
        last = NC - 1

        NP = NF // 2

        def strassen_rhs_prepare(b11, b12, b21, b22, e0, e1, e2):
            res = [strassen_rhs(*t) for t in zip(*(unpack(r[...]) for r in (b11, b12, b21, b22)))]
            for dst, n in ((e0, 0), (e1, 5), (e2, 6), (b12, 2), (b21, 3)):
                dst[...] = pack(res[0][n], res[1][n])

        def prepare_wo(i):
            ppc = OR // (2 * Dh)

            def body(b, carry):
                p, r = i * ppc + b // 4, (b % 4) * 16
                for n in range(2):
                    r0, r1, re = (pl.ds(pl.multiple_of(row * (Dh // 2) + r + 8 * n, 8), 8) for row in (2 * p, 2 * p + 1, p))
                    strassen_rhs_prepare(wo_p.at[r0, 0:D2], wo_p.at[r0, D2:Dm], wo_p.at[r1, 0:D2], wo_p.at[r1, D2:Dm],
                                         *(eo_p.at[n2, re, :] for n2 in range(3)))
                return carry
            jax.lax.fori_loop(0, ppc * 4, body, 0, unroll=4)

        def prepare_up():
            def body(b, carry):
                r = pl.multiple_of(b * 8, 8)
                top, bot = pl.ds(r, 8), pl.ds(pl.multiple_of(D2 // 2 + r, 8), 8)
                for k in range(0, DF, 512):
                    c = slice(k, k + 512)
                    strassen_rhs_prepare(wg_p.at[top, c], wu_p.at[top, c], wg_p.at[bot, c], wu_p.at[bot, c],
                                         *(eu_p.at[i, top, c] for i in range(3)))
                return carry
            jax.lax.fori_loop(0, D2 // 16, body, 0, unroll=2)

        def prepare_down():
            F2 = FC // 2
            nb = F2 // 56

            def body(b, carry):
                p, r = b // nb, (b % nb) * 56
                for i in range(7):
                    r0 = pl.ds(pl.multiple_of(2 * p * F2 + r + 8 * i, 8), 8)
                    r1 = pl.ds(pl.multiple_of((2 * p + 1) * F2 + r + 8 * i, 8), 8)
                    re = pl.ds(pl.multiple_of(p * F2 + r + 8 * i, 8), 8)
                    strassen_rhs_prepare(wd_p.at[r0, 0:D2], wd_p.at[r0, D2:Dm], wd_p.at[r1, 0:D2], wd_p.at[r1, D2:Dm],
                                         *(ed_p.at[i2, re, :] for i2 in range(3)))
                return carry
            jax.lax.fori_loop(0, NP * nb, body, 0, unroll=2)

        def ffn():
            ha = hc_ref[2 * R2:2 * R2 + S2, :]
            hb = _ln(xs_ref[S2:2 * S2, :])
            lhs = [t.astype(BF16) for t in operands((ha, hb), slice(0, D2), slice(D2, Dm))]

            def hidden(f):
                rhs = (eu_ref[0, :, fs(f)], wg_ref[0:D2, fs(f)], wu_ref[0:D2, fs(f)], wg_ref[D2:Dm, fs(f)],
                       wu_ref[D2:Dm, fs(f)], eu_ref[1, :, fs(f)], eu_ref[2, :, fs(f)])
                m = [None] * 7
                for i in (2, 3, 1, 4, 0, 5, 6):
                    m[i] = _dot(lhs[i], rhs[i])
                ga, ua, gb, ub = strassen_out(m)
                return _gelu(ga) * ua, _gelu(gb) * ub

            acc = [xs_ref[0:S2, 0:D2], xs_ref[0:S2, D2:Dm], xs_ref[S2:2 * S2, 0:D2], xs_ref[S2:2 * S2, D2:Dm]]

            def down(p, h0, h1):
                f0, f1 = fs(2 * p), fs(2 * p + 1)
                dl = [t.astype(BF16) for t in strassen_lhs(h0[0], h1[0], h0[1], h1[1])]
                rhs = (ed_ref[0, fs(p), :], wd_ref[f0, 0:D2], wd_ref[f0, D2:Dm], wd_ref[f1, 0:D2],
                       wd_ref[f1, D2:Dm], ed_ref[1, fs(p), :], ed_ref[2, fs(p), :])
                m = [None] * 7
                for i in (0, 1, 3, 4, 6, 2, 5):
                    m[i] = _dot(dl[i], rhs[i])
                acc[0] = acc[0] + m[0] + m[3] - m[4] + m[6]
                acc[1] = acc[1] + m[4] + m[2]
                acc[2] = acc[2] + m[1] + m[3]
                acc[3] = acc[3] + m[0] - m[1] + m[2] + m[5]

            dlag = 1
            hs = []
            for f in range(NF + dlag):
                if f < NF:
                    hs.append(hidden(f))
                e = f - dlag
                if e >= 0 and e % 2 == 1:
                    down(e // 2, hs[e - 1], hs[e])
            return acc

        for r in range(NS):
            for cp in raw_copies(0, r):
                cp.start()
        x_first.start()
        mem_copy.start()
        for w in range(3):
            def load(r, carry):
                for cp in raw_copies(w, r):
                    cp.wait()
                relayout(w, r)

                @pl.when(r + NS < NRC)
                def _():
                    for cp in raw_copies(w, r + NS):
                        cp.start()

                @pl.when(r + NS >= NRC)
                def _():
                    if w < 2:
                        for cp in raw_copies(w + 1, r + NS - NRC):
                            cp.start()
                    else:
                        i = r + NS - NRC
                        pltpu.make_async_copy(wo_h.at[pl.ds(pl.multiple_of(i * OR, OR), OR), :],
                                              wo_ref.at[pl.ds(pl.multiple_of(i * OR, OR), OR), :], sem_o.at[i]).start()
                return carry
            jax.lax.fori_loop(0, NRC, load, 0)
        for i in range(NS, NO):
            wo_copies[i].start()
        x_first.wait()
        mem_copy.wait()

        def single_block(c):
            @pl.when(c == 0)
            def _():
                hc_ref[0:M, :] = mem0_ref[...].astype(F32)
                y_ref[0:4 * seg, :] = x_ref[0:4 * seg, :].astype(F32)

            @pl.when(c == last)
            def _():
                hc_ref[0:M, :] = hc_ref[L:L + M, :]
                out_ref[segs(n_seg - 6, 2), :] = y_ref[segs(n_seg - 6, 2), :].astype(out_ref.dtype)
                out_copy(n_seg - 6, 2).start()

            s0 = jnp.where(c == 0, 0, n_seg - 4)
            hc_ref[R2:R2 + 4 * seg, :] = _ln(y_ref[segs(s0, 4), :])

            def single(j, carry):
                def wait_wo():
                    @pl.when(c == 0)
                    def _():
                        @pl.when(j == 0)
                        def _():
                            for i in range(NO):
                                wo_copies[i].wait()
                                if i == 0:
                                    gate.start()
                                    up.start()
                                prepare_wo(i)

                        @pl.when(j == 2)
                        def _():
                            down_copy.start()
                h = jnp.concatenate([hc_ref[0:M, :], hc_ref[h_rows(R2 + j * seg, seg), :]], axis=0)
                acc = jnp.concatenate(attention(lambda: [h], 's0 q1 k1 v1 e0 p0 w-%d' % H, 4, 2, wait_wo), axis=1)
                hc_ref[0:M, :] = acc[0:M]
                xs_ref[segs(j), :] = y_ref[segs(s0 + j), :] + acc[M:L]
                return carry
            jax.lax.fori_loop(0, 4, single, 0)
            hc_ref[2 * R2:2 * R2 + S2, :] = _ln(xs_ref[0:S2, :])

            @pl.when(c == 0)
            def _():
                hc_ref[L:L + M, :] = mem0_ref[...].astype(F32)
                gate.wait()
                up.wait()
                prepare_up()
                down_copy.wait()
                x_rest.start()
                prepare_down()

        def a_step(c, j):
            t = 2 * (c - 1) + j
            cur = j * R2
            nxt = (1 - j) * R2

            def fill_x():
                hc_ref[h_rows(nxt + M, seg), :] = _ln(x_ref[segs(jnp.minimum(t + 5, n_seg - 1)), :].astype(F32))

            def fill_y():
                hc_ref[h_rows(nxt + L + M, seg), :] = _ln(y_ref[segs(t + 1), :])

            def fill_b():
                hc_ref[2 * R2:2 * R2 + S2, :] = _ln(xs_ref[0:S2, :])

            def fill_o():
                done = jnp.maximum(t - 2, 0)
                out_ref[segs(done), :] = y_ref[segs(done), :].astype(out_ref.dtype)

            def residual():
                zero = jnp.zeros((M, Dm), F32)
                rows = [jnp.concatenate([zero, r], axis=0) for r in (x_ref[segs(t + 4), :].astype(F32), y_ref[segs(t), :])]
                return [r[:, cols] for r in rows for cols in halves]
            acc = attention(lambda: [hc_ref[h_rows(cur + l * L, L), :] for l in range(2)],
                            's0 q1 k1 v1 w-2 e0 p0', 2, 2,
                            fill_in={1: fill_o, 2: fill_x, 3: fill_y, 4: fill_b},
                            residual=residual)
            for i in (2, 1, 3, 0):
                l, cols = i // 2, halves[i % 2]
                hc_ref[h_rows(nxt + l * L, M), cols] = acc[i][0:M]
                xs_ref[segs(2 * j + l), cols] = acc[i][M:L]

        def step(c, carry):
            edge = (c == 0) | (c == last)

            @pl.when(edge)
            def _():
                single_block(c)

            @pl.when(jnp.logical_not(edge))
            def _():
                @pl.when(c == 1)
                def _():
                    x_rest.wait()
                    hc_ref[M:L, :] = _ln(x_ref[segs(4), :].astype(F32))
                    hc_ref[L + M:R2, :] = _ln(y_ref[segs(0), :])

                def both(j, inner):
                    a_step(c, j)
                    return inner
                jax.lax.fori_loop(0, 2, both, 0)

                @pl.when(c >= 2)
                def _():
                    out_copy(2 * (c - 2), 2).start()

            r = ffn()
            t0 = 2 * (c - 1)
            s0 = jnp.where(c == 0, 0, n_seg - 4)
            dst = [jnp.where(edge, s0 + i, t0 + i // 2 + (4 if i % 2 == 0 else 0)) for i in range(4)]
            for i in (0, 2, 1, 3):
                for n in range(2):
                    y_ref[segs(dst[2 * (i // 2) + n]), halves[i % 2]] = r[i][n * seg:(n + 1) * seg]
            return carry
        jax.lax.fori_loop(0, NC, step, 0)

        out_ref[segs(n_seg - 4, 4), :] = y_ref[segs(n_seg - 4, 4), :].astype(out_ref.dtype)
        out_copy(n_seg - 4, 4).start()
        for c in range(NC - 2):
            out_copy(2 * c, 2).wait()
        out_copy(n_seg - 4, 4).wait()

    def run(A_x, A_mem0, A_Wq, A_Wk, A_Wv, A_Wo, A_seg_len, B_x, B_w_gate, B_w_up, B_w_down):
        B, S, Dm = A_x.shape
        H, Dh = A_Wq.shape[1:]
        M = A_mem0.shape[1]
        seg = A_seg_len
        DF = B_w_gate.shape[1]
        hbm = pl.BlockSpec(memory_space=pl.ANY)
        packed = lambda r, c: pltpu.VMEM((r // 2, c), U32)
        proj = pltpu.VMEM((7, Dm // 4, H * Dh // 2), U32)
        out = pl.pallas_call(
            functools.partial(kernel, M=M, seg=seg, H=H, Dh=Dh, n_seg=S // seg),
            in_specs=[hbm] * 9,
            out_specs=hbm,
            out_shape=jax.ShapeDtypeStruct((S, Dm), A_x.dtype),
            scratch_shapes=[
                proj, proj, proj,
                packed(H * Dh, Dm), packed(Dm, DF), packed(Dm, DF), packed(DF, Dm),
                pltpu.VMEM((3, H * Dh // 4, Dm // 2), U32),
                pltpu.VMEM((3, Dm // 4, DF), U32),
                pltpu.VMEM((3, DF // 4, Dm // 2), U32),
                pltpu.VMEM((NS, 2, RC * H, Dh), BF16),
                pltpu.VMEM((4 * seg, Dm), F32),
                pltpu.VMEM((4 * (M + seg) + 2 * seg, Dm), F32),
                pltpu.VMEM((S, Dm), BF16),
                pltpu.VMEM((S, Dm), F32),
                pltpu.VMEM((M, Dm), BF16),
                pltpu.SemaphoreType.DMA((NS, 2)),
                pltpu.SemaphoreType.DMA((NO,)),
                pltpu.SemaphoreType.DMA((3,)),
                pltpu.SemaphoreType.DMA((3,)),
                pltpu.SemaphoreType.DMA(()),
            ],
            compiler_params=pltpu.CompilerParams(vmem_limit_bytes=126 * 1024 * 1024),
        )(A_x.reshape(S, Dm), A_mem0.reshape(M, Dm),
          A_Wq.reshape(Dm * H, Dh), A_Wk.reshape(Dm * H, Dh), A_Wv.reshape(Dm * H, Dh),
          A_Wo.reshape(H * Dh, Dm), B_w_gate, B_w_up, B_w_down)
        return out.reshape(B, S, Dm)
    return run


_run = _build()


@functools.partial(jax.jit, static_argnames=("A_seg_len",))
def pallas_interleave_layers__memory_aug_recurrent_mem_tr__glu_gated_geglu__prompt_kernel(
    A_x, A_mem0, A_Wq, A_Wk, A_Wv, A_Wo, A_seg_len, B_x, B_w_gate, B_w_up, B_w_down
):
    return _run(A_x, A_mem0, A_Wq, A_Wk, A_Wv, A_Wo, A_seg_len, B_x, B_w_gate, B_w_up, B_w_down)
```
